```python
import jax
import jax.numpy as jnp

def _softmax(x, axis=-1):
    return jax.nn.softmax(x, axis=axis)
def _gelu(x):
    return jax.nn.gelu(x, approximate=True)
def _silu(x):
    return jax.nn.silu(x)
def _sigmoid(x):
    return jax.nn.sigmoid(x)
def _layernorm(x, axis=-1, eps=1e-5):
    m = jnp.mean(x, axis=axis, keepdims=True)
    v = jnp.var(x, axis=axis, keepdims=True)
    return (x - m) / jnp.sqrt(v + eps)
def _scatter_add(tgt, idx, src, axis=0):
    return tgt.at[idx].add(src)
def _segment_sum(src, seg, n):
    return jax.ops.segment_sum(src, seg, n)
class _Rng:
    def __init__(self, key):
        self._k = key
    def _next(self):
        self._k, sub = jax.random.split(self._k)
        return sub
    def normal(self, shape):
        return jax.random.normal(self._next(), shape, dtype=jnp.bfloat16)
    def randint(self, lo, hi, shape):
        return jax.random.randint(self._next(), shape, lo, hi, dtype=jnp.int32)
    def uniform(self, shape, lo=0.0, hi=1.0):
        return jax.random.uniform(self._next(), shape, jnp.bfloat16, lo, hi)
    def permutation(self, n):
        return jax.random.permutation(self._next(), n)


kernel_name = 'concat_heads__compressed_kv_cla__sliding_local_dilated__prompt'

def setup_inputs():
    _rng = _Rng(jax.random.key(int.from_bytes(__import__("os").urandom(4), "little")))
    _w = (lambda a: (lambda t: t.astype(jnp.bfloat16) if jnp.issubdtype(t.dtype, jnp.floating) else t)(jnp.asarray(a)))
    def _A_setup():
        B, H, Sq, Sk, D, M = 1, 32, 2048, 2048, 128, 1024
        Dc = 4 * D
        return {
            "x": _w((lambda *s: _rng.normal(s) * 0.05)(B, Sq, M)),
            "c_kv": _w((lambda *s: _rng.normal(s) * 0.05)(B, Sk, Dc)),
            "w_q": _w((lambda *s: _rng.normal(s) * 0.05)(M, H, D) * (M ** -0.5)),
            "w_uk": _w((lambda *s: _rng.normal(s) * 0.05)(Dc, H, D) * (Dc ** -0.5)),
            "w_uv": _w((lambda *s: _rng.normal(s) * 0.05)(Dc, H, D) * (Dc ** -0.5)),
            "w_o": _w((lambda *s: _rng.normal(s) * 0.05)(H, D, M) * ((H * D) ** -0.5)),
        }
    _A_in = _A_setup()

    def _B_setup():
        B, S, D = 1, 2048, 1024
        return {
            "x": _w((lambda *s: _rng.normal(s) * 0.05)(B, S, D)),
            "wqkv": _w((lambda *s: _rng.normal(s) * 0.05)(D, 3 * D)),
            "wo": _w((lambda *s: _rng.normal(s) * 0.05)(D, D)),
        }
    _B_in = _B_setup()

    return {
        "A_x": _A_in["x"],
        "A_c_kv": _A_in["c_kv"],
        "A_w_q": _A_in["w_q"],
        "A_w_uk": _A_in["w_uk"],
        "A_w_uv": _A_in["w_uv"],
        "A_w_o": _A_in["w_o"],
        "B_x": _B_in["x"],
        "B_wqkv": _B_in["wqkv"],
        "B_wo": _B_in["wo"],
    }

def reference(A_x, A_c_kv, A_w_q, A_w_uk, A_w_uv, A_w_o, B_x, B_wqkv, B_wo):
    def _A_ref(x, c_kv, w_q, w_uk, w_uv, w_o):
        B, Sq, M = x.shape[0], x.shape[1], x.shape[2]
        Sk = c_kv.shape[1]
        H, D = w_q.shape[1], w_q.shape[2]
        q = jnp.einsum("bqm,mhd->bhqd", x, w_q)
        k = jnp.einsum("bkc,chd->bhkd", c_kv, w_uk)
        v = jnp.einsum("bkc,chd->bhkd", c_kv, w_uv)
        scores = jnp.einsum("bhqd,bhkd->bhqk", q, k) * (D ** -0.5)
        off = Sk - Sq
        qi = jnp.arange(Sq)[:, None]
        kj = jnp.arange(Sk)[None, :]
        cmask = kj <= (qi + off)
        scores = jnp.where(cmask[None, None], scores, -1e9)
        p = _softmax(scores, axis=-1)
        ctx = jnp.einsum("bhqk,bhkd->bhqd", p, v)
        return jnp.einsum("bhqd,hdm->bqm", ctx, w_o)

    def _B_ref(x, wqkv, wo):
        B, S, D = x.shape
        H = 32; Dh = D // H
        W, dil = 8, 2
        qkv = (lambda x, *d: x.transpose(*d))((x @ wqkv).reshape(B, S, 3, H, Dh), 2, 0, 3, 1, 4)
        q, k, v = qkv[0], qkv[1], qkv[2]
        scale = Dh ** -0.5
        pos = jnp.arange(S)
        off = jnp.arange(W) * dil
        idx = pos[:, None] - off[None, :]
        mask = idx >= 0
        idx_c = jnp.where(mask, idx, 0).reshape(-1)
        kg = k[:, :, idx_c, :].reshape(B, H, S, W, Dh)
        vg = v[:, :, idx_c, :].reshape(B, H, S, W, Dh)
        logits = jnp.einsum("bhsd,bhswd->bhsw", q, kg) * scale
        logits = jnp.where(mask[None, None, :, :], logits, -1e9)
        attn = _softmax(logits, axis=-1)
        o = jnp.einsum("bhsw,bhswd->bhsd", attn, vg)
        return (lambda x, *d: x.transpose(*d))(o, 0, 2, 1, 3).reshape(B, S, D) @ wo

    a = _A_ref(A_x, A_c_kv, A_w_q, A_w_uk, A_w_uv, A_w_o)
    b = _B_ref(B_x, B_wqkv, B_wo)
    return jnp.concatenate([a, b], axis=-1)
```

```python
import functools

import jax
import jax.numpy as jnp
import numpy as np
from jax import lax
import jax.experimental.pallas as pl
import jax.experimental.pallas.tpu as pltpu

S = 2048
M = 1024
DC = 512
H = 32
D = 128
BQ = 128
HB = 32
DB = 32
WIN = 8
DIL = 2
HALO = 16
RC = 128
LOG2E = 1.4426950408889634
NEG = -1e9 * LOG2E

F32 = jnp.float32
BF16 = jnp.bfloat16
U32 = jnp.uint32
_NT = (((1,), (1,)), ((), ()))


def _dot(a, b):
    return jnp.dot(a, b, preferred_element_type=F32)


def _unpack_half(words, shift):
    return pltpu.bitcast((words >> shift) << 16, F32).astype(BF16)


def _permute_head_columns(w):
    words = pltpu.bitcast(w, U32)
    rows = words.shape[0]
    tiles = [words[:, t * 128:(t + 1) * 128] for t in range(8)]
    lane = lax.broadcasted_iota(jnp.int32, (rows, 128), 1)
    for bit in (1, 2, 4):
        low = (lane & bit) == 0
        for t in range(8):
            if t & bit:
                continue
            a, b = tiles[t], tiles[t | bit]
            tiles[t] = jnp.where(low, a, pltpu.roll(b, bit, 1))
            tiles[t | bit] = jnp.where(low, pltpu.roll(a, 128 - bit, 1), b)
    src = ((lane & 3) << 5) | (lane >> 2)
    tiles = [jnp.take_along_axis(x, src, axis=1) for x in tiles]
    return pltpu.bitcast(jnp.concatenate(tiles, axis=1), BF16)


def _kernel(
    xa_hbm, c_hbm, wq_hbm, wk_hbm, wv_hbm, woa_hbm, xb_hbm, wqkv_hbm, wob_hbm,
    out_hbm,
    xa, c, wq_buf, wk_buf, wv_buf, q_buf, k_buf, v_buf, ctx,
    woa, xb, wqkv_raw, wqkv, wob_raw, wob, kb, vb, obuf,
    sem_in, sem_w, sem_out,
):
    wq32 = wq_hbm.bitcast(U32)
    wk32 = wk_hbm.bitcast(U32)
    wv32 = wv_hbm.bitcast(U32)
    wob32 = wob_hbm.bitcast(U32)

    def head_copies(h, slot):
        pair = h // 2
        r0 = pl.multiple_of(h * (M // H), M // H)
        return (
            pltpu.make_async_copy(wk32.at[:, pair, :], wk_buf.at[slot], sem_w.at[slot, 0]),
            pltpu.make_async_copy(wv32.at[:, pair, :], wv_buf.at[slot], sem_w.at[slot, 1]),
            pltpu.make_async_copy(wq32.at[:, pair, :], wq_buf.at[slot], sem_w.at[slot, 2]),
            pltpu.make_async_copy(
                wqkv_hbm.at[pl.ds(r0, M // H), :], wqkv_raw.at[slot], sem_w.at[slot, 3]),
            pltpu.make_async_copy(wob32.at[:, pair, :], wob_raw.at[slot], sem_w.at[slot, 4]),
        )

    c_copy = pltpu.make_async_copy(c_hbm, c, sem_in.at[0])
    xa_copy = pltpu.make_async_copy(xa_hbm, xa, sem_in.at[1])
    woa_copy = pltpu.make_async_copy(woa_hbm, woa, sem_in.at[2])
    xb_copy = pltpu.make_async_copy(xb_hbm, xb, sem_in.at[3])

    c_copy.start()
    for cp in head_copies(0, 0):
        cp.start()
    xa_copy.start()
    kb[:, 0:HALO, :] = jnp.zeros((8, HALO, 128), F32)
    vb[:, 0:HALO, :] = jnp.zeros((8, HALO, 128), F32)
    c_copy.wait()
    xa_copy.wait()
    woa_copy.start()
    xb_copy.start()

    def head_body(h, carry):
        slot = h % 2

        @pl.when(h + 1 < H)
        def _():
            for cp in head_copies(h + 1, 1 - slot):
                cp.start()

        for cp in head_copies(h, slot):
            cp.wait()

        shift = (slot * 16).astype(U32)
        wkv = jnp.concatenate(
            [_unpack_half(wk_buf[slot], shift), _unpack_half(wv_buf[slot], shift)], axis=1)
        wq = _unpack_half(wq_buf[slot], shift)

        kv = _dot(c[...], wkv)
        k_buf[...] = kv[:, :D].astype(BF16)
        v_buf[...] = kv[:, D:].astype(BF16)
        q_buf[...] = (_dot(xa[...], wq) * (D ** -0.5 * LOG2E)).astype(BF16)

        r0 = pl.multiple_of(h * (M // H), M // H)
        for part in range(3):
            wqkv[pl.ds(r0, M // H), part * M:(part + 1) * M] = _permute_head_columns(
                wqkv_raw[slot, :, part * M:(part + 1) * M])
        d0 = pl.multiple_of((h % 8) * 128 + (h // 8) * HB, HB)
        wob[pl.ds(d0, HB), :] = _unpack_half(wob_raw[slot], shift)

        row = lax.broadcasted_iota(jnp.int32, (BQ, BQ), 0)
        col = lax.broadcasted_iota(jnp.int32, (BQ, BQ), 1)
        causal = col <= row

        def scores(i):
            r = i * BQ
            s = lax.dot_general(q_buf[r:r + BQ, :], k_buf[0:r + BQ, :], _NT,
                                preferred_element_type=F32)
            diag = jnp.where(causal, s[:, r:], NEG)
            s = jnp.concatenate([s[:, :r], diag], axis=1) if r else diag
            return s, jnp.max(s, axis=1, keepdims=True)

        def weighted(i, s, m):
            r = i * BQ
            p = jnp.exp2(s - m)
            l = jnp.sum(p, axis=1, keepdims=True)
            o = _dot(p.astype(BF16), v_buf[0:r + BQ, :])
            ctx[h, r:r + BQ, :] = (o * (1.0 / l)).astype(BF16)

        pending = None
        for i in range(S // BQ):
            cur = (i,) + scores(i)
            if pending is not None:
                weighted(*pending)
            pending = cur
        weighted(*pending)
        return carry

    lax.fori_loop(0, H, head_body, 0)

    woa_copy.wait()
    xb_copy.wait()

    n_chunks = S // RC

    def out_copy(i, slot):
        r0 = pl.multiple_of(i * RC, RC)
        return pltpu.make_async_copy(obuf.at[slot], out_hbm.at[pl.ds(r0, RC), :], sem_out.at[slot])

    def chunk_body(i, carry):
        slot = i % 2
        r0 = pl.multiple_of(i * RC, RC)

        @pl.when(i >= 2)
        def _():
            out_copy(i - 2, slot).wait()

        x = xb[pl.ds(r0, RC), :]
        k = _dot(x, wqkv[:, M:2 * M])
        q = _dot(x, wqkv[:, 0:M]) * (DB ** -0.5 * LOG2E)
        v = _dot(x, wqkv[:, 2 * M:3 * M])
        for t in range(8):
            kb[t, pl.ds(r0 + HALO, RC), :] = k[:, t * 128:(t + 1) * 128]
            vb[t, pl.ds(r0 + HALO, RC), :] = v[:, t * 128:(t + 1) * 128]

        a = jnp.concatenate([ctx[hh, pl.ds(r0, RC), :] for hh in range(H)], axis=1)
        obuf[slot, :, 0:M] = _dot(a, woa[...]).astype(BF16)

        pos = r0 + lax.broadcasted_iota(jnp.int32, (RC, 128), 0)
        logits = []
        for w in range(WIN):
            acc = None
            for t in range(8):
                term = q[:, t * 128:(t + 1) * 128] * kb[t, pl.ds(r0 + HALO - DIL * w, RC), :]
                acc = term if acc is None else acc + term
            acc = acc + pltpu.roll(acc, 64, 1)
            acc = acc + pltpu.roll(acc, 32, 1)
            logits.append(jnp.where(pos >= DIL * w, acc, NEG) if w else acc)
        top = functools.reduce(jnp.maximum, logits)
        probs = [jnp.exp2(z - top) for z in logits]
        inv = 1.0 / functools.reduce(jnp.add, probs)
        probs = [p * inv for p in probs]
        cols = []
        for t in range(8):
            acc = None
            for w in range(WIN):
                term = probs[w] * vb[t, pl.ds(r0 + HALO - DIL * w, RC), :]
                acc = term if acc is None else acc + term
            cols.append(acc.astype(BF16))
        obuf[slot, :, M:2 * M] = _dot(jnp.concatenate(cols, axis=1), wob[...]).astype(BF16)

        out_copy(i, slot).start()
        return carry

    lax.fori_loop(0, n_chunks, chunk_body, 0)
    out_copy(n_chunks - 2, 0).wait()
    out_copy(n_chunks - 1, 1).wait()


@jax.jit
def pallas_concat_heads__compressed_kv_cla__sliding_local_dilated__prompt_kernel(
    A_x: jax.Array,
    A_c_kv: jax.Array,
    A_w_q: jax.Array,
    A_w_uk: jax.Array,
    A_w_uv: jax.Array,
    A_w_o: jax.Array,
    B_x: jax.Array,
    B_wqkv: jax.Array,
    B_wo: jax.Array,
):
    scratch = [
        pltpu.VMEM((S, M), BF16),
        pltpu.VMEM((S, DC), BF16),
        pltpu.VMEM((2, M, D), U32),
        pltpu.VMEM((2, DC, D), U32),
        pltpu.VMEM((2, DC, D), U32),
        pltpu.VMEM((S, D), BF16),
        pltpu.VMEM((S, D), BF16),
        pltpu.VMEM((S, D), BF16),
        pltpu.VMEM((H, S, D), BF16),
        pltpu.VMEM((H * D, M), BF16),
        pltpu.VMEM((S, M), BF16),
        pltpu.VMEM((2, M // H, 3 * M), BF16),
        pltpu.VMEM((M, 3 * M), BF16),
        pltpu.VMEM((2, HB, M), U32),
        pltpu.VMEM((M, M), BF16),
        pltpu.VMEM((8, HALO + S, 128), F32),
        pltpu.VMEM((8, HALO + S, 128), F32),
        pltpu.VMEM((2, RC, 2 * M), BF16),
        pltpu.SemaphoreType.DMA((4,)),
        pltpu.SemaphoreType.DMA((2, 5)),
        pltpu.SemaphoreType.DMA((2,)),
    ]
    out = pl.pallas_call(
        _kernel,
        out_shape=jax.ShapeDtypeStruct((S, 2 * M), BF16),
        in_specs=[pl.BlockSpec(memory_space=pl.ANY)] * 9,
        out_specs=pl.BlockSpec(memory_space=pl.ANY),
        scratch_shapes=scratch,
        compiler_params=pltpu.CompilerParams(vmem_limit_bytes=110 * 2**20),
        name="fused_mla_sliding",
    )(
        A_x.reshape(S, M),
        A_c_kv.reshape(S, DC),
        A_w_q,
        A_w_uk,
        A_w_uv,
        A_w_o.reshape(H * D, M),
        B_x.reshape(S, M),
        B_wqkv,
        B_wo.reshape(HB, DB, M),
    )
    return out.reshape(1, S, 2 * M)
```

```python
import functools

import jax
import jax.numpy as jnp
import numpy as np
from jax import lax
import jax.experimental.pallas as pl
import jax.experimental.pallas.tpu as pltpu

S = 2048
M = 1024
DC = 512
H = 32
NP = H // 2
D = 128
BQ = 128
G = 512
NG = S // G
HB = 32
DB = 32
WIN = 8
DIL = 2
HALO = 16
RC = 256
PP = 2
NS = NP // PP
LAG0 = 4
LAG2 = 6
SCHED = "v0,Sa0,Sa1,Sa2,Sa3,k1,Pa0,Pa1,Pa2,v1,Sa4,Pa3,Sa5,k2,Wa0,Wa1,Pa4,Sa6,Wa2,Pa5,Wa3,Sa7,Pa6,Wa4,v2,Sa8,Pa7,Wa5,k3,Sa9,Pa8,Wa6,Sa10,Pa9,Wa7,v3,Sa11,Pa10,Wa8,Sa12,Pa11,Wa9,Nk,Nv,Sa13,Pa12,Wa10,Sa14,Pa13,Wa11,Sa15,Sb0,Sb1,Pa14,Wa12,Sb2,Sb3,Pa15,Wa13,Pb0,Pb1,Sb4,Pb2,Pb3,Wa14,Sb5,Pb4,Wa15,Wb0,Wb1,Sb6,Wb2,Pb5,Wb3,Sb7,Pb6,Wb4,Sb8,Pb7,Wb5,Sb9,Pb8,Wb6,Sb10,Pb9,Wb7,Sb11,Pb10,Wb8,Sb12,Pb11,Wb9,Sb13,Pb12,Wb10,Sb14,Wb11,Pb13,Wb12,Sb15,Pb14,k0,Pb15,Wb13,Wb14,Wb15"
SCHED00 = "F0,X0,X1,Z,f,I,x0,X2,y0,q0,x1,X3,T0,y1,q1,x2,F1,T1,y2,q2,x3,t,F2,T2,y3,Q3"
LOG2E = 1.4426950408889634
NEG = -1e9 * LOG2E

F32 = jnp.float32
BF16 = jnp.bfloat16
U32 = jnp.uint32
_NT = (((1,), (1,)), ((), ()))

W = M // 2
OA_ROWS, B_ROWS = H * D // 4, M // 4
GATE0 = 0
OA0 = GATE0 + 8 * 7 * NG
QKV0 = OA0 + 7 * OA_ROWS
OB0 = QKV0 + 21 * B_ROWS
CS0 = OB0 + 7 * B_ROWS
PR0 = CS0 + 5 * RC
LOC0 = PR0 + 2 * RC
WIDE_ROWS = LOC0 + 2 * RC


def _dot(a, b):
    return jnp.dot(a, b, preferred_element_type=F32)


def _bf(words):
    return pltpu.bitcast(words, BF16)


def _words(x):
    return pltpu.bitcast(x.astype(BF16), U32)


def _recip(x):
    r = pl.reciprocal(x, approx=True)
    return r * (2.0 - x * r)


def _halves(words):
    return (pltpu.bitcast(words << 16, F32),
            pltpu.bitcast(words & np.uint32(0xFFFF0000), F32))


def _pack(lo, hi):
    return pltpu.bitcast(pltpu.pack_elementwise([lo, hi], packed_dtype=BF16), U32)


def _on_words(fn, *blocks):
    parts = [_halves(b) for b in blocks]
    return [_pack(lo, hi) for lo, hi in zip(fn(*[x[0] for x in parts]), fn(*[x[1] for x in parts]))]


def _words_shuffled(x):
    n, c = x.shape
    x = x.reshape(n // 16, 2, 8, c)
    return _pack(x[:, 0], x[:, 1]).reshape(n // 2, c)


def _lhs_sums(a11, a12, a21, a22):
    return a11 + a22, a21 + a22, a11 + a12, a21 - a11, a12 - a22


def _lhs_factors(a11, a22, sums):
    return sums[0], sums[1], a11, a22, sums[2], sums[3], sums[4]


def _rhs_sums(b11, b12, b21, b22):
    return b11 + b22, b12 - b22, b21 - b11, b11 + b12, b21 + b22


def _rhs_factors(b11, b12, b21, b22):
    s = _rhs_sums(b11, b12, b21, b22)
    return s[0], b11, s[1], s[2], b22, s[3], s[4]


def _rhs_factors_of_words(b11, b12, b21, b22):
    s = _on_words(_rhs_sums, b11, b12, b21, b22)
    return s[0], b11, s[1], s[2], b22, s[3], s[4]


def _strassen(mul):
    m3 = mul(2)
    m4 = mul(3)
    m5 = mul(4)
    c12 = m3 + m5
    m2 = mul(1)
    c21 = m2 + m4
    m1 = mul(0)
    c11 = (m4 - m5) + m1 + mul(6)
    c22 = (m3 - m2) + m1 + mul(5)
    return c11, c12, c21, c22


def _with_corner(x, corner):
    top = corner if x.shape[1] == 128 else jnp.concatenate([corner, x[0:8, 128:]], axis=1)
    return jnp.concatenate([top, x[8:]], axis=0)


class _SideWork:
    def __init__(self):
        self.now = 0
        self.starts = {}
        self.stores = {}

    def add(self, tasks, first, last, lag):
        for n, task in enumerate(tasks):
            when = first + n * (last - lag - first) // len(tasks)
            self.starts.setdefault(when, []).append((task, lag))

    def step(self):
        for task, lag in self.starts.pop(self.now, []):
            self.stores.setdefault(self.now + lag, []).extend(task())
        for ref, idx, val in self.stores.pop(self.now, []):
            ref[idx] = val
        self.now += 1

    @property
    def done(self):
        return not self.starts and not self.stores


def _permute_head_columns(words):
    rows = words.shape[0]
    tiles = [words[:, t * 128:(t + 1) * 128] for t in range(8)]
    lane = lax.broadcasted_iota(jnp.int32, (rows, 128), 1)
    for bit in (1, 2, 4):
        low = (lane & bit) == 0
        for t in range(8):
            if t & bit:
                continue
            a, b = tiles[t], tiles[t | bit]
            tiles[t] = jnp.where(low, a, pltpu.roll(b, bit, 1))
            tiles[t | bit] = jnp.where(low, pltpu.roll(a, 128 - bit, 1), b)
    src = ((lane & 3) << 5) | (lane >> 2)
    return jnp.concatenate([jnp.take_along_axis(x, src, axis=1) for x in tiles], axis=1)


def _mult(i, n):
    return i * n if isinstance(i, int) else pl.multiple_of(i * n, n)


def _cols(t):
    return slice(t * 128, (t + 1) * 128)


def _kernel(
    xa_hbm, c_hbm, wq_hbm, wk_hbm, wv_hbm, woa_hbm, xb_hbm, wqkv_hbm, wob_hbm,
    out_hbm,
    xa, xa_sum, wide, c, c_sum, wq_raw, wk_raw, wv_raw, wq_f, wk_f, wv_f, k_buf, v_buf, ctx,
    woa, xb, wqkv, wob_raw, qb, kb, vb, obuf,
    sem_x, sem_q, sem_t, sem_misc, sem_out,
):
    xa32, c32, woa32, xb32, wqkv32 = (
        r.bitcast(U32) for r in (xa_hbm, c_hbm, woa_hbm, xb_hbm, wqkv_hbm))
    wq32 = wq_hbm.bitcast(U32)
    wk32 = wk_hbm.bitcast(U32)
    wv32 = wv_hbm.bitcast(U32)
    wob32 = wob_hbm.bitcast(U32)

    def rows_copy(src, dst, start, n, sem):
        return pltpu.make_async_copy(src.at[pl.ds(start, n), :], dst.at[pl.ds(start, n), :], sem)

    def pair_copies(src, dst, step, sem):
        return [pltpu.make_async_copy(src.at[:, step * PP + j, :], dst.at[step * PP + j], sem)
                for j in range(PP)]

    def wq_copies(step):
        return pair_copies(wq32, wq_raw, step, sem_q.at[step])

    def tail_copies(step):
        n, sem = M // 4 // NS, sem_t.at[step]
        return pair_copies(wob32, wob_raw, step, sem) + [
            rows_copy(wqkv32, wqkv, _mult(step, n), n, sem),
            rows_copy(wqkv32, wqkv, M // 4 + _mult(step, n), n, sem),
            rows_copy(woa32, woa, _mult(step, PP * D), PP * D, sem)]

    def kv_copies(step):
        sem = sem_misc.at[0]
        return (pair_copies(wk32, wk_raw, step, sem) + pair_copies(wv32, wv_raw, step, sem)
                + [rows_copy(c32, c, _mult(step, S // 2 // NS), S // 2 // NS, sem)])

    x_copies = [rows_copy(xa32, xa, g * G // 2, G // 2, sem_x.at[g]) for g in range(NG)]
    xb_copy = pltpu.make_async_copy(xb32, xb, sem_misc.at[1])

    gw = G // 4

    def make_sums(raw, sums, g):
        k2 = raw.shape[1] // 2
        blocks = [raw[(2 * g + r) * gw:(2 * g + r + 1) * gw, k * k2:(k + 1) * k2]
                  for r in range(2) for k in range(2)]
        for j, val in enumerate(_on_words(_lhs_sums, *blocks)):
            sums[j, g * gw:(g + 1) * gw, :] = val

    def left_factor(raw, sums, j, g):
        k2 = raw.shape[1] // 2
        if j in (2, 3):
            r = j - 2
            return raw[(2 * g + r) * gw:(2 * g + r + 1) * gw, r * k2:(r + 1) * k2]
        return sums[j if j < 2 else j - 2, g * gw:(g + 1) * gw, :]

    def right_factors(raw, pair):
        k2 = raw.shape[1] // 2
        return _rhs_factors(*_halves(raw[pair, 0:k2, :]), *_halves(raw[pair, k2:2 * k2, :]))

    def blocks_of(g, mul):
        for n, val in enumerate(_strassen(mul)):
            r, e = divmod(n, 2)
            yield e, slice((2 * g + r) * gw, (2 * g + r + 1) * gw), val

    def project_kv(kind, g):
        fac, buf = (wk_f, k_buf) if kind == "k" else (wv_f, v_buf)
        for e, rows, val in blocks_of(
                g, lambda j: _dot(_bf(left_factor(c, c_sum, j, g)), _bf(fac[j]))):
            val = _words_shuffled(val)
            buf[e, rows, :] = val
            if kind == "k" and rows.start == 0:
                ctx[H + e, 0:BQ // 2, :] = val[0:BQ // 2]

    def prepare_kv(kind, pair):
        raw, fac = (wk_raw, wk_f) if kind == "k" else (wv_raw, wv_f)
        for j, val in enumerate(right_factors(raw, pair)):
            fac[j] = _words(val)

    def prepare_wqkv(r, part):
        cols = slice(part * M, (part + 1) * M)
        both = _permute_head_columns(jnp.concatenate(
            [wqkv[pl.ds(r, 8), cols], wqkv[pl.ds(M // 4 + r, 8), cols]], axis=0))
        vals = _rhs_factors_of_words(both[:8, :W], both[:8, W:], both[8:, :W], both[8:, W:])
        return [(wide, (pl.ds(QKV0 + (7 * part + j) * B_ROWS + r, 8), slice(None)), val)
                for j, val in enumerate(vals)]

    def prepare_wob(p, t):
        b11, b21 = _halves(wob_raw[p, :, _cols(t)])
        b12, b22 = _halves(wob_raw[p, :, _cols(4 + t)])
        r = _mult((p & 3) * 4 + (p >> 2), HB // 2)
        return [(wide, (pl.ds(OB0 + j * B_ROWS + r, HB // 2), _cols(t)), _words(val))
                for j, val in enumerate(_rhs_factors(b11, b12, b21, b22))]

    def prepare_woa(p, n):
        vals = _rhs_factors_of_words(*[
            woa[pl.ds(_mult(2 * p + e, D // 2) + 8 * n, 8), k * W:(k + 1) * W]
            for e in range(2) for k in range(2)])
        return [(wide, (pl.ds(OA0 + j * OA_ROWS + _mult(p, D // 2) + 8 * n, 8), slice(None)), val)
                for j, val in enumerate(vals)]

    def tail_tasks(step):
        tasks = []
        for p in (step * PP + j for j in range(PP)):
            for n in range(8):
                tasks.append(functools.partial(prepare_woa, p, n))
                if n < 6:
                    tasks.append(functools.partial(prepare_wqkv, _mult(p, 16) + 8 * (n // 3), n % 3))
                if n % 2:
                    tasks.append(functools.partial(prepare_wob, p, n // 2))
        return tasks

    def gate(g, j):
        r = GATE0 + 8 * (7 * g + j)
        return slice(r, r + 8), _cols(0)

    def project_q(pair, g, fac, side=None):
        def mul(j):
            lhs = left_factor(xa, xa_sum, j, g)
            if side is None:
                return _dot(_bf(lhs), fac(j))
            side.step()
            val = _dot(_bf(_with_corner(lhs, wide[gate(g, j)])), fac(j))
            wqkv[M // 2:M // 2 + 8, _cols(0)] = pltpu.bitcast(val[0:8], U32)
            return val

        for e, rows, val in blocks_of(g, mul):
            ctx[2 * pair + e, rows, :] = _words(val * (D ** -0.5 * LOG2E))

    def start(copies):
        for cp in copies:
            cp.start()

    def wait(copies):
        for cp in copies:
            cp.wait()

    with jax.named_scope("peel"):
        for op in SCHED00.split(","):
            kind, arg = op[0], op[1:]
            if kind == "I":
                for p in range(PP):
                    for j, val in enumerate(right_factors(wq_raw, p)):
                        wq_f[p, j] = _words(val)
            elif kind in "qQ":
                side = None
                if kind == "Q":
                    side = _SideWork()
                    side.add(tail_tasks(0), 0, 7 * PP - 1, 2)
                for p in range(PP):
                    project_q(p, int(arg), lambda j, p=p: _bf(wq_f[p, j]), side)
                assert side is None or side.done
            elif kind == "X":
                x_copies[int(arg)].start()
            elif kind == "x":
                x_copies[int(arg)].wait()
            elif kind == "y":
                make_sums(xa, xa_sum, int(arg))
                for j in range(7):
                    wide[gate(int(arg), j)] = left_factor(xa, xa_sum, j, int(arg))[0:8, 0:128]
            elif kind == "F":
                start(wq_copies(int(arg)))
            elif kind == "f":
                wait(wq_copies(0))
            elif kind == "T":
                start(tail_copies(int(arg)))
            elif kind == "t":
                wait(tail_copies(0))
            elif kind == "Z":
                kb[:, RC:RC + HALO, :] = jnp.zeros((8, HALO, 128), F32)
                vb[:, RC:RC + HALO, :] = jnp.zeros((8, HALO, 128), F32)
            else:
                raise ValueError(op)
        start(kv_copies(0))

    def q_body(step, _):
        @pl.when(step + 2 < NS)
        def _():
            start(wq_copies(step + 2) + tail_copies(step + 2))

        start(kv_copies(step))
        wait(wq_copies(step) + tail_copies(step))
        side = _SideWork()
        side.add(tail_tasks(step), 2, 7 * NG * PP - 1, LAG0)
        for p in (step * PP + j for j in range(PP)):
            fac = [val.astype(BF16) for val in right_factors(wq_raw, p)]
            for g in range(NG):
                project_q(p, g, fac.__getitem__, side)
        assert side.done

    with jax.named_scope("phase0"):
        lax.fori_loop(1, NS, q_body, None)

    with jax.named_scope("bridge"):
        for step in range(NS):
            wait(kv_copies(step))
        xb_copy.start()
        prepare_kv("k", 0)
        for g in range(NG):
            make_sums(c, c_sum, g)
        project_kv("k", 0)
        prepare_kv("v", 0)

    def pair_body(p, kslot):
        nxt = jnp.minimum(p + 1, NP - 1)
        row = lax.broadcasted_iota(jnp.int32, (BQ, BQ), 0)
        col = lax.broadcasted_iota(jnp.int32, (BQ, BQ), 1)
        causal = ((col & ~15) | ((col & 15) >> 1) | ((col & 1) << 3)) <= row
        hb = BQ // 2

        def scores(e, i):
            r = i * BQ
            k = ctx[kslot + e, 0:hb, :]
            k = _bf(jnp.concatenate([k, k_buf[e, hb:(i + 1) * hb, :]], axis=0) if i else k)
            q = _bf(ctx[2 * p + e, i * hb:(i + 1) * hb, :])
            s = lax.dot_general(q, k, _NT, preferred_element_type=F32)
            diag = jnp.where(causal, s[:, r:], NEG)
            s = jnp.concatenate([s[:, :r], diag], axis=1) if r else diag
            return s, jnp.max(s, axis=1, keepdims=True)

        def weighted(e, i, s, m):
            w = jnp.exp2(s - m)
            l = jnp.sum(w, axis=1, keepdims=True)
            o = _dot(w.astype(BF16), _bf(v_buf[e, 0:(i + 1) * hb, :]))
            return _words(o * _recip(l))

        state = {}
        for op in SCHED.split(","):
            kind, arg = op[0], op[1:]
            if kind in "kv":
                project_kv(kind, int(arg))
            elif kind == "N":
                prepare_kv(arg, nxt)
            else:
                e, i = "ab".index(arg[0]), int(arg[1:])
                if kind == "S":
                    state[e, i] = scores(e, i)
                elif kind == "P":
                    state[e, i] = weighted(e, i, *state[e, i])
                else:
                    ctx[2 * p + e, i * hb:(i + 1) * hb, :] = state.pop((e, i))
        assert not state
        return 2 * H - kslot

    with jax.named_scope("phase1"):
        lax.fori_loop(0, NP, pair_body, H)

    xb_copy.wait()

    n_chunks = S // RC
    hr = RC // 2

    def out_copy(i, slot):
        return pltpu.make_async_copy(
            obuf.at[slot], out_hbm.at[pl.ds(_mult(i, RC), RC), :], sem_out.at[slot])

    def chunk_body(i, zero):
        slot = i & 1

        @pl.when(i >= 2)
        def _():
            out_copy(i, slot).wait()

        def half_rows(r, lo=0, n=hr // 2):
            return pl.ds(_mult(i, hr) + r * (hr // 2) + lo, n)

        def ctx_block(r, e, kk, lo=0, n=hr // 2):
            return jnp.concatenate(
                [ctx[2 * (4 * kk + u) + e, half_rows(r, lo, n), :] for u in range(4)], axis=1)

        def ctx_sums(kk, lo):
            vals = _on_words(_lhs_sums, *[ctx_block(r, e, kk, lo, 8) for r in range(2) for e in range(2)])
            return [(wide, (slice(CS0 + j * RC + kk * (hr // 2) + lo, CS0 + j * RC + kk * (hr // 2) + lo + 8),
                            slice(None)), val) for j, val in enumerate(vals)]

        def taps(buf, t, w, r):
            return buf[t, HALO - DIL * w + r:HALO - DIL * w + r + 8, :]

        def weight_at(r, w):
            return slice(PR0 + (w // 4) * RC + r, PR0 + (w // 4) * RC + r + 8), _cols(w % 4)

        def window_weights(r):
            q = [qb[t + zero, HALO + r:HALO + r + 8, :] for t in range(8)]
            logits = [functools.reduce(jnp.add, [q[t] * taps(kb, t, w, r) for t in range(8)])
                      for w in range(WIN)]
            logits = [z + pltpu.roll(z, 64, 1) for z in logits]
            logits = [(z + pltpu.roll(z, 32, 1)) * (DB ** -0.5 * LOG2E) for z in logits]
            pos = i * RC + r + lax.broadcasted_iota(jnp.int32, (8, 128), 0)
            logits = [jnp.where(pos >= DIL * w, z, NEG) if DIL * w > r else z
                      for w, z in enumerate(logits)]
            peak = functools.reduce(jnp.maximum, logits)
            probs = [jnp.exp2(z - peak) for z in logits]
            inv = _recip(functools.reduce(jnp.add, probs))
            return [(wide, weight_at(r, w), pltpu.bitcast(z * inv, U32)) for w, z in enumerate(probs)]

        def window_values(r):
            probs = [pltpu.bitcast(wide[weight_at(r, w)], F32) for w in range(WIN)]
            r1 = LOC0 + 2 * (r // hr) * hr + r % hr
            return [(wide, (slice(r1 + (t % 2) * hr, r1 + (t % 2) * hr + 8), _cols(t // 2)),
                     pltpu.bitcast(functools.reduce(
                         jnp.add, [probs[w] * taps(vb, t, w, r) for w in range(WIN)]), U32))
                    for t in range(8)]

        side = _SideWork()
        P = functools.partial
        side.add([P(ctx_sums, kk, lo) for kk in range(4) for lo in range(0, hr // 2, 8)], 14, 58, 0)
        side.add([P(window_weights, r) for r in range(0, RC, 8)], 59, 130, LAG2)
        side.add([P(window_values, r) for r in range(0, RC, 8)], 131, 195, 0)

        def mul(lhs, row0, t):
            side.step()
            rhs = _with_corner(wide[row0:row0 + B_ROWS, _cols(t)],
                               wide[pl.ds(row0 + _mult(zero, 8), 8), _cols(t)])
            val = _dot(lhs, _bf(rhs))
            qb[0, 0:8, :] = val[0:8]
            return val

        x = [xb[half_rows(r), k * W:(k + 1) * W] for r in range(2) for k in range(2)]
        x_fac = [_bf(z) for z in _lhs_factors(x[0], x[3], _on_words(_lhs_sums, *x))]
        for part, buf in ((1, kb), (0, qb), (2, vb)):
            if part:
                buf[:, 0:HALO, :] = buf[:, RC:RC + HALO, :]
            for t in range(4):
                blocks = _strassen(lambda j: mul(x_fac[j], QKV0 + (7 * part + j) * B_ROWS, t))
                for n, val in enumerate(blocks):
                    r, k = divmod(n, 2)
                    buf[4 * k + t, HALO + r * hr:HALO + (r + 1) * hr, :] = val

        def ctx_factor(j, kk):
            if j in (2, 3):
                return ctx_block(j - 2, j - 2, kk)
            r = CS0 + (j if j < 2 else j - 2) * RC + kk * (hr // 2)
            return wide[r:r + hr // 2, :]

        def store_out(col0, t, blocks):
            for n, val in enumerate(blocks):
                r, k = divmod(n, 2)
                lo = col0 + k * W + t * 128
                obuf[slot, r * hr:(r + 1) * hr, lo:lo + 128] = val.astype(BF16)

        for t in range(4):
            store_out(0, t, _strassen(lambda j: functools.reduce(jnp.add, [
                mul(_bf(ctx_factor(j, kk)), OA0 + j * OA_ROWS + kk * B_ROWS, t) for kk in range(4)])))
        assert side.done

        o = [pltpu.bitcast(wide[LOC0 + n * hr:LOC0 + (n + 1) * hr, :], F32) for n in range(4)]
        o_fac = [z.astype(BF16) for z in _lhs_factors(o[0], o[3], _lhs_sums(*o))]
        for t in range(4):
            store_out(M, t, _strassen(lambda j: _dot(
                o_fac[j], _bf(wide[OB0 + j * B_ROWS:OB0 + (j + 1) * B_ROWS, _cols(t)]))))

        out_copy(i, slot).start()
        return -zero

    with jax.named_scope("phase2"):
        lax.fori_loop(0, n_chunks, chunk_body, 0)
    with jax.named_scope("tail"):
        out_copy(n_chunks - 2, 0).wait()
        out_copy(n_chunks - 1, 1).wait()


@jax.jit
def pallas_concat_heads__compressed_kv_cla__sliding_local_dilated__prompt_kernel(
    A_x, A_c_kv, A_w_q, A_w_uk, A_w_uv, A_w_o, B_x, B_wqkv, B_wo,
):
    scratch = [
        pltpu.VMEM((S // 2, M), U32),
        pltpu.VMEM((5, S // 4, M // 2), U32),
        pltpu.VMEM((WIDE_ROWS, W), U32),
        pltpu.VMEM((S // 2, DC), U32),
        pltpu.VMEM((5, S // 4, DC // 2), U32),
        pltpu.VMEM((NP, M, D), U32),
        pltpu.VMEM((NP, DC, D), U32),
        pltpu.VMEM((NP, DC, D), U32),
        pltpu.VMEM((PP, 7, M // 4, D), U32),
        pltpu.VMEM((7, DC // 4, D), U32),
        pltpu.VMEM((7, DC // 4, D), U32),
        pltpu.VMEM((2, S // 2, D), U32),
        pltpu.VMEM((2, S // 2, D), U32),
        pltpu.VMEM((H + 2, S // 2, D), U32),
        pltpu.VMEM((H * D // 2, M), U32),
        pltpu.VMEM((S // 2, M), U32),
        pltpu.VMEM((M // 2 + 8, 3 * M), U32),
        pltpu.VMEM((DB // 2, HB, M), U32),
        pltpu.VMEM((8, HALO + RC, 128), F32),
        pltpu.VMEM((8, HALO + RC, 128), F32),
        pltpu.VMEM((8, HALO + RC, 128), F32),
        pltpu.VMEM((2, RC, 2 * M), BF16),
        pltpu.SemaphoreType.DMA((NG,)),
        pltpu.SemaphoreType.DMA((NS,)),
        pltpu.SemaphoreType.DMA((NS,)),
        pltpu.SemaphoreType.DMA((2,)),
        pltpu.SemaphoreType.DMA((2,)),
    ]
    out = pl.pallas_call(
        _kernel,
        out_shape=jax.ShapeDtypeStruct((S, 2 * M), BF16),
        in_specs=[pl.BlockSpec(memory_space=pl.ANY)] * 9,
        out_specs=pl.BlockSpec(memory_space=pl.ANY),
        scratch_shapes=scratch,
        compiler_params=pltpu.CompilerParams(vmem_limit_bytes=126 * 2**20, disable_bounds_checks=True),
        name="fused_mla_sliding",
    )(
        A_x.reshape(S, M),
        A_c_kv.reshape(S, DC),
        A_w_q,
        A_w_uk,
        A_w_uv,
        A_w_o.reshape(H * D, M),
        B_x.reshape(S, M),
        B_wqkv,
        B_wo.reshape(HB, DB, M),
    )
    return out.reshape(1, S, 2 * M)
```

```python
import functools

import jax
import jax.numpy as jnp
import numpy as np
from jax import lax
import jax.experimental.pallas as pl
import jax.experimental.pallas.tpu as pltpu

S = 2048
M = 1024
DC = 512
H = 32
NP = H // 2
D = 128
BQ = 128
G = 512
NG = S // G
HB = 32
DB = 32
WIN = 8
DIL = 2
HALO = 16
RC = 256
PP = 2
NS = NP // PP
RING = 4
PAD = 8
E1 = 6
E2 = 62
E3 = 124
ROT = 0
TREE = 0
E4 = 70
XSPLIT = 1
SKIP0 = 4
SKIP1 = 0
LAG1 = 3
SUB0 = 1
JS = [((2, 3, 4, 1), (0, 5, 6)), ((2, 4, 5), (3, 1, 0, 6)), ((2, 3), (4, 1), (0, 5), (6,))][E('JS', 1)]
WT = 1
MB = 0
LAG0 = 3
LAG2 = 6
SCHED = "Sa0,Sa1,Sa2,Sa3,v0,k1,Pa0,Pa1,Pa2,v1,Sa4,Pa3,k2,Sa5,Wa0,Wa1,Pa4,v2,Sa6,Wa2,Pa5,Wa3,k3,Sa7,Pa6,Wa4,v3,Sa8,Pa7,Wa5,Sa9,Pa8,Wa6,Sa10,Pa9,Wa7,Sa11,Pa10,Wa8,Sa12,Pa11,Wa9,Sa13,Pa12,Wa10,Sa14,Pa13,Wa11,Sa15,Pa14,Wa12,Sb15,Pa15,Wa13,Sb14,Pb15,Wa14,Sb13,Pb14,Wa15,Sb12,Pb13,Wb15,Sb11,Pb12,Wb14,Sb10,Pb11,Wb13,Sb9,Pb10,Wb12,Sb8,Pb9,Wb11,Sb7,Pb8,Wb10,Sb6,Pb7,Wb9,Sb5,Pb6,Wb8,Sb4,Pb5,Wb7,Sb3,Sb2,Pb4,Wb6,Sb1,Sb0,Pb3,Pb2,k0,Pb1,Pb0,Wb5,Wb4,Wb3,Wb2,Wb1,Wb0"
SCHED00 = "F0,X0,X1,F1,X2,X3,U1,T0,T1,Z,f0,I0,x0,y0,q00,x1,y1,q01,f1,Q10,q11,x2,x3,y2,q02,q12,y3,q03,q13"
LOG2E = 1.4426950408889634
NEG = -1e9 * LOG2E

F32 = jnp.float32
BF16 = jnp.bfloat16
U32 = jnp.uint32
_NT = (((1,), (1,)), ((), ()))

W = M // 2
SLAB = M // 4
OA0 = 0
QKV0 = OA0 + 49
OB0 = QKV0 + 21
CS0 = OB0 + 7
PR0 = CS0 + 13
LOC0 = PR0 + 2
GATE = LOC0 + 2
N_SLABS = GATE + 1


def _dot(a, b):
    return jnp.dot(a, b, preferred_element_type=F32)


def _bf(words):
    return pltpu.bitcast(words, BF16)


def _words(x):
    return pltpu.bitcast(x.astype(BF16), U32)


def _recip(x):
    r = pl.reciprocal(x, approx=True)
    return r * (2.0 - x * r)


def _halves(words):
    return (pltpu.bitcast(words << 16, F32),
            pltpu.bitcast(words & np.uint32(0xFFFF0000), F32))


def _pack(lo, hi):
    return pltpu.bitcast(pltpu.pack_elementwise([lo, hi], packed_dtype=BF16), U32)


def _on_words(fn, *blocks):
    parts = [_halves(b) for b in blocks]
    return [_pack(lo, hi) for lo, hi in zip(fn(*[x[0] for x in parts]), fn(*[x[1] for x in parts]))]


def _words_shuffled(x):
    n, c = x.shape
    x = x.reshape(n // 16, 2, 8, c)
    return _pack(x[:, 0], x[:, 1]).reshape(n // 2, c)


def _lhs_sums(a11, a12, a21, a22):
    return a11 + a22, a21 + a22, a11 + a12, a21 - a11, a12 - a22


def _lhs_factors(a11, a22, sums):
    return sums[0], sums[1], a11, a22, sums[2], sums[3], sums[4]


def _rhs_sums(b11, b12, b21, b22):
    return b11 + b22, b12 - b22, b21 - b11, b11 + b12, b21 + b22


def _rhs_factors(b11, b12, b21, b22):
    s = _rhs_sums(b11, b12, b21, b22)
    return s[0], b11, s[1], s[2], b22, s[3], s[4]


def _rhs_factors_of_words(b11, b12, b21, b22):
    s = _on_words(_rhs_sums, b11, b12, b21, b22)
    return s[0], b11, s[1], s[2], b22, s[3], s[4]


def _lhs_factors_of(a11, a12, a21, a22):
    return _lhs_factors(a11, a22, _lhs_sums(a11, a12, a21, a22))


def _two_levels(factors, blocks):
    sides = []
    for side in range(2):
        vals = [[_halves(b)[side] for b in row] for row in blocks]
        inner = [factors(*[vals[2 * r + ri][2 * c + ci] for r in range(2) for c in range(2)])
                 for ri in range(2) for ci in range(2)]
        sides.append([factors(*[x[j] for x in inner]) for j in range(7)])
    return [[_pack(lo, hi) for lo, hi in zip(a, b)] for a, b in zip(*sides)]


def _strassen(mul):
    m3 = mul(2)
    m4 = mul(3)
    m5 = mul(4)
    c12 = m3 + m5
    m2 = mul(1)
    c21 = m2 + m4
    m1 = mul(0)
    c11 = (m4 - m5) + m1 + mul(6)
    c22 = (m3 - m2) + m1 + mul(5)
    return c11, c12, c21, c22


def _tree_sum(xs):
    if not TREE:
        return functools.reduce(jnp.add, xs)
    while len(xs) > 1:
        xs = [a + b for a, b in zip(xs[0::2], xs[1::2])]
    return xs[0]


def _with_vreg(x, r, t, vreg):
    mid = [x[r:r + 8, :t * 128], vreg, x[r:r + 8, (t + 1) * 128:]]
    rows = [x[:r], jnp.concatenate([z for z in mid if z.size], axis=1), x[r + 8:]]
    return jnp.concatenate([z for z in rows if z.size], axis=0)


class _SideWork:
    def __init__(self):
        self.now = 0
        self.starts = {}
        self.stores = {}

    def add(self, tasks, slots, lag):
        for n, task in enumerate(tasks):
            self.starts.setdefault(slots[n * len(slots) // len(tasks)], []).append((task, lag))

    def step(self):
        for task, lag in self.starts.pop(self.now, []):
            for n, batch in enumerate(task()):
                self.stores.setdefault(self.now + lag + n * MB, []).extend(batch)
        for ref, idx, val in self.stores.pop(self.now, []):
            ref[idx] = val
        self.now += 1

    @property
    def done(self):
        return not self.starts and not self.stores


def _permute_head_columns(words):
    rows = words.shape[0]
    tiles = [words[:, t * 128:(t + 1) * 128] for t in range(8)]
    lane = lax.broadcasted_iota(jnp.int32, (rows, 128), 1)
    for bit in (1, 2, 4):
        low = (lane & bit) == 0
        for t in range(8):
            if t & bit:
                continue
            a, b = tiles[t], tiles[t | bit]
            tiles[t] = jnp.where(low, a, pltpu.roll(b, bit, 1))
            tiles[t | bit] = jnp.where(low, pltpu.roll(a, 128 - bit, 1), b)
    src = ((lane & 3) << 5) | (lane >> 2)
    return jnp.concatenate([jnp.take_along_axis(x, src, axis=1) for x in tiles], axis=1)


def _mult(i, n):
    return i * n if isinstance(i, int) else pl.multiple_of(i * n, n)


def _cols(t):
    return slice(t * 128, (t + 1) * 128)


def _kernel(
    xa_hbm, c_hbm, wq_hbm, wk_hbm, wv_hbm, woa_hbm, xb_hbm, wqkv_hbm, wob_hbm,
    out_hbm,
    xa, xa_sum, wide, c, c_sum, kv_f, k_buf, v_buf, ctx,
    wq_raw, wk_raw, wv_raw, woa, wqkv, wob_raw, qb, kb, vb, obuf,
    sem_x, sem_w, sem_misc, sem_out,
):
    xa32, c32, woa32, xb32, wqkv32 = (
        r.bitcast(U32) for r in (xa_hbm, c_hbm, woa_hbm, xb_hbm, wqkv_hbm))
    wq32 = wq_hbm.bitcast(U32)
    wk32 = wk_hbm.bitcast(U32)
    wv32 = wv_hbm.bitcast(U32)
    wob32 = wob_hbm.bitcast(U32)

    def pair_copies(src, dst, pair, sem):
        slot = pair & ((2 if src is wq32 else RING) * PP - 1)
        if src is wob32:
            return [pltpu.make_async_copy(src.at[:, pair, :], dst.at[slot], sem)]
        return [pltpu.make_async_copy(src.at[:, odd, pair, :], dst.at[slot, odd], sem) for odd in range(2)]

    def wq_copies(step):
        return [cp for j in range(PP)
                for cp in pair_copies(wq32, wq_raw, step * PP + j, sem_w.at[step & (RING - 1)])]

    def tail_copies(part):
        sem, slot = sem_w.at[(part + 1) & (RING - 1)], part & (RING - 1)
        c_rows = [(2 * (part >> 1) + h, pl.ds(_mult(part & 1, G // 8), G // 8)) for h in range(2)]
        return [cp for src, dst in ((wk32, wk_raw), (wv32, wv_raw), (wob32, wob_raw)) for j in range(PP)
                for cp in pair_copies(src, dst, part * PP + j, sem)] + [
            *[pltpu.make_async_copy(wqkv32.at[h, pl.ds(_mult(part, PP * 16), PP * 16)], wqkv.at[slot, h, 0:PP * 16], sem)
              for h in range(2)],
            pltpu.make_async_copy(woa32.at[pl.ds(_mult(part, PP * D), PP * D)], woa.at[slot, 0:PP * D], sem),
            *[pltpu.make_async_copy(c32.at[rows], c.at[rows], sem) for rows in c_rows]]

    xn = G // 2 // XSPLIT
    x_copies = [[pltpu.make_async_copy(xa32.at[r:r + xn], xa.at[r:r + xn], sem_x.at[g])
                 for r in range(g * G // 2, (g + 1) * G // 2, xn)] for g in range(NG)]
    first_wq = [pair_copies(wq32, wq_raw, j, sem_misc.at[j]) for j in range(PP)]
    xb = xa
    xb_copy = pltpu.make_async_copy(xb32, xb, sem_misc.at[2])

    gw = G // 4

    def make_sums(raw, sums, g):
        k2 = raw.shape[1] // 2
        blocks = [raw[(2 * g + r) * gw:(2 * g + r + 1) * gw, k * k2:(k + 1) * k2]
                  for r in range(2) for k in range(2)]
        for j, val in enumerate(_on_words(_lhs_sums, *blocks)):
            sums[j, g * gw:(g + 1) * gw, :] = val

    def left_factor(raw, sums, j, g):
        k2 = raw.shape[1] // 2
        if j in (2, 3):
            r = j - 2
            return raw[(2 * g + r) * gw:(2 * g + r + 1) * gw, r * k2:(r + 1) * k2]
        return sums[j if j < 2 else j - 2, g * gw:(g + 1) * gw, :]

    def right_factors(raw, index, top, bottom, n):
        sides = [_rhs_factors(*_halves(raw[index, odd, top // 2:(top + n) // 2, :]),
                              *_halves(raw[index, odd, bottom // 2:(bottom + n) // 2, :]))
                 for odd in range(2)]
        return [_pack(even, odd) for even, odd in zip(*sides)]

    def blocks_of(g, mul):
        for n, val in enumerate(_strassen(mul)):
            r, e = divmod(n, 2)
            yield e, slice((2 * g + r) * gw, (2 * g + r + 1) * gw), val

    def project_kv(n, pair, g):
        def lhs(j):
            if j in (2, 3):
                return c[2 * g + j - 2, :, (j - 2) * DC // 2:(j - 1) * DC // 2]
            return c_sum[j if j < 2 else j - 2, g * gw:(g + 1) * gw, :]

        for e, rows, val in blocks_of(g, lambda j: _dot(_bf(lhs(j)), _bf(kv_f[pair, n, j]))):
            val = _words_shuffled(val)
            (k_buf, v_buf)[n][e, rows, :] = val
            if n == 0 and rows.start == 0:
                ctx[H + e, 0:BQ // 2, :] = val[0:BQ // 2]

    def prepare_kv(n, p, piece):
        vals = right_factors((wk_raw, wv_raw)[n], p & (RING * PP - 1),
                             piece * 32, DC // 2 + piece * 32, 32)
        return [[(kv_f, (p, n, j, slice(piece * 16, (piece + 1) * 16)), val) for j, val in enumerate(vals)]]

    def prepare_c(part, piece):
        r = _mult(part & 1, G // 8) + 16 * piece
        vals = _on_words(_lhs_sums, *[
            c[2 * (part >> 1) + h, pl.ds(r, 16), k * DC // 2:(k + 1) * DC // 2]
            for h in range(2) for k in range(2)])
        return [[(c_sum, (j, pl.ds(_mult(part >> 1, gw) + r, 16)), val) for j, val in enumerate(vals)]]

    def prepare_wqkv(part, piece, which):
        both = _permute_head_columns(jnp.concatenate([
            wqkv[part & (RING - 1), h, 8 * piece:8 * piece + 8, which * M:(which + 1) * M]
            for h in range(2)], axis=0))
        vals = _rhs_factors_of_words(both[:8, :W], both[:8, W:], both[8:, :W], both[8:, W:])
        r = _mult(part, PP * 16) + 8 * piece
        return [[(wide, (QKV0 + 7 * which + j, pl.ds(r, 8)), vals[j]) for j in js]
                for js in ((0, 1, 4), (2, 3), (5, 6))]

    def prepare_wob(p, t):
        b11, b21 = _halves(wob_raw[p & (RING * PP - 1), :, _cols(t)])
        b12, b22 = _halves(wob_raw[p & (RING * PP - 1), :, _cols(4 + t)])
        r = _mult((p & 3) * 4 + (p >> 2), HB // 2)
        vals = _rhs_factors(b11, b12, b21, b22)
        return [[(wide, (OB0 + j, pl.ds(r, HB // 2), _cols(t)), _words(vals[j])) for j in js]
                for js in ((0, 1, 4), (2, 3, 5, 6))]

    def prepare_woa(part, t, n):
        fac = _two_levels(_rhs_factors, [
            [woa[part & (RING - 1), hq * D // 2 + 8 * n:hq * D // 2 + 8 * n + 8, _cols(2 * k + t)]
             for k in range(4)] for hq in range(4)])
        rows = pl.ds(_mult(part & 3, D // 2) + 8 * n, 8)
        cols = pl.ds(_mult(2 * t + (part >> 2), 128), 128)
        return [[(wide, (OA0 + 7 * j + k, rows, cols), fac[j][k]) for j in js for k in range(7)]
                for js in ((1, 4), (0, 5), (2, 3), (6,))]

    def tail_tasks(part):
        P = functools.partial
        tasks = []
        for j in range(PP):
            p = part * PP + j
            for n in range(8):
                tasks.append(P(prepare_kv, 1, p, n))
                tasks.append(P(prepare_woa, part, j, n))
                if n < 6:
                    tasks.append(P(prepare_wqkv, part, 2 * j + n // 3, n % 3))
                tasks.append(P(prepare_kv, 0, p, n))
                if n % 2:
                    tasks.append(P(prepare_wob, p, n // 2))
                elif n % 4 == 0:
                    tasks.append(P(prepare_c, part, 2 * j + n // 4))
        return tasks

    def gate(g, j, n):
        r = 8 * (7 * g + j)
        return GATE, slice(r, r + 8), _cols(n)

    def project_q(pair, g, fac, side=None, zero=None, tokens=None):
        def mul(j):
            lhs = left_factor(xa, xa_sum, j, g)
            if side is None:
                return _dot(_bf(lhs), fac(j))
            for n in range(SUB0):
                side.step()
                lhs = _with_vreg(lhs, n * gw // SUB0, 0, wide[gate(g, j, n)])
                if tokens:
                    token = tokens.pop(0)
                    wqkv[zero, 0, PP * 16:PP * 16 + 8, _cols(0)] = token
                    if WT and isinstance(pair, int):
                        woa[zero, PP * D:PP * D + 8, _cols(0)] = token
                    wk_raw[RING * PP + zero, 0, 0:8] = token
                    wv_raw[RING * PP + zero, 0, 0:8] = token
                    c[2 * NG + zero, 0:8, _cols(0)] = token
            val = _dot(_bf(lhs), fac(j))
            tokens.extend(pltpu.bitcast(val[r:r + 8], U32) for r in range(0, 2 * gw, 2 * gw // SUB0))
            return val

        for e, rows, val in blocks_of(g, mul):
            ctx[2 * pair + e, rows, :] = _words(val * (D ** -0.5 * LOG2E))

    def start(copies):
        for cp in copies:
            cp.start()

    def wait(copies):
        for cp in copies:
            cp.wait()

    scope = []
    with jax.named_scope("peel"):
        for op in SCHED00.split(","):
            kind, arg = op[0], op[1:]
            if kind == "I":
                for j, val in enumerate(right_factors(wq_raw, int(arg), 0, M // 2, M // 2)):
                    kv_f[NP - 1 - int(arg), :, j] = val.reshape(2, DC // 4, D)
            elif kind == "q":
                project_q(int(arg[0]), int(arg[1]), lambda j: _bf(kv_f[NP - 1 - int(arg[0]), :, j].reshape(M // 4, D)))
            elif kind == "Q":
                fac = right_factors(wq_raw, int(arg[0]), 0, M // 2, M // 2)
                for j, val in enumerate(fac):
                    kv_f[NP - 1 - int(arg[0]), :, j] = val.reshape(2, DC // 4, D)
                project_q(int(arg[0]), int(arg[1]), lambda j: _bf(fac[j]))
            elif kind == "X":
                start(x_copies[int(arg)])
            elif kind == "x":
                wait(x_copies[int(arg)])
            elif kind == "y":
                make_sums(xa, xa_sum, int(arg))
                for j in range(7):
                    for n in range(SUB0):
                        r = n * gw // SUB0
                        wide[gate(int(arg), j, n)] = left_factor(xa, xa_sum, j, int(arg))[r:r + 8, 0:128]
            elif kind == "F":
                start(first_wq[int(arg)])
            elif kind == "f":
                wait(first_wq[int(arg)])
            elif kind == "T":
                start(tail_copies(int(arg)))
            elif kind == "U":
                start(wq_copies(int(arg)))
            elif kind == "|":
                if scope:
                    scope.pop().__exit__(None, None, None)
                if arg:
                    scope.append(jax.named_scope(arg))
                    scope[-1].__enter__()
            elif kind == "Z":
                kb[:, RC:RC + HALO, :] = jnp.zeros((8, HALO, 128), F32)
                vb[:, RC:RC + HALO, :] = jnp.zeros((8, HALO, 128), F32)
            else:
                raise ValueError(op)

    def q_step(step, parts, zero, skip, lag):
        side, tokens = _SideWork(), []
        side.add([task for part in parts for task in tail_tasks(part)], [n for n in range(7 * NG * PP - lag - 3) if n % (7 * NG) >= skip], lag)
        for p in (step * PP + j for j in range(PP)):
            fac = [_bf(val) for val in right_factors(wq_raw, p & (2 * PP - 1), 0, M // 2, M // 2)]
            for g in range(NG):
                project_q(p, g, fac.__getitem__, side, zero, tokens)
        assert side.done

    def q_body(step, zero):
        start(wq_copies(step + 1) + tail_copies(step + 1))
        wait(wq_copies(step) + tail_copies(step - 1))
        q_step(step, [step - 1], zero, SKIP0, LAG0)
        return -zero

    with jax.named_scope("phase0"):
        zero = lax.fori_loop(1, NS - 1, q_body, 0)

    with jax.named_scope("bridge"):
        wait(wq_copies(NS - 1) + tail_copies(NS - 2) + tail_copies(NS - 1))
        q_step(NS - 1, [zero + NS - 2, zero + NS - 1], zero, SKIP1, LAG1)
        project_kv(0, 0, 0)
        xb_copy.start()

    def pair_body(p, kslot):
        nxt = jnp.minimum(p + 1, NP - 1)
        row = lax.broadcasted_iota(jnp.int32, (BQ, BQ), 0)
        col = lax.broadcasted_iota(jnp.int32, (BQ, BQ), 1)
        causal = ((col & ~15) | ((col & 15) >> 1) | ((col & 1) << 3)) <= row
        hb = BQ // 2

        def scores(e, i):
            r = i * BQ
            k = ctx[kslot + e, 0:hb, :]
            k = _bf(jnp.concatenate([k, k_buf[e, hb:(i + 1) * hb, :]], axis=0) if i else k)
            q = _bf(ctx[2 * p + e, i * hb:(i + 1) * hb, :])
            s = lax.dot_general(q, k, _NT, preferred_element_type=F32)
            diag = jnp.where(causal, s[:, r:], NEG)
            s = jnp.concatenate([s[:, :r], diag], axis=1) if r else diag
            return s, jnp.max(s, axis=1, keepdims=True)

        def weighted(e, i, s, m, rounded):
            w = jnp.exp2(s - m)
            wb = w.astype(BF16)
            l = jnp.sum(wb.astype(F32) if rounded else w, axis=1, keepdims=True)
            o = _dot(wb, _bf(v_buf[e, 0:(i + 1) * hb, :]))
            return _words(o * _recip(l))

        state = {}
        for op in SCHED.split(","):
            kind, arg = op[0], op[1:]
            if kind in "kv":
                project_kv("kv".index(kind), nxt if op == "k0" else p, int(arg))
            else:
                e, i = "ab".index(arg[0]), int(arg[1:])
                if kind == "S":
                    state[e, i] = scores(e, i)
                elif kind in "PR":
                    state[e, i] = weighted(e, i, *state[e, i], kind == "R")
                else:
                    ctx[2 * p + e, i * hb:(i + 1) * hb, :] = state.pop((e, i))
        assert not state
        return 2 * H - kslot

    with jax.named_scope("phase1"):
        lax.fori_loop(0, NP, pair_body, H)

    xb_copy.wait()

    n_chunks = S // RC
    hr = RC // 2

    def out_copy(i, slot):
        return pltpu.make_async_copy(
            obuf.at[slot], out_hbm.at[pl.ds(_mult(i, RC), RC), :], sem_out.at[slot])

    def chunk_body(i, zero):
        slot = i & 1

        @pl.when(i >= 2)
        def _():
            out_copy(i, slot).wait()

        def half_rows(r, lo=0, n=hr // 2):
            return pl.ds(_mult(i, hr) + r * (hr // 2) + lo, n)

        qr = RC // 8

        def ctx_at(j, k, u, lo, n):
            if j in (2, 3) and k in (2, 3):
                quarter = 2 * (j - 2) + k - 2
                return ctx, (4 * u + quarter, pl.ds(_mult(i, hr) + quarter * qr + lo, n))
            slab, r = divmod((2 * (7 * j + k) + u // 4) * qr + lo, SLAB)
            return wide, (CS0 + slab, slice(r, r + n), _cols(u % 4))

        sums = {}

        def ctx_sums(u, lo, js):
            if (u, lo) not in sums:
                sums[u, lo] = _two_levels(_lhs_factors_of, [
                    [ctx[4 * u + hq, pl.ds(_mult(i, hr) + r * qr + lo, 8)] for hq in range(4)]
                    for r in range(4)])
            return [[ctx_at(j, k, u, lo, 8) + (sums[u, lo][j][k],) for j in js for k in range(7)
                     if not (j in (2, 3) and k in (2, 3))]]

        def taps(buf, t, w, r):
            back, shift = divmod(DIL * w, 8)
            lo = HALO + r - 8 * back
            if shift == 0:
                return buf[t, lo:lo + 8, :]
            if (ROT & 1 and buf is kb) or (ROT & 2 and buf is vb):
                sub = lax.broadcasted_iota(jnp.int32, (8, 128), 0)
                mixed = jnp.where(sub < 8 - shift, buf[t, lo:lo + 8, :], buf[t, lo - 8:lo, :])
                return pltpu.roll(mixed, shift, 0)
            return buf[t, lo - shift:lo - shift + 8, :]

        def weight_at(r, w):
            return PR0 + w // 4, slice(r, r + 8), _cols(w % 4)

        def window_logits(r, ws):
            q = [qb[t + zero, HALO + r:HALO + r + 8, :] for t in range(8)]
            logits = [functools.reduce(jnp.add, [q[t] * taps(kb, t, w, r) for t in range(8)])
                      for w in ws]
            logits = [z + pltpu.roll(z, 64, 1) for z in logits]
            logits = [(z + pltpu.roll(z, 32, 1)) * (DB ** -0.5 * LOG2E) for z in logits]
            pos = i * RC + r + lax.broadcasted_iota(jnp.int32, (8, 128), 0)
            return [[(wide, weight_at(r, w),
                      pltpu.bitcast(jnp.where(pos >= DIL * w, z, NEG) if DIL * w > r else z, U32))
                     for w, z in zip(ws, logits)]]

        weights = {}

        def window_softmax(r):
            logits = [pltpu.bitcast(wide[weight_at(r, w)], F32) for w in range(WIN)]
            peak = functools.reduce(jnp.maximum, logits)
            probs = [jnp.exp2(z - peak) for z in logits]
            inv = _recip(functools.reduce(jnp.add, probs))
            weights[r] = [z * inv for z in probs]
            return []

        def window_values(r, ts):
            probs = weights[r]
            r1 = r % hr
            return [[(wide, (LOC0 + r // hr, slice(r1 + (t % 2) * hr, r1 + (t % 2) * hr + 8), _cols(t // 2)),
                     pltpu.bitcast(_tree_sum([probs[w] * taps(vb, t, w, r) for w in range(WIN)]), U32))
                     for t in ts]]

        side = _SideWork()
        P = functools.partial
        side.add([P(ctx_sums, u, lo, js) for u in range(8) for lo in range(0, qr, 8)
                  for js in JS], range(E1, E4), 0)
        side.add([P(window_logits, r, ws) for r in range(0, RC, 8)
                  for ws in ((0, 4, 1, 5), (2, 6, 3, 7))], range(E2, E3 - LAG2), LAG2)
        side.add([P(window_softmax, r) for r in range(0, RC, 8)], range(E3, 181), 0)
        side.add([P(window_values, r, ts) for r in range(0, RC, 8)
                  for ts in (range(4), range(4, 8))], range(E3 + 1, 182), 0)

        wide_alias = wide.at[pl.ds(zero, PR0)]

        def mul(lhs, slab, *tiles):
            side.step()
            rhs = jnp.concatenate([wide[slab, :, _cols(t)] for t in tiles], axis=0)
            rhs = _with_vreg(rhs, 0, 0, wide_alias[slab, 0:8, _cols(tiles[0])])
            val = _dot(_bf(lhs), _bf(rhs))
            qb[0, 0:8, :] = val[0:8]
            return val

        x = [xb[half_rows(r), k * W:(k + 1) * W] for r in range(2) for k in range(2)]
        x_fac = _lhs_factors(x[0], x[3], _on_words(_lhs_sums, *x))
        for part, buf in ((1, kb), (0, qb), (2, vb)):
            if part:
                buf[:, 0:HALO, :] = buf[:, RC:RC + HALO, :]
            for t in range(4):
                blocks = _strassen(lambda j: mul(x_fac[j], QKV0 + 7 * part + j, t))
                for n, val in enumerate(blocks):
                    r, k = divmod(n, 2)
                    buf[4 * k + t, HALO + r * hr:HALO + (r + 1) * hr, :] = val

        def ctx_factor(j, k):
            return jnp.concatenate(
                [ref[idx] for ref, idx in (ctx_at(j, k, u, 0, qr) for u in range(8))], axis=1)

        def store_out(col0, t, blocks):
            for n, val in enumerate(blocks):
                r, k = divmod(n, 2)
                lo = col0 + k * W + t * 128
                obuf[slot, r * hr:(r + 1) * hr, lo:lo + 128] = val.astype(BF16)

        for t in range(2):
            blocks = _strassen(lambda j: jnp.concatenate(_strassen(
                lambda k: mul(ctx_factor(j, k), OA0 + 7 * j + k, 2 * t, 2 * t + 1)), axis=0))
            for outer, val in enumerate(blocks):
                for inner in range(4):
                    r = 2 * (outer // 2) + inner // 2
                    k = 2 * (outer % 2) + inner % 2
                    obuf[slot, r * 2 * qr:(r + 1) * 2 * qr, _cols(2 * k + t)] = (
                        val[inner * 2 * qr:(inner + 1) * 2 * qr].astype(BF16))
        assert side.done

        o = [pltpu.bitcast(wide[LOC0 + n // 2, (n % 2) * hr:(n % 2 + 1) * hr, :], F32) for n in range(4)]
        o_fac = [z.astype(BF16) for z in _lhs_factors(o[0], o[3], _lhs_sums(*o))]
        for t in range(4):
            store_out(M, t, _strassen(lambda j: _dot(
                o_fac[j], _bf(wide[OB0 + j, :, _cols(t)]))))

        out_copy(i, slot).start()
        return -zero

    with jax.named_scope("phase2"):
        lax.fori_loop(0, n_chunks, chunk_body, 0)
    with jax.named_scope("tail"):
        out_copy(n_chunks - 2, 0).wait()
        out_copy(n_chunks - 1, 1).wait()


@jax.jit
def pallas_concat_heads__compressed_kv_cla__sliding_local_dilated__prompt_kernel(
    A_x, A_c_kv, A_w_q, A_w_uk, A_w_uv, A_w_o, B_x, B_wqkv, B_wo,
):
    scratch = [
        pltpu.VMEM((S // 2, M), U32),
        pltpu.VMEM((5, S // 4, M // 2), U32),
        pltpu.VMEM((N_SLABS, SLAB, W), U32),
        pltpu.VMEM((2 * NG + 1, G // 4, DC), U32),
        pltpu.VMEM((5, S // 4, DC // 2), U32),
        pltpu.VMEM((NP, 2, 7, DC // 4, D), U32),
        pltpu.VMEM((2, S // 2, D), U32),
        pltpu.VMEM((2, S // 2, D), U32),
        pltpu.VMEM((H + 2, S // 2, D), U32),
        pltpu.VMEM((2 * PP, 2, M // 2, D), U32),
        pltpu.VMEM((RING * PP + 1, 2, DC // 2, D), U32),
        pltpu.VMEM((RING * PP + 1, 2, DC // 2, D), U32),
        pltpu.VMEM((RING, PP * D + 8, M), U32),
        pltpu.VMEM((RING, 2, PP * 16 + 8, 3 * M), U32),
        pltpu.VMEM((RING * PP, HB, M), U32),
        pltpu.VMEM((8, HALO + RC + PAD, 128), F32),
        pltpu.VMEM((8, HALO + RC + PAD, 128), F32),
        pltpu.VMEM((8, HALO + RC + PAD, 128), F32),
        pltpu.VMEM((2, RC, 2 * M), BF16),
        pltpu.SemaphoreType.DMA((NG,)),
        pltpu.SemaphoreType.DMA((RING,)),
        pltpu.SemaphoreType.DMA((3,)),
        pltpu.SemaphoreType.DMA((2,)),
    ]
    out = pl.pallas_call(
        _kernel,
        out_shape=jax.ShapeDtypeStruct((S, 2 * M), BF16),
        in_specs=[pl.BlockSpec(memory_space=pl.ANY)] * 9,
        out_specs=pl.BlockSpec(memory_space=pl.ANY),
        scratch_shapes=scratch,
        compiler_params=pltpu.CompilerParams(vmem_limit_bytes=127 * 2**20, disable_bounds_checks=True),
        name="fused_mla_sliding",
    )(
        A_x.reshape(S, M),
        A_c_kv.reshape(2 * NG, G // 2, DC),
        A_w_q.reshape(M // 2, 2, H, D),
        A_w_uk.reshape(DC // 2, 2, H, D),
        A_w_uv.reshape(DC // 2, 2, H, D),
        A_w_o.reshape(H * D, M),
        B_x.reshape(S, M),
        B_wqkv.reshape(2, M // 2, 3 * M),
        B_wo.reshape(HB, DB, M),
    )
    return out.reshape(1, S, 2 * M)
```

```python
import functools

import jax
import jax.numpy as jnp
import numpy as np
from jax import lax
import jax.experimental.pallas as pl
import jax.experimental.pallas.tpu as pltpu

S = 2048
M = 1024
DC = 512
H = 32
D = 128
HB = 32
DB = 32
WIN = 8
DIL = 2

NP = H // 2
PP = 2
NS = NP // PP
RING = 4
G = 512
NG = S // G
BQ = 128
RC = 256
HALO = 16
LOG2E = 1.4426950408889634
NEG = -1e9 * LOG2E

W = M // 2
SLAB = M // 4
OA0 = 0
QKV0 = OA0 + 49
OB0 = QKV0 + 21
CS0 = OB0 + 7
PR0 = CS0 + 13
LOC0 = PR0 + 2
GATE = LOC0 + 2
N_SLABS = GATE + 1

SKIP0 = 4
LAG0 = 3
SKIP1 = 0
LAG1 = 3
CTX_FIRST = 6
CTX_LAST = 70
LOGIT_FIRST = 62
LOGIT_LAG = 6
VALUE_FIRST = 124

F32 = jnp.float32
BF16 = jnp.bfloat16
U32 = jnp.uint32
_NT = (((1,), (1,)), ((), ()))


def _attention_order():
    ops = ("Sa0 Sa1 Sa2 Sa3 v0 k1 Pa0 Pa1 Pa2 v1 Sa4 Pa3 k2 Sa5 Wa0 Wa1 Pa4 v2 "
           "Sa6 Wa2 Pa5 Wa3 k3 Sa7 Pa6 Wa4 v3").split()
    for i in range(8, 16):
        ops += [f"Sa{i}", f"Pa{i - 1}", f"Wa{i - 3}"]
    ops += "Sb15 Pa15 Wa13 Sb14 Pb15 Wa14 Sb13 Pb14 Wa15".split()
    for i in range(12, 3, -1):
        ops += [f"Sb{i}", f"Pb{i + 1}", f"Wb{i + 3}"]
    return ops + "Sb3 Sb2 Pb4 Wb6 Sb1 Sb0 Pb3 Pb2 k0 Pb1 Pb0 Wb5 Wb4 Wb3 Wb2 Wb1 Wb0".split()


def _dot(a, b):
    return jnp.dot(a, b, preferred_element_type=F32)


def _bf(words):
    return pltpu.bitcast(words, BF16)


def _words(x):
    return pltpu.bitcast(x.astype(BF16), U32)


def _halves(words):
    return (pltpu.bitcast(words << 16, F32),
            pltpu.bitcast(words & np.uint32(0xFFFF0000), F32))


def _pack(lo, hi):
    return pltpu.bitcast(pltpu.pack_elementwise([lo, hi], packed_dtype=BF16), U32)


def _words_shuffled(x):
    n, c = x.shape
    x = x.reshape(n // 16, 2, 8, c)
    return _pack(x[:, 0], x[:, 1]).reshape(n // 2, c)


def _recip(x):
    r = pl.reciprocal(x, approx=True)
    return r * (2.0 - x * r)


def _lhs_factors(a11, a12, a21, a22):
    return a11 + a22, a21 + a22, a11, a22, a11 + a12, a21 - a11, a12 - a22


def _rhs_factors(b11, b12, b21, b22):
    return b11 + b22, b11, b12 - b22, b21 - b11, b22, b11 + b12, b21 + b22


def _strassen(mul):
    m3 = mul(2)
    m4 = mul(3)
    m5 = mul(4)
    c12 = m3 + m5
    m2 = mul(1)
    c21 = m2 + m4
    m1 = mul(0)
    c11 = (m4 - m5) + m1 + mul(6)
    c22 = (m3 - m2) + m1 + mul(5)
    return c11, c12, c21, c22


def _factors_of_words(factors, *blocks):
    parts = [_halves(b) for b in blocks]
    plain = {id(lo): b for (lo, _), b in zip(parts, blocks)}
    return [plain.get(id(lo)) if id(lo) in plain else _pack(lo, hi)
            for lo, hi in zip(factors(*[x[0] for x in parts]), factors(*[x[1] for x in parts]))]


def _nested_factors_of_words(factors, blocks):
    sides = []
    for side in range(2):
        vals = [[_halves(b)[side] for b in row] for row in blocks]
        inner = [factors(*[vals[2 * r + ri][2 * c + ci] for r in range(2) for c in range(2)])
                 for ri in range(2) for ci in range(2)]
        sides.append([factors(*[x[j] for x in inner]) for j in range(7)])
    return [[_pack(lo, hi) for lo, hi in zip(a, b)] for a, b in zip(*sides)]


def _permute_head_columns(words):
    tiles = [words[:, _cols(t)] for t in range(8)]
    lane = lax.broadcasted_iota(jnp.int32, tiles[0].shape, 1)
    for bit in (1, 2, 4):
        low = (lane & bit) == 0
        for t in range(8):
            if t & bit:
                continue
            a, b = tiles[t], tiles[t | bit]
            tiles[t] = jnp.where(low, a, pltpu.roll(b, bit, 1))
            tiles[t | bit] = jnp.where(low, pltpu.roll(a, 128 - bit, 1), b)
    src = ((lane & 3) << 5) | (lane >> 2)
    return jnp.concatenate([jnp.take_along_axis(x, src, axis=1) for x in tiles], axis=1)


def _with_corner(x, corner):
    top = corner if x.shape[1] == 128 else jnp.concatenate([corner, x[0:8, 128:]], axis=1)
    return jnp.concatenate([top, x[8:]], axis=0)


class _SideWork:
    def __init__(self):
        self.now = 0
        self.starts = {}
        self.stores = {}

    def add(self, tasks, steps, lag):
        for n, task in enumerate(tasks):
            self.starts.setdefault(steps[n * len(steps) // len(tasks)], []).append((task, lag))

    def step(self):
        for task, lag in self.starts.pop(self.now, []):
            self.stores.setdefault(self.now + lag, []).extend(task())
        for ref, idx, val in self.stores.pop(self.now, []):
            ref[idx] = val
        self.now += 1

    def check_done(self):
        assert not self.starts and not self.stores


def _mult(i, n):
    return i * n if isinstance(i, int) else pl.multiple_of(i * n, n)


def _cols(t):
    return slice(t * 128, (t + 1) * 128)


def _start(copies):
    for cp in copies:
        cp.start()


def _wait(copies):
    for cp in copies:
        cp.wait()


def _kernel(
    xa_hbm, c_hbm, wq_hbm, wk_hbm, wv_hbm, woa_hbm, xb_hbm, wqkv_hbm, wob_hbm,
    out_hbm,
    x, x_sum, wide, c, c_sum, kv_fac, k_buf, v_buf, ctx,
    wq_raw, wk_raw, wv_raw, woa_raw, wqkv_raw, wob_raw, qb, kb, vb, obuf,
    sem_x, sem_w, sem_misc, sem_out,
):
    P = functools.partial
    xa32, c32, woa32, xb32, wqkv32 = (
        r.bitcast(U32) for r in (xa_hbm, c_hbm, woa_hbm, xb_hbm, wqkv_hbm))
    wq32, wk32, wv32, wob32 = (r.bitcast(U32) for r in (wq_hbm, wk_hbm, wv_hbm, wob_hbm))

    def pair_copies(src, dst, pair, ring, sem):
        slot = pair & (ring * PP - 1)
        return [pltpu.make_async_copy(src.at[:, odd, pair, :], dst.at[slot, odd], sem)
                for odd in range(2)]

    def wq_copies(step):
        sem = sem_w.at[step & (RING - 1)]
        return [cp for j in range(PP) for cp in pair_copies(wq32, wq_raw, step * PP + j, 2, sem)]

    def later_copies(part):
        sem, slot = sem_w.at[(part + 1) & (RING - 1)], part & (RING - 1)
        copies = []
        for j in range(PP):
            pair = part * PP + j
            copies += pair_copies(wk32, wk_raw, pair, RING, sem)
            copies += pair_copies(wv32, wv_raw, pair, RING, sem)
            copies.append(pltpu.make_async_copy(
                wob32.at[:, pair, :], wob_raw.at[pair & (RING * PP - 1)], sem))
        copies.append(pltpu.make_async_copy(
            woa32.at[pl.ds(_mult(part, PP * D), PP * D)], woa_raw.at[slot, 0:PP * D], sem))
        for h in range(2):
            copies.append(pltpu.make_async_copy(
                wqkv32.at[h, pl.ds(_mult(part, PP * 16), PP * 16)],
                wqkv_raw.at[slot, h, 0:PP * 16], sem))
            rows = (2 * (part >> 1) + h, pl.ds(_mult(part & 1, G // 8), G // 8))
            copies.append(pltpu.make_async_copy(c32.at[rows], c.at[rows], sem))
        return copies

    x_copies = [pltpu.make_async_copy(xa32.at[g * G // 2:(g + 1) * G // 2],
                                      x.at[g * G // 2:(g + 1) * G // 2], sem_x.at[g])
                for g in range(NG)]
    first_wq = [pair_copies(wq32, wq_raw, j, 2, sem_misc.at[j]) for j in range(PP)]
    xb_copy = pltpu.make_async_copy(xb32, x, sem_misc.at[PP])

    gw = G // 4
    sum_index = {0: 0, 1: 1, 4: 2, 5: 3, 6: 4}

    def head_factors(raw, slot, top, bottom, n):
        sides = [_rhs_factors(*_halves(raw[slot, odd, top:top + n, :]),
                              *_halves(raw[slot, odd, bottom:bottom + n, :]))
                 for odd in range(2)]
        return [_pack(even, odd) for even, odd in zip(*sides)]

    def group_blocks(g, mul):
        for n, val in enumerate(_strassen(mul)):
            r, e = divmod(n, 2)
            yield e, slice((2 * g + r) * gw, (2 * g + r + 1) * gw), val

    def project_kv(n, pair, g):
        def lhs(j):
            if j in sum_index:
                return c_sum[sum_index[j], g * gw:(g + 1) * gw, :]
            return c[2 * g + j - 2, :, (j - 2) * DC // 2:(j - 1) * DC // 2]

        for e, rows, val in group_blocks(g, lambda j: _dot(_bf(lhs(j)), _bf(kv_fac[pair, n, j]))):
            val = _words_shuffled(val)
            (k_buf, v_buf)[n][e, rows, :] = val
            if n == 0 and rows.start == 0:
                ctx[H + e, 0:BQ // 2, :] = val[0:BQ // 2]

    def prepare_kv(n, pair, piece):
        vals = head_factors((wk_raw, wv_raw)[n], pair & (RING * PP - 1),
                            piece * 16, DC // 4 + piece * 16, 16)
        return [(kv_fac, (pair, n, j, slice(piece * 16, (piece + 1) * 16)), val)
                for j, val in enumerate(vals)]

    def prepare_c(part, piece):
        r = _mult(part & 1, G // 8) + 16 * piece
        vals = _factors_of_words(_lhs_factors, *[
            c[2 * (part >> 1) + h, pl.ds(r, 16), k * DC // 2:(k + 1) * DC // 2]
            for h in range(2) for k in range(2)])
        return [(c_sum, (n, pl.ds(_mult(part >> 1, gw) + r, 16)), vals[j])
                for j, n in sum_index.items()]

    def prepare_wqkv(part, piece, which):
        both = _permute_head_columns(jnp.concatenate([
            wqkv_raw[part & (RING - 1), h, 8 * piece:8 * piece + 8, which * M:(which + 1) * M]
            for h in range(2)], axis=0))
        vals = _factors_of_words(
            _rhs_factors, both[:8, :W], both[:8, W:], both[8:, :W], both[8:, W:])
        r = _mult(part, PP * 16) + 8 * piece
        return [(wide, (QKV0 + 7 * which + j, pl.ds(r, 8)), val) for j, val in enumerate(vals)]

    def prepare_wob(pair, t):
        b11, b21 = _halves(wob_raw[pair & (RING * PP - 1), :, _cols(t)])
        b12, b22 = _halves(wob_raw[pair & (RING * PP - 1), :, _cols(4 + t)])
        r = _mult((pair & 3) * 4 + (pair >> 2), HB // 2)
        return [(wide, (OB0 + j, pl.ds(r, HB // 2), _cols(t)), _words(val))
                for j, val in enumerate(_rhs_factors(b11, b12, b21, b22))]

    def prepare_woa(part, t, n):
        fac = _nested_factors_of_words(_rhs_factors, [
            [woa_raw[part & (RING - 1), hq * D // 2 + 8 * n:hq * D // 2 + 8 * n + 8, _cols(2 * k + t)]
             for k in range(4)] for hq in range(4)])
        rows = pl.ds(_mult(part & 3, D // 2) + 8 * n, 8)
        cols = pl.ds(_mult(2 * t + (part >> 2), 128), 128)
        return [(wide, (OA0 + 7 * j + k, rows, cols), fac[j][k]) for j in range(7) for k in range(7)]

    def later_tasks(part):
        tasks = []
        for j in range(PP):
            pair = part * PP + j
            for n in range(8):
                tasks += [P(prepare_kv, 1, pair, n), P(prepare_woa, part, j, n)]
                if n < 6:
                    tasks.append(P(prepare_wqkv, part, 2 * j + n // 3, n % 3))
                tasks.append(P(prepare_kv, 0, pair, n))
                if n % 2:
                    tasks.append(P(prepare_wob, pair, n // 2))
                elif n % 4 == 0:
                    tasks.append(P(prepare_c, part, 2 * j + n // 4))
        return tasks

    def x_factor(j, g):
        if j in sum_index:
            return x_sum[sum_index[j], g * gw:(g + 1) * gw, :]
        return x[(2 * g + j - 2) * gw:(2 * g + j - 1) * gw, (j - 2) * W:(j - 1) * W]

    def gate(g, j):
        return GATE, slice(8 * (7 * g + j), 8 * (7 * g + j + 1)), _cols(0)

    def make_x_factors(g):
        vals = _factors_of_words(_lhs_factors, *[
            x[(2 * g + r) * gw:(2 * g + r + 1) * gw, k * W:(k + 1) * W]
            for r in range(2) for k in range(2)])
        for j, n in sum_index.items():
            x_sum[n, g * gw:(g + 1) * gw, :] = vals[j]
        for j in range(7):
            wide[gate(g, j)] = vals[j][0:8, 0:128]

    def project_q(pair, g, mul):
        for e, rows, val in group_blocks(g, mul):
            ctx[2 * pair + e, rows, :] = _words(val * (D ** -0.5 * LOG2E))

    def wq_factors(pair):
        return head_factors(wq_raw, pair & (2 * PP - 1), 0, M // 4, M // 4)

    _start(first_wq[0] + x_copies[:2] + first_wq[1] + x_copies[2:]
           + wq_copies(1) + later_copies(0) + later_copies(1))
    kb[:, RC:RC + HALO, :] = jnp.zeros((8, HALO, 128), F32)
    vb[:, RC:RC + HALO, :] = jnp.zeros((8, HALO, 128), F32)

    def keep_wq_factors(pair):
        fac = wq_factors(pair)
        for j, val in enumerate(fac):
            kv_fac[NP - 1 - pair, :, j] = val.reshape(2, DC // 4, D)
        return fac

    def first_q(pair, g, fac=None):
        project_q(pair, g, lambda j: _dot(_bf(x_factor(j, g)), _bf(
            fac[j] if fac else kv_fac[NP - 1 - pair, :, j].reshape(M // 4, D))))

    _wait(first_wq[0])
    keep_wq_factors(0)
    for g in range(2):
        x_copies[g].wait()
        make_x_factors(g)
        first_q(0, g)
    _wait(first_wq[1])
    first_q(1, 0, keep_wq_factors(1))
    first_q(1, 1)
    _wait(x_copies[2:])
    for g in range(2, NG):
        make_x_factors(g)
        first_q(0, g)
        first_q(1, g)

    def q_step(step, parts, zero, skip, lag):
        side = _SideWork()
        side.add([task for part in parts for task in later_tasks(part)],
                 [n for n in range(7 * NG * PP - lag - 3) if n % (7 * NG) >= skip], lag)

        def mul(fac, g, j):
            side.step()
            val = _dot(_bf(_with_corner(x_factor(j, g), wide[gate(g, j)])), _bf(fac[j]))
            token = pltpu.bitcast(val[0:8], U32)
            wqkv_raw[zero, 0, PP * 16:PP * 16 + 8, _cols(0)] = token
            wk_raw[RING * PP + zero, 0, 0:8] = token
            wv_raw[RING * PP + zero, 0, 0:8] = token
            c[2 * NG + zero, 0:8, _cols(0)] = token
            if len(parts) > 1:
                woa_raw[zero, PP * D:PP * D + 8, _cols(0)] = token
            return val

        for pair in (step * PP + j for j in range(PP)):
            fac = wq_factors(pair)
            for g in range(NG):
                project_q(pair, g, P(mul, fac, g))
        side.check_done()

    def q_body(step, zero):
        _start(wq_copies(step + 1) + later_copies(step + 1))
        _wait(wq_copies(step) + later_copies(step - 1))
        q_step(step, [step - 1], zero, SKIP0, LAG0)
        return -zero

    zero = lax.fori_loop(1, NS - 1, q_body, 0)
    _wait(wq_copies(NS - 1) + later_copies(NS - 2) + later_copies(NS - 1))
    q_step(NS - 1, [zero + NS - 2, zero + NS - 1], zero, SKIP1, LAG1)
    project_kv(0, 0, 0)
    xb_copy.start()

    def pair_body(p, zero):
        row = lax.broadcasted_iota(jnp.int32, (BQ, BQ), 0)
        col = lax.broadcasted_iota(jnp.int32, (BQ, BQ), 1)
        causal = ((col & ~15) | ((col & 15) >> 1) | ((col & 1) << 3)) <= row
        hb = BQ // 2

        def scores(e, i):
            r = i * BQ
            k = ctx[H + e + zero, 0:hb, :]
            k = _bf(jnp.concatenate([k, k_buf[e, hb:(i + 1) * hb, :]], axis=0) if i else k)
            q = _bf(ctx[2 * p + e, i * hb:(i + 1) * hb, :])
            s = lax.dot_general(q, k, _NT, preferred_element_type=F32)
            diag = jnp.where(causal, s[:, r:], NEG)
            s = jnp.concatenate([s[:, :r], diag], axis=1) if r else diag
            return s, jnp.max(s, axis=1, keepdims=True)

        def context(e, i, s, peak):
            w = jnp.exp2(s - peak)
            total = jnp.sum(w, axis=1, keepdims=True)
            o = _dot(w.astype(BF16), _bf(v_buf[e, 0:(i + 1) * hb, :]))
            return _words(o * _recip(total))

        state = {}
        for op in _attention_order():
            if op[0] in "kv":
                pair = jnp.minimum(p + 1, NP - 1) if op == "k0" else p
                project_kv("kv".index(op[0]), pair, int(op[1:]))
                continue
            e, i = "ab".index(op[1]), int(op[2:])
            if op[0] == "S":
                state[e, i] = scores(e, i)
            elif op[0] == "P":
                state[e, i] = context(e, i, *state[e, i])
            else:
                ctx[2 * p + e, i * hb:(i + 1) * hb, :] = state.pop((e, i))
        assert not state
        return -zero

    lax.fori_loop(0, NP, pair_body, 0)
    xb_copy.wait()

    n_chunks = S // RC
    hr = RC // 2
    qw = RC // 8

    def out_copy(i, slot):
        return pltpu.make_async_copy(
            obuf.at[slot], out_hbm.at[pl.ds(_mult(i, RC), RC), :], sem_out.at[slot])

    def chunk_body(i, zero):
        slot = i & 1
        base = _mult(i, RC // 2)

        @pl.when(i >= 2)
        def _():
            out_copy(i, slot).wait()

        def is_plain(j, k):
            return j in (2, 3) and k in (2, 3)

        def ctx_at(j, k, u, lo, n):
            if is_plain(j, k):
                quarter = 2 * (j - 2) + k - 2
                return ctx, (4 * u + quarter, pl.ds(base + quarter * qw + lo, n))
            slab, r = divmod((2 * (7 * j + k) + u // 4) * qw + lo, SLAB)
            return wide, (CS0 + slab, slice(r, r + n), _cols(u % 4))

        ctx_fac = {}

        def ctx_factors(u, lo, js):
            if (u, lo) not in ctx_fac:
                ctx_fac[u, lo] = _nested_factors_of_words(_lhs_factors, [
                    [ctx[4 * u + hq, pl.ds(base + r * qw + lo, 8)] for hq in range(4)]
                    for r in range(4)])
            return [ctx_at(j, k, u, lo, 8) + (ctx_fac[u, lo][j][k],)
                    for j in js for k in range(7) if not is_plain(j, k)]

        def taps(buf, t, w, r):
            return buf[t, HALO - DIL * w + r:HALO - DIL * w + r + 8, :]

        def logit_at(r, w):
            return PR0 + w // 4, slice(r, r + 8), _cols(w % 4)

        def window_logits(r, ws):
            q = [qb[t + zero, HALO + r:HALO + r + 8, :] for t in range(8)]
            logits = [functools.reduce(jnp.add, [q[t] * taps(kb, t, w, r) for t in range(8)])
                      for w in ws]
            logits = [z + pltpu.roll(z, 64, 1) for z in logits]
            logits = [(z + pltpu.roll(z, 32, 1)) * (DB ** -0.5 * LOG2E) for z in logits]
            pos = i * RC + r + lax.broadcasted_iota(jnp.int32, (8, 128), 0)
            return [(wide, logit_at(r, w),
                     pltpu.bitcast(jnp.where(pos >= DIL * w, z, NEG) if DIL * w > r else z, U32))
                    for w, z in zip(ws, logits)]

        weights = {}

        def window_softmax(r):
            logits = [pltpu.bitcast(wide[logit_at(r, w)], F32) for w in range(WIN)]
            peak = functools.reduce(jnp.maximum, logits)
            probs = [jnp.exp2(z - peak) for z in logits]
            inv = _recip(functools.reduce(jnp.add, probs))
            weights[r] = [z * inv for z in probs]
            return []

        def window_values(r, ts):
            return [(wide, (LOC0 + r // hr, slice(r % hr + (t % 2) * hr, r % hr + (t % 2) * hr + 8),
                            _cols(t // 2)),
                     pltpu.bitcast(functools.reduce(
                         jnp.add, [weights[r][w] * taps(vb, t, w, r) for w in range(WIN)]), U32))
                    for t in ts]

        n_steps = 3 * 4 * 7 + 2 * 49
        side = _SideWork()
        side.add([P(ctx_factors, u, lo, js) for u in range(8) for lo in range(0, qw, 8)
                  for js in ((2, 4, 5), (3, 1, 0, 6))], range(CTX_FIRST, CTX_LAST), 0)
        side.add([P(window_logits, r, ws) for r in range(0, RC, 8)
                  for ws in ((0, 4, 1, 5), (2, 6, 3, 7))],
                 range(LOGIT_FIRST, VALUE_FIRST - LOGIT_LAG), LOGIT_LAG)
        side.add([P(window_softmax, r) for r in range(0, RC, 8)],
                 range(VALUE_FIRST, n_steps - 1), 0)
        side.add([P(window_values, r, ts) for r in range(0, RC, 8)
                  for ts in (range(4), range(4, 8))], range(VALUE_FIRST + 1, n_steps), 0)
        wide_alias = wide.at[pl.ds(zero, PR0)]

        def mul(lhs, slab, *tiles):
            side.step()
            rhs = jnp.concatenate([wide[slab, :, _cols(t)] for t in tiles], axis=0)
            rhs = _with_corner(rhs, wide_alias[slab, 0:8, _cols(tiles[0])])
            val = _dot(_bf(lhs), _bf(rhs))
            qb[0, 0:8, :] = val[0:8]
            return val

        x_fac = _factors_of_words(_lhs_factors, *[
            x[pl.ds(base + r * hr // 2, hr // 2), k * W:(k + 1) * W]
            for r in range(2) for k in range(2)])
        for part, buf in ((1, kb), (0, qb), (2, vb)):
            if part:
                buf[:, 0:HALO, :] = buf[:, RC:RC + HALO, :]
            for t in range(4):
                blocks = _strassen(lambda j: mul(x_fac[j], QKV0 + 7 * part + j, t))
                for n, val in enumerate(blocks):
                    r, k = divmod(n, 2)
                    buf[4 * k + t, HALO + r * hr:HALO + (r + 1) * hr, :] = val

        def ctx_factor(j, k):
            return jnp.concatenate(
                [ref[idx] for ref, idx in (ctx_at(j, k, u, 0, qw) for u in range(8))], axis=1)

        for t in range(2):
            blocks = _strassen(lambda j: jnp.concatenate(_strassen(
                lambda k: mul(ctx_factor(j, k), OA0 + 7 * j + k, 2 * t, 2 * t + 1)), axis=0))
            for outer, val in enumerate(blocks):
                for inner in range(4):
                    r = 2 * (outer // 2) + inner // 2
                    k = 2 * (outer % 2) + inner % 2
                    obuf[slot, r * 2 * qw:(r + 1) * 2 * qw, _cols(2 * k + t)] = (
                        val[inner * 2 * qw:(inner + 1) * 2 * qw].astype(BF16))
        side.check_done()

        o_fac = [z.astype(BF16) for z in _lhs_factors(*[
            pltpu.bitcast(wide[LOC0 + r, e * hr:(e + 1) * hr, :], F32)
            for r in range(2) for e in range(2)])]
        for t in range(4):
            blocks = _strassen(lambda j: _dot(o_fac[j], _bf(wide[OB0 + j, :, _cols(t)])))
            for n, val in enumerate(blocks):
                r, k = divmod(n, 2)
                obuf[slot, r * hr:(r + 1) * hr, _cols(8 + 4 * k + t)] = val.astype(BF16)

        out_copy(i, slot).start()
        return -zero

    lax.fori_loop(0, n_chunks, chunk_body, 0)
    out_copy(n_chunks - 2, 0).wait()
    out_copy(n_chunks - 1, 1).wait()


@jax.jit
def pallas_concat_heads__compressed_kv_cla__sliding_local_dilated__prompt_kernel(
    A_x: jax.Array,
    A_c_kv: jax.Array,
    A_w_q: jax.Array,
    A_w_uk: jax.Array,
    A_w_uv: jax.Array,
    A_w_o: jax.Array,
    B_x: jax.Array,
    B_wqkv: jax.Array,
    B_wo: jax.Array,
):
    window_buf = pltpu.VMEM((8, HALO + RC + 8, 128), F32)
    scratch = [
        pltpu.VMEM((S // 2, M), U32),
        pltpu.VMEM((5, S // 4, W), U32),
        pltpu.VMEM((N_SLABS, SLAB, W), U32),
        pltpu.VMEM((2 * NG + 1, G // 4, DC), U32),
        pltpu.VMEM((5, S // 4, DC // 2), U32),
        pltpu.VMEM((NP, 2, 7, DC // 4, D), U32),
        pltpu.VMEM((2, S // 2, D), U32),
        pltpu.VMEM((2, S // 2, D), U32),
        pltpu.VMEM((H + 2, S // 2, D), U32),
        pltpu.VMEM((2 * PP, 2, M // 2, D), U32),
        pltpu.VMEM((RING * PP + 1, 2, DC // 2, D), U32),
        pltpu.VMEM((RING * PP + 1, 2, DC // 2, D), U32),
        pltpu.VMEM((RING, PP * D + 8, M), U32),
        pltpu.VMEM((RING, 2, PP * 16 + 8, 3 * M), U32),
        pltpu.VMEM((RING * PP, HB, M), U32),
        window_buf,
        window_buf,
        window_buf,
        pltpu.VMEM((2, RC, 2 * M), BF16),
        pltpu.SemaphoreType.DMA((NG,)),
        pltpu.SemaphoreType.DMA((RING,)),
        pltpu.SemaphoreType.DMA((PP + 1,)),
        pltpu.SemaphoreType.DMA((2,)),
    ]
    out = pl.pallas_call(
        _kernel,
        out_shape=jax.ShapeDtypeStruct((S, 2 * M), BF16),
        in_specs=[pl.BlockSpec(memory_space=pl.ANY)] * 9,
        out_specs=pl.BlockSpec(memory_space=pl.ANY),
        scratch_shapes=scratch,
        compiler_params=pltpu.CompilerParams(
            vmem_limit_bytes=127 * 2**20, disable_bounds_checks=True),
        name="fused_mla_sliding",
    )(
        A_x.reshape(S, M),
        A_c_kv.reshape(2 * NG, G // 2, DC),
        A_w_q.reshape(M // 2, 2, H, D),
        A_w_uk.reshape(DC // 2, 2, H, D),
        A_w_uv.reshape(DC // 2, 2, H, D),
        A_w_o.reshape(H * D, M),
        B_x.reshape(S, M),
        B_wqkv.reshape(2, M // 2, 3 * M),
        B_wo.reshape(HB, DB, M),
    )
    return out.reshape(1, S, 2 * M)
```

```python
import functools

import jax
import jax.numpy as jnp
import numpy as np
from jax import lax
import jax.experimental.pallas as pl
import jax.experimental.pallas.tpu as pltpu

S = 2048
M = 1024
DC = 512
H = 32
D = 128
HB = 32
DB = 32
WIN = 8
DIL = 2

NP = H // 2
PP = 2
NS = NP // PP
RING = 4
G = 512
NG = S // G
BQ = 128
RC = 256
HALO = 16
LOG2E = 1.4426950408889634
NEG = -1e9 * LOG2E

W = M // 2
SLAB = M // 4
OA0 = 0
QKV0 = OA0 + 49
OB0 = QKV0 + 21
CS0 = OB0 + 7
LOC0 = CS0 + 13
GATE = LOC0 + 2
N_SLABS = GATE + 1

SKIP0 = 4
LAG0 = 3
SKIP1 = 0
LAG1 = 3
CTX_FIRST = 5
CTX_LAST = 85
LOGIT_FIRST = 84
LOGIT_LAST = 174
LOGIT_LAG = 6
VALUE_FIRST = 98

F32 = jnp.float32
BF16 = jnp.bfloat16
U32 = jnp.uint32
_NT = (((1,), (1,)), ((), ()))


def _attention_order():
    ops = ("Sa0 Sa1 Sa2 Sa3 v0 k1 Pa0 Pa1 Pa2 v1 Sa4 Pa3 k2 Sa5 Wa0 Wa1 Pa4 v2 "
           "Sa6 Wa2 Pa5 Wa3 k3 Sa7 Pa6 Wa4 v3").split()
    for i in range(8, 16):
        ops += [f"Sa{i}", f"Pa{i - 1}", f"Wa{i - 3}"]
    ops += "Sb15 Pa15 Wa13 Sb14 Pb15 Wa14 Sb13 Pb14 Wa15".split()
    for i in range(12, 3, -1):
        ops += [f"Sb{i}", f"Pb{i + 1}", f"Wb{i + 3}"]
    return ops + "Sb3 Sb2 Pb4 Wb6 Sb1 Sb0 Pb3 Pb2 k0 Pb1 Pb0 Wb5 Wb4 Wb3 Wb2 Wb1 Wb0".split()


def _dot(a, b):
    return jnp.dot(a, b, preferred_element_type=F32)


def _bf(words):
    return pltpu.bitcast(words, BF16)


def _words(x):
    return pltpu.bitcast(x.astype(BF16), U32)


def _halves(words):
    return (pltpu.bitcast(words << 16, F32),
            pltpu.bitcast(words & np.uint32(0xFFFF0000), F32))


def _pack(lo, hi):
    return pltpu.bitcast(pltpu.pack_elementwise([lo, hi], packed_dtype=BF16), U32)


def _words_shuffled(x):
    n, c = x.shape
    x = x.reshape(n // 16, 2, 8, c)
    return _pack(x[:, 0], x[:, 1]).reshape(n // 2, c)


def _recip(x):
    r = pl.reciprocal(x, approx=True)
    return r * (2.0 - x * r)


def _lhs_factors(a11, a12, a21, a22):
    return a11 + a22, a21 + a22, a11, a22, a11 + a12, a21 - a11, a12 - a22


def _rhs_factors(b11, b12, b21, b22):
    return b11 + b22, b11, b12 - b22, b21 - b11, b22, b11 + b12, b21 + b22


def _strassen(mul):
    m3 = mul(2)
    m4 = mul(3)
    m5 = mul(4)
    c12 = m3 + m5
    m2 = mul(1)
    c21 = m2 + m4
    m1 = mul(0)
    c11 = (m4 - m5) + m1 + mul(6)
    c22 = (m3 - m2) + m1 + mul(5)
    return c11, c12, c21, c22


def _factors_of_words(factors, *blocks):
    parts = [_halves(b) for b in blocks]
    plain = {id(lo): b for (lo, _), b in zip(parts, blocks)}
    return [plain.get(id(lo)) if id(lo) in plain else _pack(lo, hi)
            for lo, hi in zip(factors(*[x[0] for x in parts]), factors(*[x[1] for x in parts]))]


def _nested_factors_of_words(factors, blocks):
    sides = []
    for side in range(2):
        vals = [[_halves(b)[side] for b in row] for row in blocks]
        inner = [factors(*[vals[2 * r + ri][2 * c + ci] for r in range(2) for c in range(2)])
                 for ri in range(2) for ci in range(2)]
        sides.append([factors(*[x[j] for x in inner]) for j in range(7)])
    return [[_pack(lo, hi) for lo, hi in zip(a, b)] for a, b in zip(*sides)]


def _permute_head_columns(words):
    tiles = [words[:, _cols(t)] for t in range(8)]
    lane = lax.broadcasted_iota(jnp.int32, tiles[0].shape, 1)
    for bit in (1, 2, 4):
        low = (lane & bit) == 0
        for t in range(8):
            if t & bit:
                continue
            a, b = tiles[t], tiles[t | bit]
            tiles[t] = jnp.where(low, a, pltpu.roll(b, bit, 1))
            tiles[t | bit] = jnp.where(low, pltpu.roll(a, 128 - bit, 1), b)
    src = ((lane & 3) << 5) | (lane >> 2)
    return jnp.concatenate([jnp.take_along_axis(x, src, axis=1) for x in tiles], axis=1)


def _with_corner(x, corner):
    top = corner if x.shape[1] == 128 else jnp.concatenate([corner, x[0:8, 128:]], axis=1)
    return jnp.concatenate([top, x[8:]], axis=0)


class _SideWork:
    def __init__(self):
        self.now = 0
        self.starts = {}
        self.stores = {}

    def add(self, tasks, steps, lag):
        for n, task in enumerate(tasks):
            self.starts.setdefault(steps[n * len(steps) // len(tasks)], []).append((task, lag))

    def step(self):
        for task, lag in self.starts.pop(self.now, []):
            self.stores.setdefault(self.now + lag, []).extend(task())
        for ref, idx, val in self.stores.pop(self.now, []):
            ref[idx] = val
        self.now += 1

    def check_done(self):
        assert not self.starts and not self.stores


def _mult(i, n):
    return i * n if isinstance(i, int) else pl.multiple_of(i * n, n)


def _cols(t):
    return slice(t * 128, (t + 1) * 128)


def _start(copies):
    for cp in copies:
        cp.start()


def _wait(copies):
    for cp in copies:
        cp.wait()


def _kernel(
    xa_hbm, c_hbm, wq_hbm, wk_hbm, wv_hbm, woa_hbm, xb_hbm, wqkv_hbm, wob_hbm,
    out_hbm,
    x, x_sum, wide, c, c_sum, kv_fac, k_buf, v_buf, ctx,
    wq_raw, wk_raw, wv_raw, woa_raw, wqkv_raw, wob_raw, qb, kb, vb, lb, obuf,
    sem_x, sem_w, sem_misc, sem_out,
):
    P = functools.partial
    xa32, c32, woa32, xb32, wqkv32 = (
        r.bitcast(U32) for r in (xa_hbm, c_hbm, woa_hbm, xb_hbm, wqkv_hbm))
    wq32, wk32, wv32, wob32 = (r.bitcast(U32) for r in (wq_hbm, wk_hbm, wv_hbm, wob_hbm))

    def pair_copies(src, dst, pair, ring, sem):
        slot = pair & (ring * PP - 1)
        return [pltpu.make_async_copy(src.at[:, odd, pair, :], dst.at[slot, odd], sem)
                for odd in range(2)]

    def wq_copies(step):
        sem = sem_w.at[step & (RING - 1)]
        return [cp for j in range(PP) for cp in pair_copies(wq32, wq_raw, step * PP + j, 2, sem)]

    def later_copies(part):
        sem, slot = sem_w.at[(part + 1) & (RING - 1)], part & (RING - 1)
        copies = []
        for j in range(PP):
            pair = part * PP + j
            copies += pair_copies(wk32, wk_raw, pair, RING, sem)
            copies += pair_copies(wv32, wv_raw, pair, RING, sem)
            copies.append(pltpu.make_async_copy(
                wob32.at[:, pair, :], wob_raw.at[pair & (RING * PP - 1)], sem))
        copies.append(pltpu.make_async_copy(
            woa32.at[pl.ds(_mult(part, PP * D), PP * D)], woa_raw.at[slot, 0:PP * D], sem))
        for h in range(2):
            copies.append(pltpu.make_async_copy(
                wqkv32.at[h, pl.ds(_mult(part, PP * 16), PP * 16)],
                wqkv_raw.at[slot, h, 0:PP * 16], sem))
            rows = (2 * (part >> 1) + h, pl.ds(_mult(part & 1, G // 8), G // 8))
            copies.append(pltpu.make_async_copy(c32.at[rows], c.at[rows], sem))
        return copies

    x_copies = [pltpu.make_async_copy(xa32.at[g * G // 2:(g + 1) * G // 2],
                                      x.at[g * G // 2:(g + 1) * G // 2], sem_x.at[g])
                for g in range(NG)]
    first_wq = [pair_copies(wq32, wq_raw, j, 2, sem_misc.at[j]) for j in range(PP)]
    xb_copy = pltpu.make_async_copy(xb32, x, sem_misc.at[PP])

    gw = G // 4
    sum_index = {0: 0, 1: 1, 4: 2, 5: 3, 6: 4}

    def head_factors(raw, slot, top, bottom, n):
        sides = [_rhs_factors(*_halves(raw[slot, odd, top:top + n, :]),
                              *_halves(raw[slot, odd, bottom:bottom + n, :]))
                 for odd in range(2)]
        return [_pack(even, odd) for even, odd in zip(*sides)]

    def group_blocks(g, mul):
        for n, val in enumerate(_strassen(mul)):
            r, e = divmod(n, 2)
            yield e, slice((2 * g + r) * gw, (2 * g + r + 1) * gw), val

    def project_kv(n, pair, g):
        def lhs(j):
            if j in sum_index:
                return c_sum[sum_index[j], g * gw:(g + 1) * gw, :]
            return c[2 * g + j - 2, :, (j - 2) * DC // 2:(j - 1) * DC // 2]

        for e, rows, val in group_blocks(g, lambda j: _dot(_bf(lhs(j)), _bf(kv_fac[pair, n, j]))):
            val = _words_shuffled(val)
            (k_buf, v_buf)[n][e, rows, :] = val
            if n == 0 and rows.start == 0:
                ctx[H + e, 0:BQ // 2, :] = val[0:BQ // 2]

    def prepare_kv(n, pair, piece):
        vals = head_factors((wk_raw, wv_raw)[n], pair & (RING * PP - 1),
                            piece * 16, DC // 4 + piece * 16, 16)
        return [(kv_fac, (pair, n, j, slice(piece * 16, (piece + 1) * 16)), val)
                for j, val in enumerate(vals)]

    def prepare_c(part, piece):
        r = _mult(part & 1, G // 8) + 16 * piece
        vals = _factors_of_words(_lhs_factors, *[
            c[2 * (part >> 1) + h, pl.ds(r, 16), k * DC // 2:(k + 1) * DC // 2]
            for h in range(2) for k in range(2)])
        return [(c_sum, (n, pl.ds(_mult(part >> 1, gw) + r, 16)), vals[j])
                for j, n in sum_index.items()]

    def prepare_wqkv(part, piece, which):
        both = _permute_head_columns(jnp.concatenate([
            wqkv_raw[part & (RING - 1), h, 8 * piece:8 * piece + 8, which * M:(which + 1) * M]
            for h in range(2)], axis=0))
        vals = _factors_of_words(
            _rhs_factors, both[:8, :W], both[:8, W:], both[8:, :W], both[8:, W:])
        r = _mult(part, PP * 16) + 8 * piece
        return [(wide, (QKV0 + 7 * which + j, pl.ds(r, 8)), val) for j, val in enumerate(vals)]

    def prepare_wob(pair, t):
        b11, b21 = _halves(wob_raw[pair & (RING * PP - 1), :, _cols(t)])
        b12, b22 = _halves(wob_raw[pair & (RING * PP - 1), :, _cols(4 + t)])
        r = _mult((pair & 3) * 4 + (pair >> 2), HB // 2)
        return [(wide, (OB0 + j, pl.ds(r, HB // 2), _cols(t)), _words(val))
                for j, val in enumerate(_rhs_factors(b11, b12, b21, b22))]

    def prepare_woa(part, t, n):
        fac = _nested_factors_of_words(_rhs_factors, [
            [woa_raw[part & (RING - 1), hq * D // 2 + 8 * n:hq * D // 2 + 8 * n + 8, _cols(2 * k + t)]
             for k in range(4)] for hq in range(4)])
        rows = pl.ds(_mult(part & 3, D // 2) + 8 * n, 8)
        cols = pl.ds(_mult(2 * t + (part >> 2), 128), 128)
        return [(wide, (OA0 + 7 * j + k, rows, cols), fac[j][k]) for j in range(7) for k in range(7)]

    def later_tasks(part):
        tasks = []
        for j in range(PP):
            pair = part * PP + j
            for n in range(8):
                tasks += [P(prepare_kv, 1, pair, n), P(prepare_woa, part, j, n)]
                if n < 6:
                    tasks.append(P(prepare_wqkv, part, 2 * j + n // 3, n % 3))
                tasks.append(P(prepare_kv, 0, pair, n))
                if n % 2:
                    tasks.append(P(prepare_wob, pair, n // 2))
                elif n % 4 == 0:
                    tasks.append(P(prepare_c, part, 2 * j + n // 4))
        return tasks

    def x_factor(j, g):
        if j in sum_index:
            return x_sum[sum_index[j], g * gw:(g + 1) * gw, :]
        return x[(2 * g + j - 2) * gw:(2 * g + j - 1) * gw, (j - 2) * W:(j - 1) * W]

    def gate(g, j):
        return GATE, slice(8 * (7 * g + j), 8 * (7 * g + j + 1)), _cols(0)

    def make_x_factors(g):
        vals = _factors_of_words(_lhs_factors, *[
            x[(2 * g + r) * gw:(2 * g + r + 1) * gw, k * W:(k + 1) * W]
            for r in range(2) for k in range(2)])
        for j, n in sum_index.items():
            x_sum[n, g * gw:(g + 1) * gw, :] = vals[j]
        for j in range(7):
            wide[gate(g, j)] = vals[j][0:8, 0:128]

    def project_q(pair, g, mul):
        for e, rows, val in group_blocks(g, mul):
            ctx[2 * pair + e, rows, :] = _words(val * (D ** -0.5 * LOG2E))

    def wq_factors(pair):
        return head_factors(wq_raw, pair & (2 * PP - 1), 0, M // 4, M // 4)

    _start(first_wq[0] + x_copies[:2] + first_wq[1] + x_copies[2:]
           + wq_copies(1) + later_copies(0) + later_copies(1))
    kb[:, RC:RC + HALO, :] = jnp.zeros((8, HALO, 128), F32)
    vb[:, RC:RC + HALO, :] = jnp.zeros((8, HALO, 128), F32)

    def keep_wq_factors(pair):
        fac = wq_factors(pair)
        for j, val in enumerate(fac):
            kv_fac[NP - 1 - pair, :, j] = val.reshape(2, DC // 4, D)
        return fac

    def first_q(pair, g, fac=None):
        project_q(pair, g, lambda j: _dot(_bf(x_factor(j, g)), _bf(
            fac[j] if fac else kv_fac[NP - 1 - pair, :, j].reshape(M // 4, D))))

    _wait(first_wq[0])
    keep_wq_factors(0)
    for g in range(2):
        x_copies[g].wait()
        make_x_factors(g)
        first_q(0, g)
    _wait(first_wq[1])
    first_q(1, 0, keep_wq_factors(1))
    first_q(1, 1)
    _wait(x_copies[2:])
    for g in range(2, NG):
        make_x_factors(g)
        first_q(0, g)
        first_q(1, g)

    def q_step(step, parts, zero, skip, lag):
        side = _SideWork()
        side.add([task for part in parts for task in later_tasks(part)],
                 [n for n in range(7 * NG * PP - lag - 3) if n % (7 * NG) >= skip], lag)

        def mul(fac, g, j):
            side.step()
            val = _dot(_bf(_with_corner(x_factor(j, g), wide[gate(g, j)])), _bf(fac[j]))
            token = pltpu.bitcast(val[0:8], U32)
            wqkv_raw[zero, 0, PP * 16:PP * 16 + 8, _cols(0)] = token
            wk_raw[RING * PP + zero, 0, 0:8] = token
            wv_raw[RING * PP + zero, 0, 0:8] = token
            c[2 * NG + zero, 0:8, _cols(0)] = token
            if len(parts) > 1:
                woa_raw[zero, PP * D:PP * D + 8, _cols(0)] = token
            return val

        for pair in (step * PP + j for j in range(PP)):
            fac = wq_factors(pair)
            for g in range(NG):
                project_q(pair, g, P(mul, fac, g))
        side.check_done()

    def q_body(step, zero):
        _start(wq_copies(step + 1) + later_copies(step + 1))
        _wait(wq_copies(step) + later_copies(step - 1))
        q_step(step, [step - 1], zero, SKIP0, LAG0)
        return -zero

    zero = lax.fori_loop(1, NS - 1, q_body, 0)
    _wait(wq_copies(NS - 1) + later_copies(NS - 2) + later_copies(NS - 1))
    q_step(NS - 1, [zero + NS - 2, zero + NS - 1], zero, SKIP1, LAG1)
    project_kv(0, 0, 0)
    xb_copy.start()

    def pair_body(p, zero):
        row = lax.broadcasted_iota(jnp.int32, (BQ, BQ), 0)
        col = lax.broadcasted_iota(jnp.int32, (BQ, BQ), 1)
        causal = ((col & ~15) | ((col & 15) >> 1) | ((col & 1) << 3)) <= row
        hb = BQ // 2

        def scores(e, i):
            r = i * BQ
            k = ctx[H + e + zero, 0:hb, :]
            k = _bf(jnp.concatenate([k, k_buf[e, hb:(i + 1) * hb, :]], axis=0) if i else k)
            q = _bf(ctx[2 * p + e, i * hb:(i + 1) * hb, :])
            s = lax.dot_general(q, k, _NT, preferred_element_type=F32)
            diag = jnp.where(causal, s[:, r:], NEG)
            s = jnp.concatenate([s[:, :r], diag], axis=1) if r else diag
            return s, jnp.max(s, axis=1, keepdims=True)

        def context(e, i, s, peak):
            w = jnp.exp2(s - peak)
            total = jnp.sum(w, axis=1, keepdims=True)
            o = _dot(w.astype(BF16), _bf(v_buf[e, 0:(i + 1) * hb, :]))
            return _words(o * _recip(total))

        state = {}
        for op in _attention_order():
            if op[0] in "kv":
                pair = jnp.minimum(p + 1, NP - 1) if op == "k0" else p
                project_kv("kv".index(op[0]), pair, int(op[1:]))
                continue
            e, i = "ab".index(op[1]), int(op[2:])
            if op[0] == "S":
                state[e, i] = scores(e, i)
            elif op[0] == "P":
                state[e, i] = context(e, i, *state[e, i])
            else:
                ctx[2 * p + e, i * hb:(i + 1) * hb, :] = state.pop((e, i))
        assert not state
        return -zero

    lax.fori_loop(0, NP, pair_body, 0)
    xb_copy.wait()

    n_chunks = S // RC
    hr = RC // 2
    qw = RC // 8

    def out_copy(i, slot):
        return pltpu.make_async_copy(
            obuf.at[slot], out_hbm.at[pl.ds(_mult(i, RC), RC), :], sem_out.at[slot])

    def chunk_body(i, zero):
        slot = i & 1
        base = _mult(i, RC // 2)

        @pl.when(i >= 2)
        def _():
            out_copy(i - 2, slot).wait()

        def is_plain(j, k):
            return j in (2, 3) and k in (2, 3)

        def ctx_at(j, k, u, lo, n):
            if is_plain(j, k):
                quarter = 2 * (j - 2) + k - 2
                return ctx, (4 * u + quarter, pl.ds(base + quarter * qw + lo, n))
            slab, r = divmod((2 * (7 * j + k) + u // 4) * qw + lo, SLAB)
            return wide, (CS0 + slab, slice(r, r + n), _cols(u % 4))

        ctx_fac = {}

        def ctx_factor_store(u, lo, j, k):
            if (u, lo) not in ctx_fac:
                ctx_fac[u, lo] = _nested_factors_of_words(_lhs_factors, [
                    [ctx[4 * u + hq, pl.ds(base + r * qw + lo, 8)] for hq in range(4)]
                    for r in range(4)])
            return [ctx_at(j, k, u, lo, 8) + (ctx_fac[u, lo][j][k],)]

        def taps(buf, t, w, r):
            return buf[t, HALO - DIL * w + r:HALO - DIL * w + r + 8, :]

        def window_logits(r, ws):
            q = [qb[t + zero, HALO + r:HALO + r + 8, :] for t in range(8)]
            logits = [functools.reduce(jnp.add, [q[t] * taps(kb, t, w, r) for t in range(8)])
                      for w in ws]
            logits = [z + pltpu.roll(z, 64, 1) for z in logits]
            logits = [(z + pltpu.roll(z, 32, 1)) * (DB ** -0.5 * LOG2E) for z in logits]
            pos = i * RC + r + lax.broadcasted_iota(jnp.int32, (8, 128), 0)
            return [(lb, (w, slice(r, r + 8)), jnp.where(pos >= DIL * w, z, NEG) if DIL * w > r else z)
                    for w, z in zip(ws, logits)]

        weights = {}

        def window_softmax(r):
            logits = [lb[w + zero, r:r + 8, :] for w in range(WIN)]
            peak = functools.reduce(jnp.maximum, logits)
            probs = [jnp.exp2(z - peak) for z in logits]
            inv = _recip(functools.reduce(jnp.add, probs))
            weights[r] = [z * inv for z in probs]
            return []

        def window_values(r, ts):
            return [(wide, (LOC0 + r // hr, slice(r % hr + (t % 2) * hr, r % hr + (t % 2) * hr + 8),
                            _cols(t // 2)),
                     pltpu.bitcast(functools.reduce(
                         jnp.add, [weights[r][w] * taps(vb, t, w, r) for w in range(WIN)]), U32))
                    for t in ts]

        n_steps = 3 * 4 * 7 + 2 * 49
        order = (2, 4, 3, 1, 0, 6, 5)
        side = _SideWork()
        side.add([P(ctx_factor_store, u, lo, j, k) for u in range(8) for lo in range(0, qw, 8)
                  for j in order for k in order if not is_plain(j, k)], range(CTX_FIRST, CTX_LAST), 0)
        side.add([P(window_logits, r, ws) for r in range(0, RC, 8)
                  for ws in ((0, 4, 1, 5), (2, 6, 3, 7))],
                 range(LOGIT_FIRST, LOGIT_LAST - LOGIT_LAG), LOGIT_LAG)
        side.add([P(window_softmax, r) for r in range(0, RC, 8)],
                 range(VALUE_FIRST, n_steps - 2), 0)
        side.add([P(window_values, r, ts) for r in range(0, RC, 8)
                  for ts in (range(4), range(4, 8))], range(VALUE_FIRST + 2, n_steps), 0)
        wide_alias = wide.at[pl.ds(zero, CS0)]

        def mul(lhs, slab, *tiles):
            side.step()
            rhs = jnp.concatenate([wide[slab, :, _cols(t)] for t in tiles], axis=0)
            rhs = _with_corner(rhs, wide_alias[slab, 0:8, _cols(tiles[0])])
            val = _dot(_bf(lhs), _bf(rhs))
            qb[0, 0:8, :] = val[0:8]
            lb[0, RC:RC + 8, :] = val[0:8]
            return val

        x_fac = _factors_of_words(_lhs_factors, *[
            x[pl.ds(base + r * hr // 2, hr // 2), k * W:(k + 1) * W]
            for r in range(2) for k in range(2)])
        for part, buf in ((1, kb), (0, qb), (2, vb)):
            if part:
                buf[:, 0:HALO, :] = buf[:, RC:RC + HALO, :]
            for t in range(4):
                blocks = _strassen(lambda j: mul(x_fac[j], QKV0 + 7 * part + j, t))
                for n, val in enumerate(blocks):
                    r, k = divmod(n, 2)
                    buf[4 * k + t, HALO + r * hr:HALO + (r + 1) * hr, :] = val

        def ctx_factor(j, k):
            return jnp.concatenate(
                [ref[idx] for ref, idx in (ctx_at(j, k, u, 0, qw) for u in range(8))], axis=1)

        for t in range(2):
            blocks = _strassen(lambda j: jnp.concatenate(_strassen(
                lambda k: mul(ctx_factor(j, k), OA0 + 7 * j + k, 2 * t, 2 * t + 1)), axis=0))
            for outer, val in enumerate(blocks):
                for inner in range(4):
                    r = 2 * (outer // 2) + inner // 2
                    k = 2 * (outer % 2) + inner % 2
                    obuf[slot, r * 2 * qw:(r + 1) * 2 * qw, _cols(2 * k + t)] = (
                        val[inner * 2 * qw:(inner + 1) * 2 * qw].astype(BF16))
        side.check_done()

        o_fac = [z.astype(BF16) for z in _lhs_factors(*[
            pltpu.bitcast(wide[LOC0 + r, e * hr:(e + 1) * hr, :], F32)
            for r in range(2) for e in range(2)])]
        for t in range(4):
            blocks = _strassen(lambda j: _dot(o_fac[j], _bf(wide[OB0 + j, :, _cols(t)])))
            for n, val in enumerate(blocks):
                r, k = divmod(n, 2)
                obuf[slot, r * hr:(r + 1) * hr, _cols(8 + 4 * k + t)] = val.astype(BF16)

        out_copy(i, slot).start()
        return -zero

    lax.fori_loop(0, n_chunks, chunk_body, 0)
    out_copy(n_chunks - 2, 0).wait()
    out_copy(n_chunks - 1, 1).wait()


@jax.jit
def pallas_concat_heads__compressed_kv_cla__sliding_local_dilated__prompt_kernel(
    A_x: jax.Array,
    A_c_kv: jax.Array,
    A_w_q: jax.Array,
    A_w_uk: jax.Array,
    A_w_uv: jax.Array,
    A_w_o: jax.Array,
    B_x: jax.Array,
    B_wqkv: jax.Array,
    B_wo: jax.Array,
):
    window_buf = pltpu.VMEM((8, HALO + RC + 8, 128), F32)
    scratch = [
        pltpu.VMEM((S // 2, M), U32),
        pltpu.VMEM((5, S // 4, W), U32),
        pltpu.VMEM((N_SLABS, SLAB, W), U32),
        pltpu.VMEM((2 * NG + 1, G // 4, DC), U32),
        pltpu.VMEM((5, S // 4, DC // 2), U32),
        pltpu.VMEM((NP, 2, 7, DC // 4, D), U32),
        pltpu.VMEM((2, S // 2, D), U32),
        pltpu.VMEM((2, S // 2, D), U32),
        pltpu.VMEM((H + 2, S // 2, D), U32),
        pltpu.VMEM((2 * PP, 2, M // 2, D), U32),
        pltpu.VMEM((RING * PP + 1, 2, DC // 2, D), U32),
        pltpu.VMEM((RING * PP + 1, 2, DC // 2, D), U32),
        pltpu.VMEM((RING, PP * D + 8, M), U32),
        pltpu.VMEM((RING, 2, PP * 16 + 8, 3 * M), U32),
        pltpu.VMEM((RING * PP, HB, M), U32),
        window_buf,
        window_buf,
        window_buf,
        window_buf,
        pltpu.VMEM((2, RC, 2 * M), BF16),
        pltpu.SemaphoreType.DMA((NG,)),
        pltpu.SemaphoreType.DMA((RING,)),
        pltpu.SemaphoreType.DMA((PP + 1,)),
        pltpu.SemaphoreType.DMA((2,)),
    ]
    out = pl.pallas_call(
        _kernel,
        out_shape=jax.ShapeDtypeStruct((S, 2 * M), BF16),
        in_specs=[pl.BlockSpec(memory_space=pl.ANY)] * 9,
        out_specs=pl.BlockSpec(memory_space=pl.ANY),
        scratch_shapes=scratch,
        compiler_params=pltpu.CompilerParams(
            vmem_limit_bytes=127 * 2**20, disable_bounds_checks=True),
        name="fused_mla_sliding",
    )(
        A_x.reshape(S, M),
        A_c_kv.reshape(2 * NG, G // 2, DC),
        A_w_q.reshape(M // 2, 2, H, D),
        A_w_uk.reshape(DC // 2, 2, H, D),
        A_w_uv.reshape(DC // 2, 2, H, D),
        A_w_o.reshape(H * D, M),
        B_x.reshape(S, M),
        B_wqkv.reshape(2, M // 2, 3 * M),
        B_wo.reshape(HB, DB, M),
    )
    return out.reshape(1, S, 2 * M)
```

```python
import functools

import jax
import jax.numpy as jnp
import numpy as np
from jax import lax
import jax.experimental.pallas as pl
import jax.experimental.pallas.tpu as pltpu

S = 2048
M = 1024
DC = 512
H = 32
D = 128
HB = 32
DB = 32
WIN = 8
DIL = 2

NP = H // 2
PP = 2
NS = NP // PP
RING = 3
G = 512
NG = S // G
BQ = 128
RC = 256
HALO = 16
LOG2E = 1.4426950408889634
NEG = -1e9 * LOG2E

W = M // 2
SLAB = M // 4
OA0 = 0
QKV0 = OA0 + 49
OB0 = QKV0 + 21
CS0 = OB0 + 7
LOC0 = CS0 + 13
GATE = CS0
N_SLABS = LOC0 + 2

SPLIT = 2
PACE0 = (0, 88, (3, 6, 0), (7, 1, 0.5), (0, 2, 0.5), (0, 2, 0))
PACE1 = (0, 80, (6, 1, 0), (7, 1, 0.25), (0, 1, 0), (1, 1, 0.5))
CTX_FIRST = 5
CTX_LAST = 85
LOGIT_FIRST = 84
LOGIT_LAST = 174
LOGIT_LAG = 6
VALUE_FIRST = 98

F32 = jnp.float32
BF16 = jnp.bfloat16
U32 = jnp.uint32
_NT = (((1,), (1,)), ((), ()))


def _attention_order():
    ops = ("Sa0 Sa1 Sa2 Sa3 v0 k1 Pa0 Pa1 Pa2 v1 Sa4 Pa3 k2 Sa5 Wa0 Wa1 Pa4 v2 "
           "Sa6 Wa2 Pa5 Wa3 k3 Sa7 Pa6 Wa4 v3").split()
    for i in range(8, 16):
        ops += [f"Sa{i}", f"Pa{i - 1}", f"Wa{i - 3}"]
    ops += "Sb15 Pa15 Wa13 Sb14 Pb15 Wa14 Sb13 Pb14 Wa15".split()
    for i in range(12, 3, -1):
        ops += [f"Sb{i}", f"Pb{i + 1}", f"Wb{i + 3}"]
    return ops + "Sb3 Sb2 Pb4 Wb6 Sb1 Sb0 Pb3 Pb2 k0 Pb1 Pb0 Wb5 Wb4 Wb3 Wb2 Wb1 Wb0".split()


def _dot(a, b):
    return jnp.dot(a, b, preferred_element_type=F32)


def _bf(words):
    return pltpu.bitcast(words, BF16)


def _words(x):
    return pltpu.bitcast(x.astype(BF16), U32)


def _halves(words):
    return (pltpu.bitcast(words << 16, F32),
            pltpu.bitcast(words & np.uint32(0xFFFF0000), F32))


def _pack(lo, hi):
    return pltpu.bitcast(pltpu.pack_elementwise([lo, hi], packed_dtype=BF16), U32)


def _words_shuffled(x):
    n, c = x.shape
    x = x.reshape(n // 16, 2, 8, c)
    return _pack(x[:, 0], x[:, 1]).reshape(n // 2, c)


def _recip(x):
    r = pl.reciprocal(x, approx=True)
    return r * (2.0 - x * r)


def _lhs_factors(a11, a12, a21, a22):
    return a11 + a22, a21 + a22, a11, a22, a11 + a12, a21 - a11, a12 - a22


def _rhs_factors(b11, b12, b21, b22):
    return b11 + b22, b11, b12 - b22, b21 - b11, b22, b11 + b12, b21 + b22


def _strassen(mul):
    m3 = mul(2)
    m4 = mul(3)
    m5 = mul(4)
    c12 = m3 + m5
    m2 = mul(1)
    c21 = m2 + m4
    m1 = mul(0)
    c11 = (m4 - m5) + m1 + mul(6)
    c22 = (m3 - m2) + m1 + mul(5)
    return c11, c12, c21, c22


def _factors_of_words(factors, *blocks):
    parts = [_halves(b) for b in blocks]
    plain = {id(lo): b for (lo, _), b in zip(parts, blocks)}
    return [plain.get(id(lo)) if id(lo) in plain else _pack(lo, hi)
            for lo, hi in zip(factors(*[x[0] for x in parts]), factors(*[x[1] for x in parts]))]


def _nested_factors(factors, blocks):
    inner = [factors(*[blocks[2 * r + ri][2 * c + ci] for r in range(2) for c in range(2)])
             for ri in range(2) for ci in range(2)]
    return [factors(*[x[j] for x in inner]) for j in range(7)]


def _nested_factors_of_words(factors, blocks):
    sides = [_nested_factors(factors, [[_halves(b)[side] for b in row] for row in blocks])
             for side in range(2)]
    return [[_pack(lo, hi) for lo, hi in zip(a, b)] for a, b in zip(*sides)]


def _nested_strassen(mul):
    blocks = _strassen(lambda j: jnp.concatenate(_strassen(lambda k: mul(j, k)), axis=0))
    for outer, val in enumerate(blocks):
        n = val.shape[0] // 4
        for inner in range(4):
            yield (2 * (outer // 2) + inner // 2, 2 * (outer % 2) + inner % 2,
                   val[inner * n:(inner + 1) * n])


def _permute_head_columns(words):
    tiles = [words[:, _cols(t)] for t in range(8)]
    lane = lax.broadcasted_iota(jnp.int32, tiles[0].shape, 1)
    for bit in (1, 2, 4):
        low = (lane & bit) == 0
        for t in range(8):
            if t & bit:
                continue
            a, b = tiles[t], tiles[t | bit]
            tiles[t] = jnp.where(low, a, pltpu.roll(b, bit, 1))
            tiles[t | bit] = jnp.where(low, pltpu.roll(a, 128 - bit, 1), b)
    src = ((lane & 3) << 5) | (lane >> 2)
    return jnp.concatenate([jnp.take_along_axis(x, src, axis=1) for x in tiles], axis=1)


def _with_corner(x, corner):
    top = corner if x.shape[1] == 128 else jnp.concatenate([corner, x[0:8, 128:]], axis=1)
    return jnp.concatenate([top, x[8:]], axis=0)


class _SideWork:
    def __init__(self):
        self.now = 0
        self.starts = {}
        self.stores = {}

    def add(self, tasks, steps, lag, width=1, phase=0.0):
        for n, task in enumerate(tasks):
            when = steps[int((n + phase) * len(steps)) // len(tasks)]
            self.starts.setdefault(when, []).append((task, lag, width))

    def step(self):
        for task, lag, width in self.starts.pop(self.now, []):
            stores = task()
            for n, store in enumerate(stores):
                self.stores.setdefault(self.now + lag + n * width // len(stores), []).append(store)
        for ref, idx, val in self.stores.pop(self.now, []):
            ref[idx] = val
        self.now += 1

    def check_done(self):
        assert not self.starts and not self.stores


def _mult(i, n):
    return i * n if isinstance(i, int) else pl.multiple_of(i * n, n)


def _wrap(i, n):
    return i % n if isinstance(i, int) else lax.rem(i, n)


def _cols(t):
    return slice(t * 128, (t + 1) * 128)


def _start(copies):
    for cp in copies:
        cp.start()


def _wait(copies):
    for cp in copies:
        cp.wait()


def _kernel(
    xa_hbm, c_hbm, wq_hbm, wk_hbm, wv_hbm, woa_hbm, xb_hbm, wqkv_hbm, wob_hbm,
    out_hbm,
    x_fac, wide, c, c_sum, kv_fac, k_buf, v_buf, ctx,
    wq_raw, wk_raw, wv_raw, woa_raw, wqkv_raw, wob_raw, kb, vb, obuf,
    sem_x, sem_w, sem_out,
):
    P = functools.partial
    xa32, c32, woa32, xb32, wqkv32 = (
        r.bitcast(U32) for r in (xa_hbm, c_hbm, woa_hbm, xb_hbm, wqkv_hbm))
    wq32, wk32, wv32, wob32 = (r.bitcast(U32) for r in (wq_hbm, wk_hbm, wv_hbm, wob_hbm))

    def pair_copies(src, dst, pair, ring, sem):
        slot = _wrap(pair, ring * PP)
        return [pltpu.make_async_copy(src.at[:, odd, pair, :], dst.at[slot, odd], sem)
                for odd in range(2)]

    def wq_copies(step):
        sem = sem_w.at[step & 3]
        return [cp for j in range(PP) for cp in pair_copies(wq32, wq_raw, step * PP + j, 2, sem)]

    def later_copies(part):
        sem, slot = sem_w.at[(part + 1) & 3], _wrap(part, RING)
        copies = []
        for j in range(PP):
            pair = part * PP + j
            copies += pair_copies(wk32, wk_raw, pair, RING, sem)
            copies += pair_copies(wv32, wv_raw, pair, RING, sem)
            copies.append(pltpu.make_async_copy(
                wob32.at[:, pair, :], wob_raw.at[_wrap(pair, RING * PP)], sem))
        copies.append(pltpu.make_async_copy(
            woa32.at[pl.ds(_mult(part, PP * D), PP * D)], woa_raw.at[slot], sem))
        for h in range(2):
            copies.append(pltpu.make_async_copy(
                wqkv32.at[h, pl.ds(_mult(part, PP * 16), PP * 16)],
                wqkv_raw.at[slot, h, 0:PP * 16], sem))
            rows = (2 * (part >> 1) + h, pl.ds(_mult(part & 1, G // 8), G // 8))
            copies.append(pltpu.make_async_copy(c32.at[rows], c.at[rows], sem))
        return copies

    def x_copy(g):
        return pltpu.make_async_copy(xa32.at[g * G // 2:(g + 1) * G // 2],
                                     woa_raw.at[(g + 2) % RING], sem_x.at[g])

    xb_copies = [pltpu.make_async_copy(
        xb32.at[r * S // 8:(r + 1) * S // 8, k * M // 4:(k + 1) * M // 4],
        x_fac.at[4 * r + k], sem_x.at[0]) for r in range(4) for k in range(4)]

    gw = G // 4
    sum_index = {0: 0, 1: 1, 4: 2, 5: 3, 6: 4}

    def head_factors(raw, slot, top, bottom, n):
        sides = [_rhs_factors(*_halves(raw[slot, odd, top:top + n, :]),
                              *_halves(raw[slot, odd, bottom:bottom + n, :]))
                 for odd in range(2)]
        return [_pack(even, odd) for even, odd in zip(*sides)]

    def group_blocks(g, mul):
        for n, val in enumerate(_strassen(mul)):
            r, e = divmod(n, 2)
            yield e, slice((2 * g + r) * gw, (2 * g + r + 1) * gw), val

    def project_kv(n, pair, g):
        def lhs(j):
            if j in sum_index:
                return c_sum[sum_index[j], g * gw:(g + 1) * gw, :]
            return c[2 * g + j - 2, :, (j - 2) * DC // 2:(j - 1) * DC // 2]

        for e, rows, val in group_blocks(g, lambda j: _dot(_bf(lhs(j)), _bf(kv_fac[pair, n, j]))):
            val = _words_shuffled(val)
            (k_buf, v_buf)[n][e, rows, :] = val
            if n == 0 and rows.start == 0:
                ctx[H + e, 0:BQ // 2, :] = val[0:BQ // 2]

    def prepare_kv(n, pair, piece):
        vals = head_factors((wk_raw, wv_raw)[n], _wrap(pair, RING * PP),
                            piece * 16, DC // 4 + piece * 16, 16)
        return [(kv_fac, (pair, n, j, slice(piece * 16, (piece + 1) * 16)), val)
                for j, val in enumerate(vals)]

    def prepare_c(part, piece):
        r = _mult(part & 1, G // 8) + 16 * piece
        vals = _factors_of_words(_lhs_factors, *[
            c[2 * (part >> 1) + h, pl.ds(r, 16), k * DC // 2:(k + 1) * DC // 2]
            for h in range(2) for k in range(2)])
        return [(c_sum, (n, pl.ds(_mult(part >> 1, gw) + r, 16)), vals[j])
                for j, n in sum_index.items()]

    def prepare_wqkv(part, piece, which):
        both = _permute_head_columns(jnp.concatenate([
            wqkv_raw[_wrap(part, RING), h, 8 * piece:8 * piece + 8, which * M:(which + 1) * M]
            for h in range(2)], axis=0))
        vals = _factors_of_words(
            _rhs_factors, both[:8, :W], both[:8, W:], both[8:, :W], both[8:, W:])
        r = _mult(part, PP * 16) + 8 * piece
        return [(wide, (QKV0 + 7 * which + j, pl.ds(r, 8)), val) for j, val in enumerate(vals)]

    def prepare_wob(pair, t):
        b11, b21 = _halves(wob_raw[_wrap(pair, RING * PP), :, _cols(t)])
        b12, b22 = _halves(wob_raw[_wrap(pair, RING * PP), :, _cols(4 + t)])
        r = _mult((pair & 3) * 4 + (pair >> 2), HB // 2)
        return [(wide, (OB0 + j, pl.ds(r, HB // 2), _cols(t)), _words(val))
                for j, val in enumerate(_rhs_factors(b11, b12, b21, b22))]

    def prepare_woa(part, t, n):
        fac = _nested_factors_of_words(_rhs_factors, [
            [woa_raw[_wrap(part, RING), hq * D // 2 + 8 * n:hq * D // 2 + 8 * n + 8, _cols(2 * k + t)]
             for k in range(4)] for hq in range(4)])
        order = (1, 5, 4, 2, 0, 6, 3)
        rows = pl.ds(_mult(part & 3, D // 2) + 8 * n, 8)
        cols = pl.ds(_mult(2 * t + (part >> 2), 128), 128)
        return [(wide, (OA0 + 7 * j + k, rows, cols), fac[j][k]) for j in order for k in order]

    def later_tasks(parts):
        quads = [(part, j, part * PP + j) for part in parts for j in range(PP)]
        return (
            [P(prepare_woa, part, j, n) for part, j, _ in quads for n in range(8)],
            [P(prepare_wqkv, part, 2 * j + n // 3, n % 3) for part, j, _ in quads for n in range(6)],
            [P(prepare_kv, n % 2, pair, n // 2) for _, _, pair in quads for n in range(16)],
            [task for part, j, pair in quads for n in range(2) for task in (
                P(prepare_wob, pair, 2 * n), P(prepare_c, part, 2 * j + n),
                P(prepare_wob, pair, 2 * n + 1))])

    qw0 = G // 8

    def gate(g, j, k):
        n = 7 * j + k
        return GATE + n // 32, slice(n % 32 * 8, n % 32 * 8 + 8), _cols(g)

    def make_x_factors(g):
        fac = _nested_factors_of_words(_lhs_factors, [
            [woa_raw[(g + 2) % RING, r * qw0:(r + 1) * qw0, k * M // 4:(k + 1) * M // 4]
             for k in range(4)] for r in range(4)])
        for j in range(7):
            for k in range(7):
                x_fac[7 * j + k, g * qw0:(g + 1) * qw0] = fac[j][k]
                if g % (NG // SPLIT) == 0:
                    wide[gate(g, j, k)] = fac[j][k][0:8, 0:128]
        return fac

    def wq_factors(step):
        n = M // 8
        sides = [_nested_factors(_rhs_factors, [
            [half for j in range(PP) for half in _halves(
                wq_raw[(step * PP + j) & (2 * PP - 1), odd, k * n:(k + 1) * n, :])]
            for k in range(4)]) for odd in range(2)]
        return [[_pack(even, odd) for even, odd in zip(a, b)] for a, b in zip(*sides)]

    def store_q(step, g, r, head, val):
        ctx[4 * step + head, (4 * g + r) * qw0:(4 * g + r + 1) * qw0, :] = _words(
            val * (D ** -0.5 * LOG2E))

    _start(wq_copies(0) + [x_copy(g) for g in range(RING)])
    kb[:, RC:RC + HALO, :] = jnp.zeros((8, HALO, 128), F32)
    vb[:, RC:RC + HALO, :] = jnp.zeros((8, HALO, 128), F32)
    _wait(wq_copies(0))

    def kept(j, k):
        return (NP - 1 - j // 2, j % 2, k)

    for j, row in enumerate(wq_factors(0)):
        for k, val in enumerate(row):
            kv_fac[kept(j, k)] = val
    for g in range(NG):
        x_copy(g).wait()
        if g == 1:
            _start([x_copy(3)] + wq_copies(1))
        elif g > 1:
            _start(later_copies(g - 2))
        lhs = make_x_factors(g)
        for r, head, val in _nested_strassen(
                lambda j, k: _dot(_bf(lhs[j][k]), _bf(kv_fac[kept(j, k)]))):
            store_q(0, g, r, head, val)

    def q_step(step, parts, zero, first, last, *pace):
        side = _SideWork()
        for tasks, (lag, width, phase) in zip(later_tasks(parts), pace):
            side.add(tasks, range(first, min(last, 49 * SPLIT - lag - width + 1)), lag, width, phase)
        fac = wq_factors(step)

        def mul_rows(j, k, n):
            side.step()
            lhs = x_fac[7 * j + k, n * S // 8 // SPLIT:(n + 1) * S // 8 // SPLIT]
            val = _dot(_bf(_with_corner(lhs, wide[gate(n * NG // SPLIT, j, k)])), _bf(fac[j][k]))
            token = pltpu.bitcast(val[0:8], U32)
            wqkv_raw[zero, 0, PP * 16:PP * 16 + 8, _cols(0)] = token
            wk_raw[RING * PP + zero, 0, 0:8] = token
            wv_raw[RING * PP + zero, 0, 0:8] = token
            c[2 * NG + zero, 0:8, _cols(0)] = token
            return val

        for r, head, val in _nested_strassen(lambda j, k: jnp.concatenate(
                [mul_rows(j, k, n) for n in range(SPLIT)], axis=0)):
            for g in range(NG):
                store_q(step, g, r, head, val[g * G // 4:(g + 1) * G // 4])
        side.check_done()

    def q_body(step, zero):
        _start(wq_copies(step + 1) + later_copies(step + 1))
        _wait(wq_copies(step) + later_copies(step - 1))
        q_step(step, [step - 1], zero, *PACE0)
        return -zero

    zero = lax.fori_loop(1, NS - 1, q_body, 0)
    _wait(wq_copies(NS - 1) + later_copies(NS - 2) + later_copies(NS - 1))
    q_step(NS - 1, [zero + NS - 2, zero + NS - 1], zero, *PACE1)
    project_kv(0, 0, 0)
    _start(xb_copies)

    def pair_body(p, zero):
        row = lax.broadcasted_iota(jnp.int32, (BQ, BQ), 0)
        col = lax.broadcasted_iota(jnp.int32, (BQ, BQ), 1)
        causal = ((col & ~15) | ((col & 15) >> 1) | ((col & 1) << 3)) <= row
        hb = BQ // 2

        def scores(e, i):
            r = i * BQ
            k = ctx[H + e + zero, 0:hb, :]
            k = _bf(jnp.concatenate([k, k_buf[e, hb:(i + 1) * hb, :]], axis=0) if i else k)
            q = _bf(ctx[2 * p + e, i * hb:(i + 1) * hb, :])
            s = lax.dot_general(q, k, _NT, preferred_element_type=F32)
            diag = jnp.where(causal, s[:, r:], NEG)
            s = jnp.concatenate([s[:, :r], diag], axis=1) if r else diag
            return s, jnp.max(s, axis=1, keepdims=True)

        def context(e, i, s, peak):
            w = jnp.exp2(s - peak)
            total = jnp.sum(w, axis=1, keepdims=True)
            o = _dot(w.astype(BF16), _bf(v_buf[e, 0:(i + 1) * hb, :]))
            return _words(o * _recip(total))

        state = {}
        for op in _attention_order():
            if op[0] in "kv":
                pair = jnp.minimum(p + 1, NP - 1) if op == "k0" else p
                project_kv("kv".index(op[0]), pair, int(op[1:]))
                continue
            e, i = "ab".index(op[1]), int(op[2:])
            if op[0] == "S":
                state[e, i] = scores(e, i)
            elif op[0] == "P":
                state[e, i] = context(e, i, *state[e, i])
            else:
                ctx[2 * p + e, i * hb:(i + 1) * hb, :] = state.pop((e, i))
        assert not state
        return -zero

    lax.fori_loop(0, NP, pair_body, 0)
    _wait(xb_copies)

    n_chunks = S // RC
    hr = RC // 2
    qw = RC // 8

    def out_copy(i, slot):
        return pltpu.make_async_copy(
            obuf.at[slot], out_hbm.at[pl.ds(_mult(i, RC), RC), :], sem_out.at[slot])

    def last_copy(n):
        lo, hi = ((0, M), (M, M + 256), (M + W, M + W + 256), (M + 256, M + W), (M + W + 256, 2 * M))[n]
        return pltpu.make_async_copy(
            obuf.at[1, :, lo:hi], out_hbm.at[S - RC:S, lo:hi], sem_out.at[1])

    def chunk_body(i, zero, last=False):
        slot = i & 1
        base = _mult(i, RC // 2)

        @pl.when(i >= 2)
        def _():
            out_copy(i - 2, slot).wait()

        def is_plain(j, k):
            return j in (2, 3) and k in (2, 3)

        def ctx_at(j, k, u, lo, n):
            if is_plain(j, k):
                quarter = 2 * (j - 2) + k - 2
                return ctx, (4 * u + quarter, pl.ds(base + quarter * qw + lo, n))
            slab, r = divmod((2 * (7 * j + k) + u // 4) * qw + lo, SLAB)
            return wide, (CS0 + slab, slice(r, r + n), _cols(u % 4))

        ctx_fac = {}

        def ctx_factor_store(u, lo, j, k):
            if (u, lo) not in ctx_fac:
                ctx_fac[u, lo] = _nested_factors_of_words(_lhs_factors, [
                    [ctx[4 * u + hq, pl.ds(base + r * qw + lo, 8)] for hq in range(4)]
                    for r in range(4)])
            return [ctx_at(j, k, u, lo, 8) + (ctx_fac[u, lo][j][k],)]

        def taps(buf, t, w, r):
            return buf[t, HALO - DIL * w + r:HALO - DIL * w + r + 8, :]

        def tile_at(n, r, rows):
            return n // 4, slice(n % 4 * RC + r, n % 4 * RC + r + rows)

        q_alias = v_buf.at[pl.ds(zero, 2)]
        logit_alias = k_buf.at[pl.ds(zero, 2)]

        def window_logits(r, ws):
            q = [pltpu.bitcast(q_alias[tile_at(t, r, 8)], F32) for t in range(8)]
            logits = [functools.reduce(jnp.add, [q[t] * taps(kb, t, w, r) for t in range(8)])
                      for w in ws]
            logits = [z + pltpu.roll(z, 64, 1) for z in logits]
            logits = [(z + pltpu.roll(z, 32, 1)) * (DB ** -0.5 * LOG2E) for z in logits]
            pos = i * RC + r + lax.broadcasted_iota(jnp.int32, (8, 128), 0)
            return [(k_buf, tile_at(w, r, 8), pltpu.bitcast(
                jnp.where(pos >= DIL * w, z, NEG) if DIL * w > r else z, U32))
                for w, z in zip(ws, logits)]

        weights = {}

        def window_softmax(r):
            logits = [pltpu.bitcast(logit_alias[tile_at(w, r, 8)], F32) for w in range(WIN)]
            peak = functools.reduce(jnp.maximum, logits)
            probs = [jnp.exp2(z - peak) for z in logits]
            inv = _recip(functools.reduce(jnp.add, probs))
            weights[r] = [z * inv for z in probs]
            return []

        def window_values(r, ts):
            return [(wide, (LOC0 + r // hr, slice(r % hr + (t % 2) * hr, r % hr + (t % 2) * hr + 8),
                            _cols(t // 2)),
                     pltpu.bitcast(functools.reduce(
                         jnp.add, [weights[r][w] * taps(vb, t, w, r) for w in range(WIN)]), U32))
                    for t in ts]

        n_steps = 3 * 4 * 7 + 2 * 49
        order = (2, 4, 3, 1, 0, 6, 5)
        side = _SideWork()
        side.add([P(ctx_factor_store, u, lo, j, k) for u in range(8) for lo in range(0, qw, 8)
                  for j in order for k in order if not is_plain(j, k)], range(CTX_FIRST, CTX_LAST), 0)
        side.add([P(window_logits, r, ws) for r in range(0, RC, 8)
                  for ws in ((0, 4, 1, 5), (2, 6, 3, 7))],
                 range(LOGIT_FIRST, LOGIT_LAST - LOGIT_LAG), LOGIT_LAG)
        side.add([P(window_softmax, r) for r in range(0, RC, 8)],
                 range(VALUE_FIRST, n_steps - 2), 0)
        side.add([P(window_values, r, ts) for r in range(0, RC, 8)
                  for ts in (range(4), range(4, 8))], range(VALUE_FIRST + 2, n_steps), 0)
        wide_alias = wide.at[pl.ds(zero, CS0)]

        def mul(lhs, slab, *tiles):
            side.step()
            rhs = jnp.concatenate([wide[slab, :, _cols(t)] for t in tiles], axis=0)
            rhs = _with_corner(rhs, wide_alias[slab, 0:8, _cols(tiles[0])])
            val = _dot(_bf(lhs), _bf(rhs))
            for buf in (k_buf, v_buf):
                buf[0, S // 2:S // 2 + 8, :] = pltpu.bitcast(val[0:8], U32)
            return val

        xb_fac = _factors_of_words(_lhs_factors, *[
            jnp.concatenate([
                x_fac[4 * (i >> 1) + 2 * k + t, pl.ds(_mult(2 * (i & 1) + r, hr // 2), hr // 2)]
                for t in range(2)], axis=1) for r in range(2) for k in range(2)])
        for part, buf in ((1, kb), (0, None), (2, vb)):
            if part:
                buf[:, 0:HALO, :] = buf[:, RC:RC + HALO, :]
            for t in range(4):
                blocks = _strassen(lambda j: mul(xb_fac[j], QKV0 + 7 * part + j, t))
                for n, val in enumerate(blocks):
                    r, k = divmod(n, 2)
                    if part:
                        buf[4 * k + t, HALO + r * hr:HALO + (r + 1) * hr, :] = val
                    else:
                        v_buf[tile_at(4 * k + t, r * hr, hr)] = pltpu.bitcast(val, U32)

        def ctx_factor(j, k):
            return jnp.concatenate(
                [ref[idx] for ref, idx in (ctx_at(j, k, u, 0, qw) for u in range(8))], axis=1)

        for t in range(2):
            for r, k, val in _nested_strassen(
                    lambda j, k: mul(ctx_factor(j, k), OA0 + 7 * j + k, 2 * t, 2 * t + 1)):
                obuf[slot, r * RC // 4:(r + 1) * RC // 4, _cols(2 * k + t)] = val.astype(BF16)
        side.check_done()
        if last:
            last_copy(0).start()

        o_fac = [z.astype(BF16) for z in _lhs_factors(*[
            pltpu.bitcast(wide[LOC0 + r, e * hr:(e + 1) * hr, :], F32)
            for r in range(2) for e in range(2)])]
        for t in range(4):
            blocks = _strassen(lambda j: _dot(o_fac[j], _bf(wide[OB0 + j, :, _cols(t)])))
            for n, val in enumerate(blocks):
                r, k = divmod(n, 2)
                obuf[slot, r * hr:(r + 1) * hr, _cols(8 + 4 * k + t)] = val.astype(BF16)
            if last and t == 1:
                _start([last_copy(1), last_copy(2)])

        if last:
            _start([last_copy(n) for n in range(3, 5)])
        else:
            out_copy(i, slot).start()
        return -zero

    zero = lax.fori_loop(0, n_chunks - 1, chunk_body, 0)
    chunk_body(n_chunks - 1, zero, last=True)
    out_copy(n_chunks - 2, 0).wait()
    _wait([last_copy(n) for n in range(5)])


@jax.jit
def pallas_concat_heads__compressed_kv_cla__sliding_local_dilated__prompt_kernel(
    A_x: jax.Array,
    A_c_kv: jax.Array,
    A_w_q: jax.Array,
    A_w_uk: jax.Array,
    A_w_uv: jax.Array,
    A_w_o: jax.Array,
    B_x: jax.Array,
    B_wqkv: jax.Array,
    B_wo: jax.Array,
):
    window_buf = pltpu.VMEM((8, HALO + RC + 8, 128), F32)
    scratch = [
        pltpu.VMEM((49, S // 8, M // 4), U32),
        pltpu.VMEM((N_SLABS, SLAB, W), U32),
        pltpu.VMEM((2 * NG + 1, G // 4, DC), U32),
        pltpu.VMEM((5, S // 4, DC // 2), U32),
        pltpu.VMEM((NP, 2, 7, DC // 4, D), U32),
        pltpu.VMEM((2, S // 2 + 8, D), U32),
        pltpu.VMEM((2, S // 2 + 8, D), U32),
        pltpu.VMEM((H + 2, S // 2, D), U32),
        pltpu.VMEM((2 * PP, 2, M // 2, D), U32),
        pltpu.VMEM((RING * PP + 1, 2, DC // 2, D), U32),
        pltpu.VMEM((RING * PP + 1, 2, DC // 2, D), U32),
        pltpu.VMEM((RING, PP * D, M), U32),
        pltpu.VMEM((RING, 2, PP * 16 + 8, 3 * M), U32),
        pltpu.VMEM((RING * PP, HB, M), U32),
        window_buf,
        window_buf,
        pltpu.VMEM((2, RC, 2 * M), BF16),
        pltpu.SemaphoreType.DMA((NG,)),
        pltpu.SemaphoreType.DMA((4,)),
        pltpu.SemaphoreType.DMA((2,)),
    ]
    out = pl.pallas_call(
        _kernel,
        out_shape=jax.ShapeDtypeStruct((S, 2 * M), BF16),
        in_specs=[pl.BlockSpec(memory_space=pl.ANY)] * 9,
        out_specs=pl.BlockSpec(memory_space=pl.ANY),
        scratch_shapes=scratch,
        compiler_params=pltpu.CompilerParams(
            vmem_limit_bytes=127 * 2**20, disable_bounds_checks=True),
        name="fused_mla_sliding",
    )(
        A_x.reshape(S, M),
        A_c_kv.reshape(2 * NG, G // 2, DC),
        A_w_q.reshape(M // 2, 2, H, D),
        A_w_uk.reshape(DC // 2, 2, H, D),
        A_w_uv.reshape(DC // 2, 2, H, D),
        A_w_o.reshape(H * D, M),
        B_x.reshape(S, M),
        B_wqkv.reshape(2, M // 2, 3 * M),
        B_wo.reshape(HB, DB, M),
    )
    return out.reshape(1, S, 2 * M)
```

```python
import functools

import jax
import jax.numpy as jnp
import numpy as np
from jax import lax
import jax.experimental.pallas as pl
import jax.experimental.pallas.tpu as pltpu

S = 2048
M = 1024
DC = 512
H = 32
D = 128
HB = 32
DB = 32
WIN = 8
DIL = 2

NP = H // 2
PP = 2
NS = NP // PP
RING = 3
G = 512
NG = S // G
BQ = 128
RC = 256
HALO = 16
KV_ROWS = HALO + RC + 8
LOG2E = 1.4426950408889634
NEG = -1e9 * LOG2E

W = M // 2
SLAB = M // 4
OA0 = 0
QKV0 = OA0 + 49
OB0 = QKV0 + 21
CS0 = OB0 + 7
LOC0 = CS0 + 13
GATE = CS0
N_SLABS = LOC0 + 2

SPLIT = 2
PACE2 = (0, 28, 0, 4)
PACE0 = (0, 88, (7, 1, 0.5), (0, 2, 0.5), (0, 2, 0))
PACE1 = (2, 88, (7, 1, 0.5), (0, 2, 0.5), (0, 1, 0))
CTX_FIRST = 5
CTX_LAST = 85
LOGIT_FIRST = 84
LOGIT_LAST = 174
LOGIT_LAG = 6
VALUE_FIRST = 98

F32 = jnp.float32
BF16 = jnp.bfloat16
U32 = jnp.uint32
_NT = (((1,), (1,)), ((), ()))


def _attention_order():
    ops = ("Sa0 Sa1 Sa2 Sa3 v0 k1 Pa0 Pa1 Pa2 v1 Sa4 Pa3 k2 Sa5 Wa0 Wa1 Pa4 v2 "
           "Sa6 Wa2 Pa5 Wa3 k3 Sa7 Pa6 Wa4 v3").split()
    for i in range(8, 16):
        ops += [f"Sa{i}", f"Pa{i - 1}", f"Wa{i - 3}"]
    ops += "Sb15 Pa15 Wa13 Sb14 Pb15 Wa14 Sb13 Pb14 Wa15".split()
    for i in range(12, 3, -1):
        ops += [f"Sb{i}", f"Pb{i + 1}", f"Wb{i + 3}"]
    return ops + "Sb3 Sb2 Pb4 Wb6 Sb1 Sb0 Pb3 Pb2 k0 Pb1 Pb0 Wb5 Wb4 Wb3 Wb2 Wb1 Wb0".split()


def _dot(a, b):
    return jnp.dot(a, b, preferred_element_type=F32)


def _bf(words):
    return pltpu.bitcast(words, BF16)


def _words(x):
    return pltpu.bitcast(x.astype(BF16), U32)


def _halves(words):
    return (pltpu.bitcast(words << 16, F32),
            pltpu.bitcast(words & np.uint32(0xFFFF0000), F32))


def _pack(lo, hi):
    return pltpu.bitcast(pltpu.pack_elementwise([lo, hi], packed_dtype=BF16), U32)


def _words_shuffled(x):
    n, c = x.shape
    x = x.reshape(n // 16, 2, 8, c)
    return _pack(x[:, 0], x[:, 1]).reshape(n // 2, c)


def _recip(x):
    r = pl.reciprocal(x, approx=True)
    return r * (2.0 - x * r)


def _lhs_factors(a11, a12, a21, a22):
    return a11 + a22, a21 + a22, a11, a22, a11 + a12, a21 - a11, a12 - a22


def _rhs_factors(b11, b12, b21, b22):
    return b11 + b22, b11, b12 - b22, b21 - b11, b22, b11 + b12, b21 + b22


def _strassen(mul):
    m3 = mul(2)
    m4 = mul(3)
    m5 = mul(4)
    c12 = m3 + m5
    m2 = mul(1)
    c21 = m2 + m4
    m1 = mul(0)
    c11 = (m4 - m5) + m1 + mul(6)
    c22 = (m3 - m2) + m1 + mul(5)
    return c11, c12, c21, c22


def _factors_of_words(factors, *blocks):
    parts = [_halves(b) for b in blocks]
    plain = {id(lo): b for (lo, _), b in zip(parts, blocks)}
    return [plain.get(id(lo)) if id(lo) in plain else _pack(lo, hi)
            for lo, hi in zip(factors(*[x[0] for x in parts]), factors(*[x[1] for x in parts]))]


def _nested_factors(factors, blocks):
    inner = [factors(*[blocks[2 * r + ri][2 * c + ci] for r in range(2) for c in range(2)])
             for ri in range(2) for ci in range(2)]
    return [factors(*[x[j] for x in inner]) for j in range(7)]


def _nested_factors_of_words(factors, blocks):
    sides = [_nested_factors(factors, [[_halves(b)[side] for b in row] for row in blocks])
             for side in range(2)]
    return [[_pack(lo, hi) for lo, hi in zip(a, b)] for a, b in zip(*sides)]


def _nested_strassen(mul):
    blocks = _strassen(lambda j: jnp.concatenate(_strassen(lambda k: mul(j, k)), axis=0))
    for outer, val in enumerate(blocks):
        n = val.shape[0] // 4
        for inner in range(4):
            yield (2 * (outer // 2) + inner // 2, 2 * (outer % 2) + inner % 2,
                   val[inner * n:(inner + 1) * n])


def _permute_head_columns(words):
    tiles = [words[:, _cols(t)] for t in range(8)]
    lane = lax.broadcasted_iota(jnp.int32, tiles[0].shape, 1)
    for bit in (1, 2, 4):
        low = (lane & bit) == 0
        for t in range(8):
            if t & bit:
                continue
            a, b = tiles[t], tiles[t | bit]
            tiles[t] = jnp.where(low, a, pltpu.roll(b, bit, 1))
            tiles[t | bit] = jnp.where(low, pltpu.roll(a, 128 - bit, 1), b)
    src = ((lane & 3) << 5) | (lane >> 2)
    return jnp.concatenate([jnp.take_along_axis(x, src, axis=1) for x in tiles], axis=1)


def _with_corner(x, corner):
    top = corner if x.shape[1] == 128 else jnp.concatenate([corner, x[0:8, 128:]], axis=1)
    return jnp.concatenate([top, x[8:]], axis=0)


class _SideWork:
    def __init__(self):
        self.now = 0
        self.starts = {}
        self.stores = {}

    def add(self, tasks, steps, lag, width=1, phase=0.0):
        for n, task in enumerate(tasks):
            when = steps[int((n + phase) * len(steps)) // len(tasks)]
            self.starts.setdefault(when, []).append((task, lag, width))

    def step(self):
        for task, lag, width in self.starts.pop(self.now, []):
            stores = task()
            for n, store in enumerate(stores):
                self.stores.setdefault(self.now + lag + n * width // len(stores), []).append(store)
        for ref, idx, val in self.stores.pop(self.now, []):
            ref[idx] = val
        self.now += 1

    def check_done(self):
        assert not self.starts and not self.stores


def _mult(i, n):
    return i * n if isinstance(i, int) else pl.multiple_of(i * n, n)


def _wrap(i, n):
    return i % n if isinstance(i, int) else lax.rem(i, n)


def _cols(t):
    return slice(t * 128, (t + 1) * 128)


def _start(copies):
    for cp in copies:
        cp.start()


def _wait(copies):
    for cp in copies:
        cp.wait()


def _kernel(
    xa_hbm, c_hbm, wq_hbm, wk_hbm, wv_hbm, woa_hbm, xb_hbm, wqkv_hbm, wob_hbm,
    out_hbm,
    x_fac, wide, c, c_sum, kv_fac, k_buf, v_buf, ctx,
    wq_raw, wk_raw, wv_raw, woa_raw, wqkv_raw, wob_raw, obuf,
    sem_x, sem_w, sem_out,
):
    P = functools.partial
    xa32, c32, woa32, xb32, wqkv32 = (
        r.bitcast(U32) for r in (xa_hbm, c_hbm, woa_hbm, xb_hbm, wqkv_hbm))
    wq32, wk32, wv32, wob32 = (r.bitcast(U32) for r in (wq_hbm, wk_hbm, wv_hbm, wob_hbm))

    def pair_copies(src, dst, pair, ring, sem):
        slot = _wrap(pair, ring * PP)
        return [pltpu.make_async_copy(
            src.at[:, odd, pair, :], dst.at[slot, odd, 0:src.shape[0]], sem) for odd in range(2)]

    def wq_copies(step):
        sem = sem_w.at[step & 3]
        return [cp for j in range(PP) for cp in pair_copies(wq32, wq_raw, step * PP + j, 2, sem)]

    def later_copies(part):
        sem, slot = sem_w.at[(part + 1) & 3], _wrap(part, RING)
        copies = []
        for j in range(PP):
            pair = part * PP + j
            copies += pair_copies(wk32, wk_raw, pair, RING, sem)
            copies += pair_copies(wv32, wv_raw, pair, RING, sem)
            copies.append(pltpu.make_async_copy(
                wob32.at[:, pair, :], wob_raw.at[_wrap(pair, RING * PP)], sem))
        for h in range(2):
            copies.append(pltpu.make_async_copy(
                wqkv32.at[h, pl.ds(_mult(part, PP * 16), PP * 16)],
                wqkv_raw.at[slot, h, 0:PP * 16], sem))
            rows = (2 * (part >> 1) + h, pl.ds(_mult(part & 1, G // 8), G // 8))
            copies.append(pltpu.make_async_copy(c32.at[rows], c.at[rows], sem))
        return copies

    def woa_copy(part):
        return pltpu.make_async_copy(woa32.at[pl.ds(_mult(part, PP * D), PP * D)],
                                     woa_raw.at[part & 1], sem_w.at[part & 1])

    def x_copy(g):
        return pltpu.make_async_copy(xa32.at[g * G // 2:(g + 1) * G // 2],
                                     woa_raw.at[g], sem_x.at[g])

    xb_copies = [pltpu.make_async_copy(
        xb32.at[r * S // 8:(r + 1) * S // 8, k * M // 4:(k + 1) * M // 4],
        x_fac.at[4 * r + k], sem_x.at[0]) for r in range(4) for k in range(4)]

    gw = G // 4
    sum_index = {0: 0, 1: 1, 4: 2, 5: 3, 6: 4}

    def head_factors(raw, slot, top, bottom, n):
        sides = [_rhs_factors(*_halves(raw[slot, odd, top:top + n, :]),
                              *_halves(raw[slot, odd, bottom:bottom + n, :]))
                 for odd in range(2)]
        return [_pack(even, odd) for even, odd in zip(*sides)]

    def group_blocks(g, mul):
        for n, val in enumerate(_strassen(mul)):
            r, e = divmod(n, 2)
            yield e, slice((2 * g + r) * gw, (2 * g + r + 1) * gw), val

    def c_factor(g, j):
        if j in sum_index:
            return c_sum[sum_index[j], g * gw:(g + 1) * gw, :]
        return c[2 * g + j - 2, :, (j - 2) * DC // 2:(j - 1) * DC // 2]

    def c_gate(g, j):
        return GATE + 2, slice(8 * (7 * g + j), 8 * (7 * g + j + 1)), _cols(0)

    def project_kv(n, pair, g, side=None):
        def mul(j):
            lhs = c_factor(g, j)
            if side:
                side.step()
                lhs = _with_corner(lhs, wide[c_gate(g, j)])
            return _dot(_bf(lhs), _bf(kv_fac[pair, n, j]))

        for e, rows, val in group_blocks(g, mul):
            val = _words_shuffled(val)
            (k_buf, v_buf)[n][e, rows, :] = val
            if n == 0 and rows.start == 0:
                ctx[H + e, 0:BQ // 2, :] = val[0:BQ // 2]

    def prepare_kv(n, pair, piece):
        vals = head_factors((wk_raw, wv_raw)[n], _wrap(pair, RING * PP),
                            piece * 16, DC // 4 + piece * 16, 16)
        return [(kv_fac, (pair, n, j, slice(piece * 16, (piece + 1) * 16)), val)
                for j, val in enumerate(vals)]

    def prepare_c(part, piece):
        r = _mult(part & 1, G // 8) + 16 * piece
        vals = _factors_of_words(_lhs_factors, *[
            c[2 * (part >> 1) + h, pl.ds(r, 16), k * DC // 2:(k + 1) * DC // 2]
            for h in range(2) for k in range(2)])
        return [(c_sum, (n, pl.ds(_mult(part >> 1, gw) + r, 16)), vals[j])
                for j, n in sum_index.items()]

    def prepare_wqkv(part, piece, which):
        both = _permute_head_columns(jnp.concatenate([
            wqkv_raw[_wrap(part, RING), h, 8 * piece:8 * piece + 8, which * M:(which + 1) * M]
            for h in range(2)], axis=0))
        vals = _factors_of_words(
            _rhs_factors, both[:8, :W], both[:8, W:], both[8:, :W], both[8:, W:])
        r = _mult(part, PP * 16) + 8 * piece
        return [(wide, (QKV0 + 7 * which + j, pl.ds(r, 8)), val) for j, val in enumerate(vals)]

    def prepare_wob(pair, t):
        b11, b21 = _halves(wob_raw[_wrap(pair, RING * PP), :, _cols(t)])
        b12, b22 = _halves(wob_raw[_wrap(pair, RING * PP), :, _cols(4 + t)])
        r = _mult((pair & 3) * 4 + (pair >> 2), HB // 2)
        return [(wide, (OB0 + j, pl.ds(r, HB // 2), _cols(t)), _words(val))
                for j, val in enumerate(_rhs_factors(b11, b12, b21, b22))]

    def prepare_woa(part, t, n):
        fac = _nested_factors_of_words(_rhs_factors, [
            [woa_raw[part & 1, hq * D // 2 + 8 * n:hq * D // 2 + 8 * n + 8,
                     pl.ds(_mult(2 * k + t, 128), 128)]
             for k in range(4)] for hq in range(4)])
        order = (1, 5, 4, 2, 0, 6, 3)
        rows = pl.ds(_mult(part & 3, D // 2) + 8 * n, 8)
        cols = pl.ds(_mult(2 * t + (part >> 2), 128), 128)
        return [(wide, (OA0 + 7 * j + k, rows, cols), fac[j][k]) for j in order for k in order]

    def later_tasks(parts):
        quads = [(part, j, part * PP + j) for part in parts for j in range(PP)]
        return (
            [P(prepare_wqkv, part, 2 * j + n // 3, n % 3) for part, j, _ in quads for n in range(6)],
            [P(prepare_kv, n % 2, pair, n // 2) for _, _, pair in quads for n in range(16)],
            [task for part, j, pair in quads for n in range(2) for task in (
                P(prepare_wob, pair, 2 * n), P(prepare_c, part, 2 * j + n),
                P(prepare_wob, pair, 2 * n + 1))])

    qw0 = G // 8

    def gate(g, j, k):
        n = 7 * j + k
        return GATE + n // 32, slice(n % 32 * 8, n % 32 * 8 + 8), _cols(g)

    def make_x_factors(g):
        fac = _nested_factors_of_words(_lhs_factors, [
            [woa_raw[g, r * qw0:(r + 1) * qw0, k * M // 4:(k + 1) * M // 4]
             for k in range(4)] for r in range(4)])
        for j in range(7):
            for k in range(7):
                x_fac[7 * j + k, g * qw0:(g + 1) * qw0] = fac[j][k]
                if g % (NG // SPLIT) == 0:
                    wide[gate(g, j, k)] = fac[j][k][0:8, 0:128]
        return fac

    def wq_factors(step):
        n = M // 8
        sides = [_nested_factors(_rhs_factors, [
            [half for j in range(PP) for half in _halves(
                wq_raw[(step * PP + j) & (2 * PP - 1), odd, k * n:(k + 1) * n, :])]
            for k in range(4)]) for odd in range(2)]
        return [[_pack(even, odd) for even, odd in zip(a, b)] for a, b in zip(*sides)]

    def store_q(step, g, r, head, val):
        ctx[4 * step + head, (4 * g + r) * qw0:(4 * g + r + 1) * qw0, :] = _words(
            val * (D ** -0.5 * LOG2E))

    _start(wq_copies(0) + [x_copy(g) for g in range(NG)]
           + wq_copies(1) + later_copies(0) + later_copies(1))
    _wait(wq_copies(0))

    def kept(j, k):
        return (NP - 1 - j // 2, j % 2, k)

    for j, row in enumerate(wq_factors(0)):
        for k, val in enumerate(row):
            kv_fac[kept(j, k)] = val
    for g in range(NG):
        x_copy(g).wait()
        lhs = make_x_factors(g)
        for r, head, val in _nested_strassen(
                lambda j, k: _dot(_bf(lhs[j][k]), _bf(kv_fac[kept(j, k)]))):
            store_q(0, g, r, head, val)

    def q_step(step, parts, zero, first, last, *pace):
        side = _SideWork()
        for tasks, (lag, width, phase) in zip(later_tasks(parts), pace):
            side.add(tasks, range(first, min(last, 49 * SPLIT - lag - width + 1)), lag, width, phase)
        fac = wq_factors(step)

        def mul_rows(j, k, n):
            side.step()
            lhs = x_fac[7 * j + k, n * S // 8 // SPLIT:(n + 1) * S // 8 // SPLIT]
            val = _dot(_bf(_with_corner(lhs, wide[gate(n * NG // SPLIT, j, k)])), _bf(fac[j][k]))
            token = pltpu.bitcast(val[0:8], U32)
            wqkv_raw[zero, 0, PP * 16:PP * 16 + 8, _cols(0)] = token
            wk_raw[RING * PP + zero, 0, 0:8] = token
            wv_raw[RING * PP + zero, 0, 0:8] = token
            c[2 * NG + zero, 0:8, _cols(0)] = token
            return val

        for r, head, val in _nested_strassen(lambda j, k: jnp.concatenate(
                [mul_rows(j, k, n) for n in range(SPLIT)], axis=0)):
            for g in range(NG):
                store_q(step, g, r, head, val[g * G // 4:(g + 1) * G // 4])
        side.check_done()

    def q_body(step, zero):
        _start(wq_copies(step + 1) + later_copies(step + 1))
        _wait(wq_copies(step) + later_copies(step - 1))
        q_step(step, [step - 1], zero, *PACE0)
        return -zero

    zero = lax.fori_loop(1, NS - 1, q_body, 0)
    _wait(wq_copies(NS - 1) + later_copies(NS - 2) + later_copies(NS - 1))
    woa_copy(0).start()
    q_step(NS - 1, [zero + NS - 2, zero + NS - 1], zero, *PACE1)
    project_kv(0, 0, 0)
    for g in range(NG):
        for j in range(7):
            wide[c_gate(g, j)] = c_factor(g, j)[0:8, 0:128]
    kb, vb = 0, KV_ROWS
    for buf in (kb, vb):
        wq_raw[:, :, buf + RC:buf + RC + HALO, :] = jnp.zeros((2 * PP, 2, HALO, D), U32)
    _start(xb_copies)

    def pair_body(p, zero):
        part = p >> 1

        @pl.when((p & 1) == 0)
        def _():
            pl.when(part + 1 < NS)(lambda: woa_copy(part + 1).start())
            woa_copy(part).wait()

        side = _SideWork()
        side.add([P(prepare_woa, part, p & 1, n) for n in range(8)], range(*PACE2[:2]), *PACE2[2:])
        row = lax.broadcasted_iota(jnp.int32, (BQ, BQ), 0)
        col = lax.broadcasted_iota(jnp.int32, (BQ, BQ), 1)
        causal = ((col & ~15) | ((col & 15) >> 1) | ((col & 1) << 3)) <= row
        hb = BQ // 2

        def scores(e, i):
            r = i * BQ
            k = ctx[H + e + zero, 0:hb, :]
            k = _bf(jnp.concatenate([k, k_buf[e, hb:(i + 1) * hb, :]], axis=0) if i else k)
            q = _bf(ctx[2 * p + e, i * hb:(i + 1) * hb, :])
            s = lax.dot_general(q, k, _NT, preferred_element_type=F32)
            diag = jnp.where(causal, s[:, r:], NEG)
            s = jnp.concatenate([s[:, :r], diag], axis=1) if r else diag
            return s, jnp.max(s, axis=1, keepdims=True)

        def context(e, i, s, peak):
            w = jnp.exp2(s - peak)
            total = jnp.sum(w, axis=1, keepdims=True)
            o = _dot(w.astype(BF16), _bf(v_buf[e, 0:(i + 1) * hb, :]))
            return _words(o * _recip(total))

        state = {}
        for op in _attention_order():
            if op[0] in "kv":
                pair = jnp.minimum(p + 1, NP - 1) if op == "k0" else p
                project_kv("kv".index(op[0]), pair, int(op[1:]), side)
                continue
            e, i = "ab".index(op[1]), int(op[2:])
            if op[0] == "S":
                state[e, i] = scores(e, i)
            elif op[0] == "P":
                state[e, i] = context(e, i, *state[e, i])
            else:
                ctx[2 * p + e, i * hb:(i + 1) * hb, :] = state.pop((e, i))
        assert not state
        side.check_done()
        return -zero

    lax.fori_loop(0, NP, pair_body, 0)
    _wait(xb_copies)

    n_chunks = S // RC
    hr = RC // 2
    qw = RC // 8

    def out_copy(i, slot):
        return pltpu.make_async_copy(
            obuf.at[slot], out_hbm.at[pl.ds(_mult(i, RC), RC), :], sem_out.at[slot])

    def last_copy(n):
        lo, hi = ((0, M), (M, M + 256), (M + W, M + W + 256), (M + 256, M + W), (M + W + 256, 2 * M))[n]
        return pltpu.make_async_copy(
            obuf.at[1, :, lo:hi], out_hbm.at[S - RC:S, lo:hi], sem_out.at[1])

    def chunk_body(i, zero, last=False):
        slot = i & 1
        base = _mult(i, RC // 2)

        @pl.when(i >= 2)
        def _():
            out_copy(i - 2, slot).wait()

        def is_plain(j, k):
            return j in (2, 3) and k in (2, 3)

        def ctx_at(j, k, u, lo, n):
            if is_plain(j, k):
                quarter = 2 * (j - 2) + k - 2
                return ctx, (4 * u + quarter, pl.ds(base + quarter * qw + lo, n))
            slab, r = divmod((2 * (7 * j + k) + u // 4) * qw + lo, SLAB)
            return wide, (CS0 + slab, slice(r, r + n), _cols(u % 4))

        ctx_fac = {}

        def ctx_factor_store(u, lo, j, k):
            if (u, lo) not in ctx_fac:
                ctx_fac[u, lo] = _nested_factors_of_words(_lhs_factors, [
                    [ctx[4 * u + hq, pl.ds(base + r * qw + lo, 8)] for hq in range(4)]
                    for r in range(4)])
            return [ctx_at(j, k, u, lo, 8) + (ctx_fac[u, lo][j][k],)]

        def taps(buf, t, w, r):
            lo = buf + HALO - DIL * w + r
            return pltpu.bitcast(wq_raw[t // 2, t % 2, lo:lo + 8, :], F32)

        def tile_at(n, r, rows):
            return n // 4, slice(n % 4 * RC + r, n % 4 * RC + r + rows)

        q_alias = v_buf.at[pl.ds(zero, 2)]
        logit_alias = k_buf.at[pl.ds(zero, 2)]

        def window_logits(r, ws):
            q = [pltpu.bitcast((v_buf if t else q_alias)[tile_at(t, r, 8)], F32) for t in range(8)]
            logits = [functools.reduce(jnp.add, [q[t] * taps(kb, t, w, r) for t in range(8)])
                      for w in ws]
            logits = [z + pltpu.roll(z, 64, 1) for z in logits]
            logits = [(z + pltpu.roll(z, 32, 1)) * (DB ** -0.5 * LOG2E) for z in logits]
            pos = i * RC + r + lax.broadcasted_iota(jnp.int32, (8, 128), 0)
            return [(k_buf, tile_at(w, r, 8), pltpu.bitcast(
                jnp.where(pos >= DIL * w, z, NEG) if DIL * w > r else z, U32))
                for w, z in zip(ws, logits)]

        weights = {}

        def window_softmax(r):
            logits = [pltpu.bitcast((k_buf if w else logit_alias)[tile_at(w, r, 8)], F32)
                      for w in range(WIN)]
            peak = functools.reduce(jnp.maximum, logits)
            probs = [jnp.exp2(z - peak) for z in logits]
            inv = _recip(functools.reduce(jnp.add, probs))
            weights[r] = [z * inv for z in probs]
            return []

        def window_values(r, ts):
            return [(wide, (LOC0 + r // hr, slice(r % hr + (t % 2) * hr, r % hr + (t % 2) * hr + 8),
                            _cols(t // 2)),
                     pltpu.bitcast(functools.reduce(
                         jnp.add, [weights[r][w] * taps(vb, t, w, r) for w in range(WIN)]), U32))
                    for t in ts]

        n_steps = 3 * 4 * 7 + 2 * 49
        order = (2, 4, 3, 1, 0, 6, 5)
        side = _SideWork()
        side.add([P(ctx_factor_store, u, lo, j, k) for u in range(8) for lo in range(0, qw, 8)
                  for j in order for k in order if not is_plain(j, k)], range(CTX_FIRST, CTX_LAST), 0)
        side.add([P(window_logits, r, ws) for r in range(0, RC, 8)
                  for ws in ((0, 4, 1, 5), (2, 6, 3, 7))],
                 range(LOGIT_FIRST, LOGIT_LAST - LOGIT_LAG), LOGIT_LAG)
        side.add([P(window_softmax, r) for r in range(0, RC, 8)],
                 range(VALUE_FIRST, n_steps - 2), 0)
        side.add([P(window_values, r, ts) for r in range(0, RC, 8)
                  for ts in (range(4), range(4, 8))], range(VALUE_FIRST + 2, n_steps), 0)
        wide_alias = wide.at[pl.ds(zero, CS0)]

        def mul(lhs, slab, *tiles):
            side.step()
            rhs = jnp.concatenate([wide[slab, :, _cols(t)] for t in tiles], axis=0)
            rhs = _with_corner(rhs, wide_alias[slab, 0:8, _cols(tiles[0])])
            val = _dot(_bf(lhs), _bf(rhs))
            for buf in (k_buf, v_buf):
                buf[0, S // 2:S // 2 + 8, :] = pltpu.bitcast(val[0:8], U32)
            return val

        xb_fac = _factors_of_words(_lhs_factors, *[
            jnp.concatenate([
                x_fac[4 * (i >> 1) + 2 * k + t, pl.ds(_mult(2 * (i & 1) + r, hr // 2), hr // 2)]
                for t in range(2)], axis=1) for r in range(2) for k in range(2)])
        for part, buf in ((1, kb), (0, None), (2, vb)):
            if part:
                wq_raw[:, :, buf:buf + HALO, :] = wq_raw[:, :, buf + RC:buf + RC + HALO, :]
            for t in range(4):
                blocks = _strassen(lambda j: mul(xb_fac[j], QKV0 + 7 * part + j, t))
                for n, val in enumerate(blocks):
                    r, k = divmod(n, 2)
                    if part:
                        lo = buf + HALO + r * hr
                        wq_raw[2 * k + t // 2, t % 2, lo:lo + hr, :] = pltpu.bitcast(val, U32)
                    else:
                        v_buf[tile_at(4 * k + t, r * hr, hr)] = pltpu.bitcast(val, U32)

        def ctx_factor(j, k):
            return jnp.concatenate(
                [ref[idx] for ref, idx in (ctx_at(j, k, u, 0, qw) for u in range(8))], axis=1)

        for t in range(2):
            for r, k, val in _nested_strassen(
                    lambda j, k: mul(ctx_factor(j, k), OA0 + 7 * j + k, 2 * t, 2 * t + 1)):
                obuf[slot, r * RC // 4:(r + 1) * RC // 4, _cols(2 * k + t)] = val.astype(BF16)
        side.check_done()
        if last:
            last_copy(0).start()

        o_fac = [z.astype(BF16) for z in _lhs_factors(*[
            pltpu.bitcast(wide[LOC0 + r, e * hr:(e + 1) * hr, :], F32)
            for r in range(2) for e in range(2)])]
        for t in range(4):
            blocks = _strassen(lambda j: _dot(o_fac[j], _bf(wide[OB0 + j, :, _cols(t)])))
            for n, val in enumerate(blocks):
                r, k = divmod(n, 2)
                obuf[slot, r * hr:(r + 1) * hr, _cols(8 + 4 * k + t)] = val.astype(BF16)
            if last and t == 1:
                _start([last_copy(1), last_copy(2)])

        if last:
            _start([last_copy(n) for n in range(3, 5)])
        else:
            out_copy(i, slot).start()
        return -zero

    zero = lax.fori_loop(0, n_chunks - 1, chunk_body, 0)
    chunk_body(n_chunks - 1, zero, last=True)
    out_copy(n_chunks - 2, 0).wait()
    _wait([last_copy(n) for n in range(5)])


@jax.jit
def pallas_concat_heads__compressed_kv_cla__sliding_local_dilated__prompt_kernel(
    A_x: jax.Array,
    A_c_kv: jax.Array,
    A_w_q: jax.Array,
    A_w_uk: jax.Array,
    A_w_uv: jax.Array,
    A_w_o: jax.Array,
    B_x: jax.Array,
    B_wqkv: jax.Array,
    B_wo: jax.Array,
):
    scratch = [
        pltpu.VMEM((49, S // 8, M // 4), U32),
        pltpu.VMEM((N_SLABS, SLAB, W), U32),
        pltpu.VMEM((2 * NG + 1, G // 4, DC), U32),
        pltpu.VMEM((5, S // 4, DC // 2), U32),
        pltpu.VMEM((NP, 2, 7, DC // 4, D), U32),
        pltpu.VMEM((2, S // 2 + 8, D), U32),
        pltpu.VMEM((2, S // 2 + 8, D), U32),
        pltpu.VMEM((H + 2, S // 2, D), U32),
        pltpu.VMEM((2 * PP, 2, 2 * KV_ROWS + 8, D), U32),
        pltpu.VMEM((RING * PP + 1, 2, DC // 2, D), U32),
        pltpu.VMEM((RING * PP + 1, 2, DC // 2, D), U32),
        pltpu.VMEM((NG, PP * D, M), U32),
        pltpu.VMEM((RING, 2, PP * 16 + 8, 3 * M), U32),
        pltpu.VMEM((RING * PP, HB, M), U32),
        pltpu.VMEM((2, RC, 2 * M), BF16),
        pltpu.SemaphoreType.DMA((NG,)),
        pltpu.SemaphoreType.DMA((4,)),
        pltpu.SemaphoreType.DMA((2,)),
    ]
    out = pl.pallas_call(
        _kernel,
        out_shape=jax.ShapeDtypeStruct((S, 2 * M), BF16),
        in_specs=[pl.BlockSpec(memory_space=pl.ANY)] * 9,
        out_specs=pl.BlockSpec(memory_space=pl.ANY),
        scratch_shapes=scratch,
        compiler_params=pltpu.CompilerParams(
            vmem_limit_bytes=127 * 2**20, disable_bounds_checks=True),
        name="fused_mla_sliding",
    )(
        A_x.reshape(S, M),
        A_c_kv.reshape(2 * NG, G // 2, DC),
        A_w_q.reshape(M // 2, 2, H, D),
        A_w_uk.reshape(DC // 2, 2, H, D),
        A_w_uv.reshape(DC // 2, 2, H, D),
        A_w_o.reshape(H * D, M),
        B_x.reshape(S, M),
        B_wqkv.reshape(2, M // 2, 3 * M),
        B_wo.reshape(HB, DB, M),
    )
    return out.reshape(1, S, 2 * M)
```

```python
import functools

import jax
import jax.numpy as jnp
import numpy as np
from jax import lax
import jax.experimental.pallas as pl
import jax.experimental.pallas.tpu as pltpu

S = 2048
M = 1024
DC = 512
H = 32
D = 128
HB = 32
DB = 32
WIN = 8
DIL = 2

NP = H // 2
PP = 2
NS = NP // PP
RING = 3
G = 512
NG = S // G
BQ = 128
RC = 256
HALO = 16
KV_ROWS = HALO + RC + 8
LOG2E = 1.4426950408889634
NEG = -1e9 * LOG2E

W = M // 2
SLAB = M // 4
OA0 = 0
QKV0 = OA0 + 49
OB0 = QKV0 + 21
CS0 = OB0 + 7
LOC0 = CS0 + 13
GATE = CS0
N_SLABS = LOC0 + 2

SPLIT = 2
Q_ORDER = (1, 4, 2, 3, 0, 6, 5)
KV_ORDER = (0, 5, 6, 2, 3, 4, 1)
A_ORDER = (2, 3, 4, 1, 0, 6, 5)
B_ORDER = (2, 4, 3, 1, 0, 6, 5)
PACE2 = (0, 28, 0, 4)
PACE0 = (0, 88, (7, 1, 0.5), (0, 2, 0.5), (0, 2, 0))
PACE1 = (2, 88, (7, 1, 0.5), (0, 2, 0.5), (0, 1, 0))
CTX_FIRST = 5
CTX_LAST = 85
LOGIT_FIRST = 84
LOGIT_LAST = 174
LOGIT_LAG = 6
VALUE_FIRST = 98

F32 = jnp.float32
BF16 = jnp.bfloat16
U32 = jnp.uint32
_NT = (((1,), (1,)), ((), ()))


def _attention_order():
    ops = ("Sa0 Sa1 Sa2 Sa3 v0 k1 Pa0 Pa1 Pa2 v1 Sa4 Pa3 k2 Sa5 Wa0 Wa1 Pa4 v2 "
           "Sa6 Wa2 Pa5 Wa3 k3 Sa7 Pa6 Wa4 v3").split()
    for i in range(8, 16):
        ops += [f"Sa{i}", f"Pa{i - 1}", f"Wa{i - 3}"]
    ops += "Sb15 Pa15 Wa13 Sb14 Pb15 Wa14 Sb13 Pb14 Wa15".split()
    for i in range(12, 3, -1):
        ops += [f"Sb{i}", f"Pb{i + 1}", f"Wb{i + 3}"]
    return ops + "Sb3 Sb2 Pb4 Wb6 Sb1 Sb0 Pb3 Pb2 k0 Pb1 Pb0 Wb5 Wb4 Wb3 Wb2 Wb1 Wb0".split()


def _dot(a, b):
    return jnp.dot(a, b, preferred_element_type=F32)


def _bf(words):
    return pltpu.bitcast(words, BF16)


def _words(x):
    return pltpu.bitcast(x.astype(BF16), U32)


def _halves(words):
    return (pltpu.bitcast(words << 16, F32),
            pltpu.bitcast(words & np.uint32(0xFFFF0000), F32))


def _pack(lo, hi):
    return pltpu.bitcast(pltpu.pack_elementwise([lo, hi], packed_dtype=BF16), U32)


def _words_shuffled(x):
    n, c = x.shape
    x = x.reshape(n // 16, 2, 8, c)
    return _pack(x[:, 0], x[:, 1]).reshape(n // 2, c)


def _recip(x):
    r = pl.reciprocal(x, approx=True)
    return r * (2.0 - x * r)


def _lhs_factors(a11, a12, a21, a22):
    return a11 + a22, a21 + a22, a11, a22, a11 + a12, a21 - a11, a12 - a22


def _rhs_factors(b11, b12, b21, b22):
    return b11 + b22, b11, b12 - b22, b21 - b11, b22, b11 + b12, b21 + b22


def _strassen(mul, order=(2, 3, 4, 1, 0, 6, 5)):
    m = {j + 1: mul(j) for j in order}
    return (m[4] - m[5]) + m[1] + m[7], m[3] + m[5], m[2] + m[4], (m[3] - m[2]) + m[1] + m[6]


def _factors_of_words(factors, *blocks):
    parts = [_halves(b) for b in blocks]
    plain = {id(lo): b for (lo, _), b in zip(parts, blocks)}
    return [plain.get(id(lo)) if id(lo) in plain else _pack(lo, hi)
            for lo, hi in zip(factors(*[x[0] for x in parts]), factors(*[x[1] for x in parts]))]


def _nested_factors(factors, blocks):
    inner = [factors(*[blocks[2 * r + ri][2 * c + ci] for r in range(2) for c in range(2)])
             for ri in range(2) for ci in range(2)]
    return [factors(*[x[j] for x in inner]) for j in range(7)]


def _nested_factors_of_words(factors, blocks):
    sides = [_nested_factors(factors, [[_halves(b)[side] for b in row] for row in blocks])
             for side in range(2)]
    return [[_pack(lo, hi) for lo, hi in zip(a, b)] for a, b in zip(*sides)]


def _nested_strassen(mul, *order):
    blocks = _strassen(lambda j: jnp.concatenate(
        _strassen(lambda k: mul(j, k), *order), axis=0), *order)
    for outer, val in enumerate(blocks):
        n = val.shape[0] // 4
        for inner in range(4):
            yield (2 * (outer // 2) + inner // 2, 2 * (outer % 2) + inner % 2,
                   val[inner * n:(inner + 1) * n])


def _permute_head_columns(words):
    tiles = [words[:, _cols(t)] for t in range(8)]
    lane = lax.broadcasted_iota(jnp.int32, tiles[0].shape, 1)
    for bit in (1, 2, 4):
        low = (lane & bit) == 0
        for t in range(8):
            if t & bit:
                continue
            a, b = tiles[t], tiles[t | bit]
            tiles[t] = jnp.where(low, a, pltpu.roll(b, bit, 1))
            tiles[t | bit] = jnp.where(low, pltpu.roll(a, 128 - bit, 1), b)
    src = ((lane & 3) << 5) | (lane >> 2)
    return jnp.concatenate([jnp.take_along_axis(x, src, axis=1) for x in tiles], axis=1)


def _with_corner(x, corner):
    top = corner if x.shape[1] == 128 else jnp.concatenate([corner, x[0:8, 128:]], axis=1)
    return jnp.concatenate([top, x[8:]], axis=0)


class _SideWork:
    def __init__(self):
        self.now = 0
        self.starts = {}
        self.stores = {}

    def add(self, tasks, steps, lag, width=1, phase=0.0):
        for n, task in enumerate(tasks):
            when = steps[int((n + phase) * len(steps)) // len(tasks)]
            self.starts.setdefault(when, []).append((task, lag, width))

    def step(self):
        for task, lag, width in self.starts.pop(self.now, []):
            stores = task()
            for n, store in enumerate(stores):
                self.stores.setdefault(self.now + lag + n * width // len(stores), []).append(store)
        for ref, idx, val in self.stores.pop(self.now, []):
            ref[idx] = val
        self.now += 1

    def check_done(self):
        assert not self.starts and not self.stores


def _mult(i, n):
    return i * n if isinstance(i, int) else pl.multiple_of(i * n, n)


def _wrap(i, n):
    if isinstance(i, int):
        return i % n
    return jnp.where(i >= 2 * n, i - 2 * n, jnp.where(i >= n, i - n, i))


def _cols(t):
    return slice(t * 128, (t + 1) * 128)


def _start(copies):
    for cp in copies:
        cp.start()


def _wait(copies):
    for cp in copies:
        cp.wait()


def _kernel(
    xa_hbm, c_hbm, wq_hbm, wk_hbm, wv_hbm, woa_hbm, xb_hbm, wqkv_hbm, wob_hbm,
    out_hbm,
    x_fac, wide, c, c_sum, kv_fac, k_buf, v_buf, ctx,
    wq_raw, wk_raw, wv_raw, woa_raw, wqkv_raw, wob_raw, obuf,
    sem_x, sem_w, sem_out,
):
    P = functools.partial
    xa32, c32, woa32, xb32, wqkv32 = (
        r.bitcast(U32) for r in (xa_hbm, c_hbm, woa_hbm, xb_hbm, wqkv_hbm))
    wq32, wk32, wv32, wob32 = (r.bitcast(U32) for r in (wq_hbm, wk_hbm, wv_hbm, wob_hbm))

    def pair_copies(src, dst, pair, slot, sem):
        return [pltpu.make_async_copy(
            src.at[:, odd, pair, :], dst.at[slot, odd, 0:src.shape[0]], sem) for odd in range(2)]

    def wq_copies(step):
        sem = sem_w.at[step & 3]
        return [cp for j in range(PP) for cp in pair_copies(
            wq32, wq_raw, step * PP + j, (step & 1) * PP + j, sem)]

    def later_copies(part):
        sem, slot = sem_w.at[(part + 1) & 3], _wrap(part, RING)
        copies = []
        for j in range(PP):
            pair = part * PP + j
            copies += pair_copies(wk32, wk_raw, pair, slot * PP + j, sem)
            copies += pair_copies(wv32, wv_raw, pair, slot * PP + j, sem)
            copies.append(pltpu.make_async_copy(
                wob32.at[:, pair, :], wob_raw.at[slot * PP + j], sem))
        for h in range(2):
            copies.append(pltpu.make_async_copy(
                wqkv32.at[h, pl.ds(_mult(part, PP * 16), PP * 16)],
                wqkv_raw.at[slot, h, 0:PP * 16], sem))
            rows = (2 * (part >> 1) + h, pl.ds(_mult(part & 1, G // 8), G // 8))
            copies.append(pltpu.make_async_copy(c32.at[rows], c.at[rows], sem))
        return copies

    def woa_copy(part):
        return pltpu.make_async_copy(woa32.at[pl.ds(_mult(part, PP * D), PP * D)],
                                     woa_raw.at[part & 1], sem_w.at[part & 1])

    def x_copy(g):
        return pltpu.make_async_copy(xa32.at[g * G // 2:(g + 1) * G // 2],
                                     woa_raw.at[g], sem_x.at[g])

    xb_copies = [pltpu.make_async_copy(
        xb32.at[r * S // 8:(r + 1) * S // 8, k * M // 4:(k + 1) * M // 4],
        x_fac.at[4 * r + k], sem_x.at[0]) for r in range(4) for k in range(4)]

    gw = G // 4
    sum_index = {0: 0, 1: 1, 4: 2, 5: 3, 6: 4}

    def head_factors(raw, slot, top, bottom, n):
        sides = [_rhs_factors(*_halves(raw[slot, odd, top:top + n, :]),
                              *_halves(raw[slot, odd, bottom:bottom + n, :]))
                 for odd in range(2)]
        return [_pack(even, odd) for even, odd in zip(*sides)]

    def group_blocks(g, mul):
        for n, val in enumerate(_strassen(mul, KV_ORDER)):
            r, e = divmod(n, 2)
            yield e, slice((2 * g + r) * gw, (2 * g + r + 1) * gw), val

    def c_factor(g, j):
        if j in sum_index:
            return c_sum[sum_index[j], g * gw:(g + 1) * gw, :]
        return c[2 * g + j - 2, :, (j - 2) * DC // 2:(j - 1) * DC // 2]

    def c_gate(g, j):
        return GATE + 2, slice(8 * (7 * g + j), 8 * (7 * g + j + 1)), _cols(0)

    def project_kv(n, pair, g, side=None):
        def mul(j):
            lhs = c_factor(g, j)
            if side:
                side.step()
                lhs = _with_corner(lhs, wide[c_gate(g, j)])
            return _dot(_bf(lhs), _bf(kv_fac[pair, n, j]))

        for e, rows, val in group_blocks(g, mul):
            val = _words_shuffled(val)
            (k_buf, v_buf)[n][e, rows, :] = val
            if n == 0 and rows.start == 0:
                ctx[H + e, 0:BQ // 2, :] = val[0:BQ // 2]

    def prepare_kv(n, pair, piece):
        vals = head_factors((wk_raw, wv_raw)[n], _wrap(pair, RING * PP),
                            piece * 16, DC // 4 + piece * 16, 16)
        return [(kv_fac, (pair, n, j, slice(piece * 16, (piece + 1) * 16)), val)
                for j, val in enumerate(vals)]

    def prepare_c(part, piece):
        r = _mult(part & 1, G // 8) + 16 * piece
        vals = _factors_of_words(_lhs_factors, *[
            c[2 * (part >> 1) + h, pl.ds(r, 16), k * DC // 2:(k + 1) * DC // 2]
            for h in range(2) for k in range(2)])
        return [(c_sum, (n, pl.ds(_mult(part >> 1, gw) + r, 16)), vals[j])
                for j, n in sum_index.items()]

    def prepare_wqkv(part, piece, which):
        both = _permute_head_columns(jnp.concatenate([
            wqkv_raw[_wrap(part, RING), h, 8 * piece:8 * piece + 8, which * M:(which + 1) * M]
            for h in range(2)], axis=0))
        vals = _factors_of_words(
            _rhs_factors, both[:8, :W], both[:8, W:], both[8:, :W], both[8:, W:])
        r = _mult(part, PP * 16) + 8 * piece
        return [(wide, (QKV0 + 7 * which + j, pl.ds(r, 8)), val) for j, val in enumerate(vals)]

    def prepare_wob(pair, t):
        b11, b21 = _halves(wob_raw[_wrap(pair, RING * PP), :, _cols(t)])
        b12, b22 = _halves(wob_raw[_wrap(pair, RING * PP), :, _cols(4 + t)])
        r = _mult((pair & 3) * 4 + (pair >> 2), HB // 2)
        return [(wide, (OB0 + j, pl.ds(r, HB // 2), _cols(t)), _words(val))
                for j, val in enumerate(_rhs_factors(b11, b12, b21, b22))]

    def prepare_woa(part, t, n):
        fac = _nested_factors_of_words(_rhs_factors, [
            [woa_raw[part & 1, hq * D // 2 + 8 * n:hq * D // 2 + 8 * n + 8,
                     pl.ds(_mult(2 * k + t, 128), 128)]
             for k in range(4)] for hq in range(4)])
        order = (1, 5, 4, 2, 0, 6, 3)
        rows = pl.ds(_mult(part & 3, D // 2) + 8 * n, 8)
        cols = pl.ds(_mult(2 * t + (part >> 2), 128), 128)
        return [(wide, (OA0 + 7 * j + k, rows, cols), fac[j][k]) for j in order for k in order]

    def later_tasks(parts):
        quads = [(part, j, part * PP + j) for part in parts for j in range(PP)]
        return (
            [P(prepare_wqkv, part, 2 * j + n // 3, n % 3) for part, j, _ in quads for n in range(6)],
            [P(prepare_kv, n % 2, pair, n // 2) for _, _, pair in quads for n in range(16)],
            [task for part, j, pair in quads for n in range(2) for task in (
                P(prepare_wob, pair, 2 * n), P(prepare_c, part, 2 * j + n),
                P(prepare_wob, pair, 2 * n + 1))])

    qw0 = G // 8

    def gate(g, j, k):
        n = 7 * j + k
        return GATE + n // 32, slice(n % 32 * 8, n % 32 * 8 + 8), _cols(g)

    def make_x_factors(g):
        fac = _nested_factors_of_words(_lhs_factors, [
            [woa_raw[g, r * qw0:(r + 1) * qw0, k * M // 4:(k + 1) * M // 4]
             for k in range(4)] for r in range(4)])
        for j in range(7):
            for k in range(7):
                x_fac[7 * j + k, g * qw0:(g + 1) * qw0] = fac[j][k]
                if g % (NG // SPLIT) == 0:
                    wide[gate(g, j, k)] = fac[j][k][0:8, 0:128]
        return fac

    def wq_factors(step):
        n = M // 8
        sides = [_nested_factors(_rhs_factors, [
            [half for j in range(PP) for half in _halves(
                wq_raw[(step * PP + j) & (2 * PP - 1), odd, k * n:(k + 1) * n, :])]
            for k in range(4)]) for odd in range(2)]
        return [[_pack(even, odd) for even, odd in zip(a, b)] for a, b in zip(*sides)]

    def store_q(step, g, r, head, val):
        ctx[4 * step + head, (4 * g + r) * qw0:(4 * g + r + 1) * qw0, :] = _words(
            val * (D ** -0.5 * LOG2E))

    _start(wq_copies(0) + [x_copy(g) for g in range(NG)]
           + wq_copies(1) + later_copies(0) + later_copies(1))
    _wait(wq_copies(0))

    def kept(j, k):
        return (NP - 1 - j // 2, j % 2, k)

    for j, row in enumerate(wq_factors(0)):
        for k, val in enumerate(row):
            kv_fac[kept(j, k)] = val
    for g in range(NG):
        x_copy(g).wait()
        lhs = make_x_factors(g)
        for r, head, val in _nested_strassen(
                lambda j, k: _dot(_bf(lhs[j][k]), _bf(kv_fac[kept(j, k)]))):
            store_q(0, g, r, head, val)

    def q_step(step, parts, zero, first, last, *pace):
        side = _SideWork()
        for tasks, (lag, width, phase) in zip(later_tasks(parts), pace):
            side.add(tasks, range(first, min(last, 49 * SPLIT - lag - width + 1)), lag, width, phase)
        fac = wq_factors(step)

        def mul_rows(j, k, n):
            side.step()
            lhs = x_fac[7 * j + k, n * S // 8 // SPLIT:(n + 1) * S // 8 // SPLIT]
            val = _dot(_bf(_with_corner(lhs, wide[gate(n * NG // SPLIT, j, k)])), _bf(fac[j][k]))
            token = pltpu.bitcast(val[0:8], U32)
            wqkv_raw[zero, 0, PP * 16:PP * 16 + 8, _cols(0)] = token
            wk_raw[RING * PP + zero, 0, 0:8] = token
            wv_raw[RING * PP + zero, 0, 0:8] = token
            c[2 * NG + zero, 0:8, _cols(0)] = token
            return val

        for r, head, val in _nested_strassen(lambda j, k: jnp.concatenate(
                [mul_rows(j, k, n) for n in range(SPLIT)], axis=0), Q_ORDER):
            for g in range(NG):
                store_q(step, g, r, head, val[g * G // 4:(g + 1) * G // 4])
        side.check_done()

    def q_body(step, zero):
        _start(wq_copies(step + 1) + later_copies(step + 1))
        _wait(wq_copies(step) + later_copies(step - 1))
        q_step(step, [step - 1], zero, *PACE0)
        return -zero

    zero = lax.fori_loop(1, NS - 1, q_body, 0)
    _wait(wq_copies(NS - 1) + later_copies(NS - 2) + later_copies(NS - 1))
    woa_copy(0).start()
    q_step(NS - 1, [zero + NS - 2, zero + NS - 1], zero, *PACE1)
    project_kv(0, 0, 0)
    for g in range(NG):
        for j in range(7):
            wide[c_gate(g, j)] = c_factor(g, j)[0:8, 0:128]
    kb, vb = 0, KV_ROWS
    for buf in (kb, vb):
        wq_raw[:, :, buf + RC:buf + RC + HALO, :] = jnp.zeros((2 * PP, 2, HALO, D), U32)
    _start(xb_copies)

    def pair_body(p, zero):
        part = p >> 1

        @pl.when((p & 1) == 0)
        def _():
            pl.when(part + 1 < NS)(lambda: woa_copy(part + 1).start())
            woa_copy(part).wait()

        side = _SideWork()
        side.add([P(prepare_woa, part, p & 1, n) for n in range(8)], range(*PACE2[:2]), *PACE2[2:])
        row = lax.broadcasted_iota(jnp.int32, (BQ, BQ), 0)
        col = lax.broadcasted_iota(jnp.int32, (BQ, BQ), 1)
        causal = ((col & ~15) | ((col & 15) >> 1) | ((col & 1) << 3)) <= row
        hb = BQ // 2

        def scores(e, i):
            r = i * BQ
            k = ctx[H + e + zero, 0:hb, :]
            k = _bf(jnp.concatenate([k, k_buf[e, hb:(i + 1) * hb, :]], axis=0) if i else k)
            q = _bf(ctx[2 * p + e, i * hb:(i + 1) * hb, :])
            s = lax.dot_general(q, k, _NT, preferred_element_type=F32)
            diag = jnp.where(causal, s[:, r:], NEG)
            s = jnp.concatenate([s[:, :r], diag], axis=1) if r else diag
            return s, jnp.max(s, axis=1, keepdims=True)

        def context(e, i, s, peak):
            w = jnp.exp2(s - peak)
            total = jnp.sum(w, axis=1, keepdims=True)
            o = _dot(w.astype(BF16), _bf(v_buf[e, 0:(i + 1) * hb, :]))
            return _words(o * _recip(total))

        state = {}
        for op in _attention_order():
            if op[0] in "kv":
                pair = jnp.minimum(p + 1, NP - 1) if op == "k0" else p
                project_kv("kv".index(op[0]), pair, int(op[1:]), side)
                continue
            e, i = "ab".index(op[1]), int(op[2:])
            if op[0] == "S":
                state[e, i] = scores(e, i)
            elif op[0] == "P":
                state[e, i] = context(e, i, *state[e, i])
            else:
                ctx[2 * p + e, i * hb:(i + 1) * hb, :] = state.pop((e, i))
        assert not state
        side.check_done()
        return -zero

    lax.fori_loop(0, NP, pair_body, 0)
    _wait(xb_copies)

    n_chunks = S // RC
    hr = RC // 2
    qw = RC // 8

    def out_copy(i, slot):
        return pltpu.make_async_copy(
            obuf.at[slot], out_hbm.at[pl.ds(_mult(i, RC), RC), :], sem_out.at[slot])

    def last_copy(n):
        lo, hi = ((0, M), (M, M + 256), (M + W, M + W + 256), (M + 256, M + W), (M + W + 256, 2 * M))[n]
        return pltpu.make_async_copy(
            obuf.at[1, :, lo:hi], out_hbm.at[S - RC:S, lo:hi], sem_out.at[1])

    def chunk_body(i, zero, last=False):
        slot = i & 1
        base = _mult(i, RC // 2)

        @pl.when(i >= 2)
        def _():
            out_copy(i - 2, slot).wait()

        def is_plain(j, k):
            return j in (2, 3) and k in (2, 3)

        def ctx_at(j, k, u, lo, n):
            if is_plain(j, k):
                quarter = 2 * (j - 2) + k - 2
                return ctx, (4 * u + quarter, pl.ds(base + quarter * qw + lo, n))
            slab, r = divmod((2 * (7 * j + k) + u // 4) * qw + lo, SLAB)
            return wide, (CS0 + slab, slice(r, r + n), _cols(u % 4))

        ctx_fac = {}

        def ctx_factor_store(u, lo, j, k):
            if (u, lo) not in ctx_fac:
                ctx_fac[u, lo] = _nested_factors_of_words(_lhs_factors, [
                    [ctx[4 * u + hq, pl.ds(base + r * qw + lo, 8)] for hq in range(4)]
                    for r in range(4)])
            return [ctx_at(j, k, u, lo, 8) + (ctx_fac[u, lo][j][k],)]

        def taps(buf, t, w, r):
            lo = buf + HALO - DIL * w + r
            return pltpu.bitcast(wq_raw[t // 2, t % 2, lo:lo + 8, :], F32)

        def tile_at(n, r, rows):
            return n // 4, slice(n % 4 * RC + r, n % 4 * RC + r + rows)

        q_alias = v_buf.at[pl.ds(zero, 2)]
        logit_alias = k_buf.at[pl.ds(zero, 2)]

        def window_logits(r, ws):
            q = [pltpu.bitcast((v_buf if t else q_alias)[tile_at(t, r, 8)], F32) for t in range(8)]
            logits = [functools.reduce(jnp.add, [q[t] * taps(kb, t, w, r) for t in range(8)])
                      for w in ws]
            logits = [z + pltpu.roll(z, 64, 1) for z in logits]
            logits = [(z + pltpu.roll(z, 32, 1)) * (DB ** -0.5 * LOG2E) for z in logits]
            pos = i * RC + r + lax.broadcasted_iota(jnp.int32, (8, 128), 0)
            return [(k_buf, tile_at(w, r, 8), pltpu.bitcast(
                jnp.where(pos >= DIL * w, z, NEG) if DIL * w > r else z, U32))
                for w, z in zip(ws, logits)]

        weights = {}

        def window_softmax(r):
            logits = [pltpu.bitcast((k_buf if w else logit_alias)[tile_at(w, r, 8)], F32)
                      for w in range(WIN)]
            peak = functools.reduce(jnp.maximum, logits)
            probs = [jnp.exp2(z - peak) for z in logits]
            inv = _recip(functools.reduce(jnp.add, probs))
            weights[r] = [z * inv for z in probs]
            return []

        def window_values(r, ts):
            return [(wide, (LOC0 + r // hr, slice(r % hr + (t % 2) * hr, r % hr + (t % 2) * hr + 8),
                            _cols(t // 2)),
                     pltpu.bitcast(functools.reduce(
                         jnp.add, [weights[r][w] * taps(vb, t, w, r) for w in range(WIN)]), U32))
                    for t in ts]

        n_steps = 3 * 4 * 7 + 2 * 49
        order = (2, 4, 3, 1, 0, 6, 5)
        side = _SideWork()
        side.add([P(ctx_factor_store, u, lo, j, k) for u in range(8) for lo in range(0, qw, 8)
                  for j in order for k in order if not is_plain(j, k)], range(CTX_FIRST, CTX_LAST), 0)
        side.add([P(window_logits, r, ws) for r in range(0, RC, 8)
                  for ws in ((0, 4, 1, 5), (2, 6, 3, 7))],
                 range(LOGIT_FIRST, LOGIT_LAST - LOGIT_LAG), LOGIT_LAG)
        side.add([P(window_softmax, r) for r in range(0, RC, 8)],
                 range(VALUE_FIRST, n_steps - 2), 0)
        side.add([P(window_values, r, ts) for r in range(0, RC, 8)
                  for ts in (range(4), range(4, 8))], range(VALUE_FIRST + 2, n_steps), 0)
        wide_alias = wide.at[pl.ds(zero, CS0)]

        def mul(lhs, slab, *tiles):
            side.step()
            rhs = jnp.concatenate([wide[slab, :, _cols(t)] for t in tiles], axis=0)
            rhs = _with_corner(rhs, wide_alias[slab, 0:8, _cols(tiles[0])])
            val = _dot(_bf(lhs), _bf(rhs))
            for buf in (k_buf, v_buf):
                buf[0, S // 2:S // 2 + 8, :] = pltpu.bitcast(val[0:8], U32)
            return val

        xb_fac = _factors_of_words(_lhs_factors, *[
            jnp.concatenate([
                x_fac[4 * (i >> 1) + 2 * k + t, pl.ds(_mult(2 * (i & 1) + r, hr // 2), hr // 2)]
                for t in range(2)], axis=1) for r in range(2) for k in range(2)])
        for part, buf in ((1, kb), (0, None), (2, vb)):
            if part:
                wq_raw[:, :, buf:buf + HALO, :] = wq_raw[:, :, buf + RC:buf + RC + HALO, :]
            for t in range(4):
                blocks = _strassen(lambda j: mul(xb_fac[j], QKV0 + 7 * part + j, t), B_ORDER)
                for n, val in enumerate(blocks):
                    r, k = divmod(n, 2)
                    if part:
                        lo = buf + HALO + r * hr
                        wq_raw[2 * k + t // 2, t % 2, lo:lo + hr, :] = pltpu.bitcast(val, U32)
                    else:
                        v_buf[tile_at(4 * k + t, r * hr, hr)] = pltpu.bitcast(val, U32)

        def ctx_factor(j, k):
            return jnp.concatenate(
                [ref[idx] for ref, idx in (ctx_at(j, k, u, 0, qw) for u in range(8))], axis=1)

        for t in range(2):
            for r, k, val in _nested_strassen(
                    lambda j, k: mul(ctx_factor(j, k), OA0 + 7 * j + k, 2 * t, 2 * t + 1),
                    A_ORDER):
                obuf[slot, r * RC // 4:(r + 1) * RC // 4, _cols(2 * k + t)] = val.astype(BF16)
        side.check_done()
        if last:
            last_copy(0).start()

        o_fac = [z.astype(BF16) for z in _lhs_factors(*[
            pltpu.bitcast(wide[LOC0 + r, e * hr:(e + 1) * hr, :], F32)
            for r in range(2) for e in range(2)])]
        for t in range(4):
            blocks = _strassen(lambda j: _dot(o_fac[j], _bf(wide[OB0 + j, :, _cols(t)])))
            for n, val in enumerate(blocks):
                r, k = divmod(n, 2)
                obuf[slot, r * hr:(r + 1) * hr, _cols(8 + 4 * k + t)] = val.astype(BF16)
            if last and t == 1:
                _start([last_copy(1), last_copy(2)])

        if last:
            _start([last_copy(n) for n in range(3, 5)])
        else:
            out_copy(i, slot).start()
        return -zero

    zero = lax.fori_loop(0, n_chunks - 1, chunk_body, 0)
    chunk_body(n_chunks - 1, zero, last=True)
    out_copy(n_chunks - 2, 0).wait()
    _wait([last_copy(n) for n in range(5)])


@jax.jit
def pallas_concat_heads__compressed_kv_cla__sliding_local_dilated__prompt_kernel(
    A_x: jax.Array,
    A_c_kv: jax.Array,
    A_w_q: jax.Array,
    A_w_uk: jax.Array,
    A_w_uv: jax.Array,
    A_w_o: jax.Array,
    B_x: jax.Array,
    B_wqkv: jax.Array,
    B_wo: jax.Array,
):
    scratch = [
        pltpu.VMEM((49, S // 8, M // 4), U32),
        pltpu.VMEM((N_SLABS, SLAB, W), U32),
        pltpu.VMEM((2 * NG + 1, G // 4, DC), U32),
        pltpu.VMEM((5, S // 4, DC // 2), U32),
        pltpu.VMEM((NP, 2, 7, DC // 4, D), U32),
        pltpu.VMEM((2, S // 2 + 8, D), U32),
        pltpu.VMEM((2, S // 2 + 8, D), U32),
        pltpu.VMEM((H + 2, S // 2, D), U32),
        pltpu.VMEM((2 * PP, 2, 2 * KV_ROWS + 8, D), U32),
        pltpu.VMEM((RING * PP + 1, 2, DC // 2, D), U32),
        pltpu.VMEM((RING * PP + 1, 2, DC // 2, D), U32),
        pltpu.VMEM((NG, PP * D, M), U32),
        pltpu.VMEM((RING, 2, PP * 16 + 8, 3 * M), U32),
        pltpu.VMEM((RING * PP, HB, M), U32),
        pltpu.VMEM((2, RC, 2 * M), BF16),
        pltpu.SemaphoreType.DMA((NG,)),
        pltpu.SemaphoreType.DMA((4,)),
        pltpu.SemaphoreType.DMA((2,)),
    ]
    out = pl.pallas_call(
        _kernel,
        out_shape=jax.ShapeDtypeStruct((S, 2 * M), BF16),
        in_specs=[pl.BlockSpec(memory_space=pl.ANY)] * 9,
        out_specs=pl.BlockSpec(memory_space=pl.ANY),
        scratch_shapes=scratch,
        compiler_params=pltpu.CompilerParams(
            vmem_limit_bytes=127 * 2**20, disable_bounds_checks=True),
        name="fused_mla_sliding",
    )(
        A_x.reshape(S, M),
        A_c_kv.reshape(2 * NG, G // 2, DC),
        A_w_q.reshape(M // 2, 2, H, D),
        A_w_uk.reshape(DC // 2, 2, H, D),
        A_w_uv.reshape(DC // 2, 2, H, D),
        A_w_o.reshape(H * D, M),
        B_x.reshape(S, M),
        B_wqkv.reshape(2, M // 2, 3 * M),
        B_wo.reshape(HB, DB, M),
    )
    return out.reshape(1, S, 2 * M)
```

```python
import functools

import jax
import jax.numpy as jnp
import numpy as np
from jax import lax
import jax.experimental.pallas as pl
import jax.experimental.pallas.tpu as pltpu

S = 2048
M = 1024
DC = 512
H = 32
D = 128
HB = 32
DB = 32
WIN = 8
DIL = 2

NP = H // 2
PP = 2
NS = NP // PP
RING = 3
G = 512
NG = S // G
BQ = 128
RC = 256
HALO = 16
KV_ROWS = HALO + RC + 8
LOG2E = 1.4426950408889634
NEG = -1e9 * LOG2E

W = M // 2
SLAB = M // 4
OA0 = 0
QKV0 = OA0 + 49
OB0 = QKV0 + 21
CS0 = OB0 + 7
LOC0 = CS0 + 13
GATE = CS0
N_SLABS = LOC0 + 2

SPLIT = 2
Q_ORDER = (1, 4, 2, 3, 0, 6, 5)
KV_ORDER = (0, 5, 6, 2, 3, 4, 1)
B_ORDER = (2, 4, 3, 1, 0, 6, 5)
PACE0 = (1, 98, (9, 1, 0), (1, 2, 0), (3, 1, 0))
PACE1 = (1, 98, (9, 1, 0), (0, 1, 0), (3, 1, 0))
PACE2 = (0, 44, 0, 5)
CTX_FIRST = 5
CTX_LAST = 85
LOGIT_FIRST = 84
LOGIT_LAST = 174
LOGIT_LAG = 6
VALUE_FIRST = 98

F32 = jnp.float32
BF16 = jnp.bfloat16
U32 = jnp.uint32
_NT = (((1,), (1,)), ((), ()))


def _attention_order():
    ops = ("Sa0 Sa1 Sa2 Sa3 v0 k1 Pa0 Pa1 Pa2 v1 Sa4 Pa3 k2 Sa5 Wa0 Wa1 Pa4 v2 "
           "Sa6 Wa2 Pa5 Wa3 k3 Sa7 Pa6 Wa4 v3").split()
    for i in range(8, 16):
        ops += [f"Sa{i}", f"Pa{i - 1}", f"Wa{i - 3}"]
    ops += "Sb15 Pa15 Wa13 Sb14 Pb15 Wa14 Sb13 Pb14 Wa15".split()
    for i in range(12, 3, -1):
        ops += [f"Sb{i}", f"Pb{i + 1}", f"Wb{i + 3}"]
    return ops + "Sb3 Sb2 Pb4 Wb6 Sb1 Sb0 Pb3 Pb2 k0 Pb1 Pb0 Wb5 Wb4 Wb3 Wb2 Wb1 Wb0".split()


def _dot(a, b):
    return jnp.dot(a, b, preferred_element_type=F32)


def _bf(words):
    return pltpu.bitcast(words, BF16)


def _words(x):
    return pltpu.bitcast(x.astype(BF16), U32)


def _halves(words):
    return (pltpu.bitcast(words << 16, F32),
            pltpu.bitcast(words & np.uint32(0xFFFF0000), F32))


def _pack(lo, hi):
    lo, hi = (pltpu.bitcast(x, U32) + np.uint32(0x8000) for x in (lo, hi))
    return (lo >> 16) | (hi & np.uint32(0xFFFF0000))


def _repack(lo, hi):
    return (pltpu.bitcast(lo, U32) >> 16) | pltpu.bitcast(hi, U32)


def _pack_all(los, his, exact):
    return [(_repack if any(lo is x for x in exact) else _pack)(lo, hi) for lo, hi in zip(los, his)]


def _words_shuffled(x):
    n, c = x.shape
    x = x.reshape(n // 16, 2, 8, c)
    return _pack(x[:, 0], x[:, 1]).reshape(n // 2, c)


def _recip(x):
    r = pl.reciprocal(x, approx=True)
    return r * (2.0 - x * r)


def _lhs_factors(a11, a12, a21, a22):
    return a11 + a22, a21 + a22, a11, a22, a11 + a12, a21 - a11, a12 - a22


def _rhs_factors(b11, b12, b21, b22):
    return b11 + b22, b11, b12 - b22, b21 - b11, b22, b11 + b12, b21 + b22


def _strassen(mul, order=(2, 3, 4, 1, 0, 6, 5)):
    m = {j + 1: mul(j) for j in order}
    return (m[4] - m[5]) + m[1] + m[7], m[3] + m[5], m[2] + m[4], (m[3] - m[2]) + m[1] + m[6]


def _factors_of_words(factors, *blocks):
    parts = [_halves(b) for b in blocks]
    out = []
    for lo, hi in zip(factors(*[x[0] for x in parts]), factors(*[x[1] for x in parts])):
        plain = [b for b, x in zip(blocks, parts) if x[0] is lo]
        out.append(plain[0] if plain else _pack(lo, hi))
    return out


def _nested_factors(factors, blocks):
    inner = [factors(*[blocks[2 * r + ri][2 * c + ci] for r in range(2) for c in range(2)])
             for ri in range(2) for ci in range(2)]
    return [factors(*[x[j] for x in inner]) for j in range(7)]


def _nested_factors_of_words(factors, blocks):
    sides = [_nested_factors(factors, [[_halves(b)[side] for b in row] for row in blocks])
             for side in range(2)]
    return [[_pack(lo, hi) for lo, hi in zip(a, b)] for a, b in zip(*sides)]


def _nested_strassen(mul, *order):
    blocks = _strassen(lambda j: jnp.concatenate(
        _strassen(lambda k: mul(j, k), *order), axis=0), *order)
    for outer, val in enumerate(blocks):
        n = val.shape[0] // 4
        for inner in range(4):
            yield (2 * (outer // 2) + inner // 2, 2 * (outer % 2) + inner % 2,
                   val[inner * n:(inner + 1) * n])


def _permute_head_columns(words):
    tiles = [words[:, _cols(t)] for t in range(8)]
    lane = lax.broadcasted_iota(jnp.int32, tiles[0].shape, 1)
    for tile_bit, lane_bit in ((4, 16), (1, 8), (2, 1), (4, 64), (1, 32), (4, 4), (1, 2)):
        low = (lane & lane_bit) == 0
        for t in range(8):
            if t & tile_bit:
                continue
            a, b = tiles[t], tiles[t | tile_bit]
            tiles[t] = jnp.where(low, a, pltpu.roll(b, lane_bit, 1))
            tiles[t | tile_bit] = jnp.where(low, pltpu.roll(a, 128 - lane_bit, 1), b)
    return jnp.concatenate(tiles, axis=1)


def _with_corner(x, corner):
    top = corner if x.shape[1] == 128 else jnp.concatenate([corner, x[0:8, 128:]], axis=1)
    return jnp.concatenate([top, x[8:]], axis=0)


class _SideWork:
    def __init__(self):
        self.now = 0
        self.starts = {}
        self.stores = {}

    def add(self, tasks, steps, lag, width=1, phase=0.0):
        for n, task in enumerate(tasks):
            when = steps[int((n + phase) * len(steps)) // len(tasks)]
            self.starts.setdefault(when, []).append((task, lag, width))

    def step(self):
        for task, lag, width in self.starts.pop(self.now, []):
            stores = task()
            for n, store in enumerate(stores):
                self.stores.setdefault(self.now + lag + n * width // len(stores), []).append(store)
        for ref, idx, val in self.stores.pop(self.now, []):
            ref[idx] = val
        self.now += 1

    def check_done(self):
        assert not self.starts and not self.stores


def _mult(i, n):
    return i * n if isinstance(i, int) else pl.multiple_of(i * n, n)


def _wrap(i, n):
    if isinstance(i, int):
        return i % n
    return jnp.where(i >= 2 * n, i - 2 * n, jnp.where(i >= n, i - n, i))


def _cols(t):
    return slice(t * 128, (t + 1) * 128)


def _start(copies):
    for cp in copies:
        cp.start()


def _wait(copies):
    for cp in copies:
        cp.wait()


def _kernel(
    xa_hbm, c_hbm, wq_hbm, wk_hbm, wv_hbm, woa_hbm, xb_hbm, wqkv_hbm, wob_hbm,
    out_hbm,
    x_fac, wide, c, c_sum, kv_fac, k_buf, v_buf, ctx,
    wq_raw, wk_raw, wv_raw, woa_raw, wqkv_raw, wob_raw, obuf,
    sem_x, sem_w, sem_out,
):
    P = functools.partial
    xa32, c32, woa32, xb32, wqkv32 = (
        r.bitcast(U32) for r in (xa_hbm, c_hbm, woa_hbm, xb_hbm, wqkv_hbm))
    wq32, wk32, wv32, wob32 = (r.bitcast(U32) for r in (wq_hbm, wk_hbm, wv_hbm, wob_hbm))

    def pair_copies(src, dst, pair, slot, sem):
        return [pltpu.make_async_copy(
            src.at[:, odd, pair, :], dst.at[slot, odd, 0:src.shape[0]], sem) for odd in range(2)]

    def wq_copies(step):
        sem = sem_w.at[step & 3]
        return [cp for j in range(PP) for cp in pair_copies(
            wq32, wq_raw, step * PP + j, (step & 1) * PP + j, sem)]

    def later_copies(part):
        sem, slot = sem_w.at[(part + 1) & 3], _wrap(part, RING)
        copies = []
        for j in range(PP):
            pair = part * PP + j
            copies += pair_copies(wk32, wk_raw, pair, slot * PP + j, sem)
            copies += pair_copies(wv32, wv_raw, pair, slot * PP + j, sem)
            copies.append(pltpu.make_async_copy(
                wob32.at[:, pair, :], wob_raw.at[slot * PP + j], sem))
        for h in range(2):
            copies.append(pltpu.make_async_copy(
                wqkv32.at[h, pl.ds(_mult(part, PP * 16), PP * 16)],
                wqkv_raw.at[slot, h, 0:PP * 16], sem))
            rows = (2 * (part >> 1) + h, pl.ds(_mult(part & 1, G // 8), G // 8))
            copies.append(pltpu.make_async_copy(c32.at[rows], c.at[rows], sem))
        return copies

    def woa_copy(part):
        return pltpu.make_async_copy(woa32.at[pl.ds(_mult(part, PP * D), PP * D)],
                                     woa_raw.at[part & 1], sem_w.at[part & 1])

    def x_copy(g, lo=0, n=G // 2, sem=None):
        return pltpu.make_async_copy(
            xa32.at[g * G // 2 + lo:g * G // 2 + lo + n], woa_raw.at[g, lo:lo + n],
            sem_x.at[g if sem is None else sem])

    xb_copies = [pltpu.make_async_copy(
        xb32.at[r * S // 8:(r + 1) * S // 8, k * M // 4:(k + 1) * M // 4],
        x_fac.at[4 * r + k], sem_x.at[0]) for r in range(4) for k in range(4)]

    gw = G // 4
    sum_index = {0: 0, 1: 1, 4: 2, 5: 3, 6: 4}

    def head_factors(raw, slot, top, bottom, n):
        even, odd = (_halves(raw[slot, o, top:top + n, :])
                     + _halves(raw[slot, o, bottom:bottom + n, :]) for o in range(2))
        return _pack_all(_rhs_factors(*even), _rhs_factors(*odd), even)

    def group_blocks(g, mul):
        for n, val in enumerate(_strassen(mul, KV_ORDER)):
            r, e = divmod(n, 2)
            yield e, slice((2 * g + r) * gw, (2 * g + r + 1) * gw), val

    def c_factor(g, j):
        if j in sum_index:
            return c_sum[sum_index[j], g * gw:(g + 1) * gw, :]
        return c[2 * g + j - 2, :, (j - 2) * DC // 2:(j - 1) * DC // 2]

    def c_gate(g, j):
        return GATE + 2, slice(8 * (7 * g + j), 8 * (7 * g + j + 1)), _cols(0)

    def project_kv(n, pair, g, side=None):
        def mul(j):
            lhs = c_factor(g, j)
            if side:
                side.step()
                lhs = _with_corner(lhs, wide[c_gate(g, j)])
            return _dot(_bf(lhs), _bf(kv_fac[pair, n, j]))

        for e, rows, val in group_blocks(g, mul):
            val = _words(val)
            (k_buf, v_buf)[n][e, rows, :] = val
            if n == 0 and rows.start == 0:
                ctx[H + e, 0:BQ // 2, :] = val[0:BQ // 2]

    def prepare_kv(n, pair, piece):
        vals = head_factors((wk_raw, wv_raw)[n], _wrap(pair, RING * PP),
                            piece * 16, DC // 4 + piece * 16, 16)
        return [(kv_fac, (pair, n, j, slice(piece * 16, (piece + 1) * 16)), val)
                for j, val in enumerate(vals)]

    def prepare_c(part, piece):
        r = _mult(part & 1, G // 8) + 16 * piece
        vals = _factors_of_words(_lhs_factors, *[
            c[2 * (part >> 1) + h, pl.ds(r, 16), k * DC // 2:(k + 1) * DC // 2]
            for h in range(2) for k in range(2)])
        return [(c_sum, (n, pl.ds(_mult(part >> 1, gw) + r, 16)), vals[j])
                for j, n in sum_index.items()]

    def prepare_wqkv(parts, piece, which):
        moved = _permute_head_columns(jnp.concatenate([
            wqkv_raw[_wrap(part, RING), h, 8 * piece:8 * piece + 8, which * M:(which + 1) * M]
            for part in parts for h in range(2)], axis=0))
        stores = []
        for n, part in enumerate(parts):
            top, bottom = moved[16 * n:16 * n + 8], moved[16 * n + 8:16 * n + 16]
            vals = _factors_of_words(
                _rhs_factors, top[:, :W], top[:, W:], bottom[:, :W], bottom[:, W:])
            r = _mult(part, PP * 16) + 8 * piece
            stores += [(wide, (QKV0 + 7 * which + j, pl.ds(r, 8)), val)
                       for j, val in enumerate(vals)]
        return stores

    def prepare_wob(pair, t):
        b11, b21 = _halves(wob_raw[_wrap(pair, RING * PP), :, _cols(t)])
        b12, b22 = _halves(wob_raw[_wrap(pair, RING * PP), :, _cols(4 + t)])
        r = _mult((pair & 3) * 4 + (pair >> 2), HB // 2)
        return [(wide, (OB0 + j, pl.ds(r, HB // 2), _cols(t)), _words_shuffled(val))
                for j, val in enumerate(_rhs_factors(b11, b12, b21, b22))]

    def prepare_woa(part, t, n):
        fac = _nested_factors_of_words(_rhs_factors, [
            [woa_raw[part & 1, hq * D // 2 + 8 * n:hq * D // 2 + 8 * n + 8,
                     pl.ds(_mult(2 * k + t, 128), 128)]
             for k in range(4)] for hq in range(4)])
        order = (1, 5, 4, 2, 0, 6, 3)
        rows = pl.ds(_mult(part & 3, D // 2) + 8 * n, 8)
        cols = pl.ds(_mult(2 * t + (part >> 2), 128), 128)
        return [(wide, (OA0 + 7 * j + k, rows, cols), fac[j][k]) for j in order for k in order]

    def later_tasks(parts):
        quads = [(part, j, part * PP + j) for part in parts for j in range(PP)]
        return (
            [P(prepare_wqkv, parts, n // 3, n % 3) for n in range(6 * PP)],
            [P(prepare_kv, n % 2, pair, n // 2) for _, _, pair in quads for n in range(16)],
            [task for part, j, pair in quads for n in range(2) for task in (
                P(prepare_wob, pair, 2 * n), P(prepare_c, part, 2 * j + n),
                P(prepare_wob, pair, 2 * n + 1))])

    qw0 = G // 8

    def gate(g, j, k):
        n = 7 * j + k
        return GATE + n // 32, slice(n % 32 * 8, n % 32 * 8 + 8), _cols(g)

    def make_x_factors(g, lo, rows):
        fac = _nested_factors_of_words(_lhs_factors, [
            [woa_raw[g, r * qw0 + lo:r * qw0 + lo + rows, k * M // 4:(k + 1) * M // 4]
             for k in range(4)] for r in range(4)])
        for j in range(7):
            for k in range(7):
                x_fac[7 * j + k, g * qw0 + lo:g * qw0 + lo + rows] = fac[j][k]
                if g % (NG // SPLIT) == 0 and lo == 0:
                    wide[gate(g, j, k)] = fac[j][k][0:8, 0:128]
        return fac

    def wq_factors(step):
        n = M // 8
        sides = [_nested_factors(_rhs_factors, [
            [half for j in range(PP) for half in _halves(
                wq_raw[(step * PP + j) & (2 * PP - 1), odd, k * n:(k + 1) * n, :])]
            for k in range(4)]) for odd in range(2)]
        return [[_pack(even, odd) for even, odd in zip(a, b)] for a, b in zip(*sides)]

    def store_q(step, g, r, head, val, lo=0):
        first = (4 * g + r) * qw0 + lo
        ctx[4 * step + head, first:first + val.shape[0] // 2, :] = _words(
            val * (D ** -0.5 * LOG2E))

    units = [(0, h * qw0 // 2, qw0 // 2) for h in range(2)] + [(g, 0, qw0) for g in range(1, NG)]
    unit_copies = [[x_copy(0, r * qw0 + h * qw0 // 2, qw0 // 2, NG * h) for r in range(4)]
                   for h in range(2)] + [[x_copy(1)], [x_copy(2), x_copy(3)], []]
    _start(wq_copies(0) + [cp for copies in unit_copies for cp in copies]
           + wq_copies(1) + later_copies(0) + later_copies(1))
    _wait(wq_copies(0))

    def kept(j, k):
        return (NP - 1 - j // 2, j % 2, k)

    for j, row in enumerate(wq_factors(0)):
        for k, val in enumerate(row):
            kv_fac[kept(j, k)] = val
    for (g, lo, rows), copies in zip(units, unit_copies):
        _wait(copies)
        lhs = make_x_factors(g, lo, rows)
        for r, head, val in _nested_strassen(
                lambda j, k: _dot(_bf(lhs[j][k]), _bf(kv_fac[kept(j, k)]))):
            store_q(0, g, r, head, val, lo)

    def q_step(step, parts, zero, first, last, *pace):
        side = _SideWork()
        for tasks, (lag, width, phase) in zip(later_tasks(parts), pace):
            side.add(tasks, range(first, min(last, 49 * SPLIT - lag - width + 1)), lag, width, phase)
        fac = wq_factors(step)

        def mul_rows(j, k, n):
            side.step()
            lhs = x_fac[7 * j + k, n * S // 8 // SPLIT:(n + 1) * S // 8 // SPLIT]
            val = _dot(_bf(_with_corner(lhs, wide[gate(n * NG // SPLIT, j, k)])), _bf(fac[j][k]))
            token = pltpu.bitcast(val[0:8], U32)
            wqkv_raw[zero, 0, PP * 16:PP * 16 + 8, _cols(0)] = token
            wk_raw[RING * PP + zero, 0, 0:8] = token
            wv_raw[RING * PP + zero, 0, 0:8] = token
            c[2 * NG + zero, 0:8, _cols(0)] = token
            return val

        for r, head, val in _nested_strassen(lambda j, k: jnp.concatenate(
                [mul_rows(j, k, n) for n in range(SPLIT)], axis=0), Q_ORDER):
            for g in range(NG):
                store_q(step, g, r, head, val[g * G // 4:(g + 1) * G // 4])
        side.check_done()

    def q_body(step, zero):
        _start(wq_copies(step + 1) + later_copies(step + 1))
        _wait(wq_copies(step) + later_copies(step - 1))
        q_step(step, [step - 1], zero, *PACE0)
        return -zero

    zero = lax.fori_loop(1, NS - 1, q_body, 0)
    _wait(wq_copies(NS - 1) + later_copies(NS - 2) + later_copies(NS - 1))
    woa_copy(0).start()
    q_step(NS - 1, [zero + NS - 2, zero + NS - 1], zero, *PACE1)
    project_kv(0, 0, 0)
    for g in range(NG):
        for j in range(7):
            wide[c_gate(g, j)] = c_factor(g, j)[0:8, 0:128]
    kb, vb = 0, KV_ROWS
    for buf in (kb, vb):
        wq_raw[:, :, buf + RC:buf + RC + HALO, :] = jnp.zeros((2 * PP, 2, HALO, D), U32)
    _start(xb_copies)

    def pair_body(p, zero):
        part = p >> 1

        @pl.when((p & 1) == 0)
        def _():
            pl.when(part + 1 < NS)(lambda: woa_copy(part + 1).start())
            woa_copy(part).wait()

        side = _SideWork()
        side.add([P(prepare_woa, part, p & 1, n) for n in range(8)], range(*PACE2[:2]), *PACE2[2:])
        row = lax.broadcasted_iota(jnp.int32, (BQ, BQ), 0)
        col = lax.broadcasted_iota(jnp.int32, (BQ, BQ), 1)
        causal = col <= row
        hb = BQ // 2

        def scores(e, i):
            r = i * BQ
            k = ctx[H + e + zero, 0:hb, :]
            k = _bf(jnp.concatenate([k, k_buf[e, hb:(i + 1) * hb, :]], axis=0) if i else k)
            q = _bf(ctx[2 * p + e, i * hb:(i + 1) * hb, :])
            s = lax.dot_general(q, k, _NT, preferred_element_type=F32)
            diag = jnp.where(causal, s[:, r:], NEG)
            s = jnp.concatenate([s[:, :r], diag], axis=1) if r else diag
            return s, jnp.max(s, axis=1, keepdims=True)

        def context(e, i, s, peak):
            w = jnp.exp2(s - peak)
            total = jnp.sum(w, axis=1, keepdims=True)
            o = _dot(w.astype(BF16), _bf(v_buf[e, 0:(i + 1) * hb, :]))
            return _words(o * _recip(total))

        state = {}
        for op in _attention_order():
            if op[0] in "kv":
                pair = jnp.minimum(p + 1, NP - 1) if op == "k0" else p
                project_kv("kv".index(op[0]), pair, int(op[1:]), side)
                continue
            e, i = "ab".index(op[1]), int(op[2:])
            if op[0] == "S":
                state[e, i] = scores(e, i)
            elif op[0] == "P":
                state[e, i] = context(e, i, *state[e, i])
            else:
                ctx[2 * p + e, i * hb:(i + 1) * hb, :] = state.pop((e, i))
        assert not state
        side.check_done()
        return -zero

    lax.fori_loop(0, NP, pair_body, 0)
    _wait(xb_copies)

    n_chunks = S // RC
    hr = RC // 2
    qw = RC // 8

    def out_copy(i, slot):
        return pltpu.make_async_copy(
            obuf.at[slot], out_hbm.at[pl.ds(_mult(i, RC), RC), :], sem_out.at[slot])

    def last_copy(n):
        lo, hi = ((0, M), (M, M + 256), (M + W, M + W + 256), (M + 256, M + W), (M + W + 256, 2 * M))[n]
        return pltpu.make_async_copy(
            obuf.at[1, :, lo:hi], out_hbm.at[S - RC:S, lo:hi], sem_out.at[1])

    def chunk_body(i, zero, last=False):
        slot = i & 1
        base = _mult(i, RC // 2)

        @pl.when(i >= 2)
        def _():
            out_copy(i - 2, slot).wait()

        def is_plain(j, k):
            return j in (2, 3) and k in (2, 3)

        def ctx_at(j, k, u, lo, n):
            if is_plain(j, k):
                quarter = 2 * (j - 2) + k - 2
                return ctx, (4 * u + quarter, pl.ds(base + quarter * qw + lo, n))
            slab, r = divmod((2 * (7 * j + k) + u // 4) * qw + lo, SLAB)
            return wide, (CS0 + slab, slice(r, r + n), _cols(u % 4))

        ctx_fac = {}

        def ctx_factor_store(u, lo, j, k):
            if (u, lo) not in ctx_fac:
                ctx_fac[u, lo] = _nested_factors_of_words(_lhs_factors, [
                    [ctx[4 * u + hq, pl.ds(base + r * qw + lo, 8)] for hq in range(4)]
                    for r in range(4)])
            return [ctx_at(j, k, u, lo, 8) + (ctx_fac[u, lo][j][k],)]

        def taps(buf, t, w, r):
            lo = buf + HALO - DIL * w + r
            return pltpu.bitcast(wq_raw[t // 2, t % 2, lo:lo + 8, :], F32)

        def tile_at(n, r, rows):
            return n // 4, slice(n % 4 * RC + r, n % 4 * RC + r + rows)

        q_alias = v_buf.at[pl.ds(zero, 2)]
        logit_alias = k_buf.at[pl.ds(zero, 2)]

        def window_logits(r, ws):
            q = [pltpu.bitcast((v_buf if t else q_alias)[tile_at(t, r, 8)], F32) for t in range(8)]
            logits = [functools.reduce(jnp.add, [q[t] * taps(kb, t, w, r) for t in range(8)])
                      for w in ws]
            logits = [z + pltpu.roll(z, 64, 1) for z in logits]
            logits = [(z + pltpu.roll(z, 32, 1)) * (DB ** -0.5 * LOG2E) for z in logits]
            pos = i * RC + r + lax.broadcasted_iota(jnp.int32, (8, 128), 0)
            return [(k_buf, tile_at(w, r, 8), pltpu.bitcast(
                jnp.where(pos >= DIL * w, z, NEG) if DIL * w > r else z, U32))
                for w, z in zip(ws, logits)]

        weights = {}

        def window_softmax(r):
            logits = [pltpu.bitcast((k_buf if w else logit_alias)[tile_at(w, r, 8)], F32)
                      for w in range(WIN)]
            peak = functools.reduce(jnp.maximum, logits)
            probs = [jnp.exp2(z - peak) for z in logits]
            inv = _recip(functools.reduce(jnp.add, probs))
            weights[r] = [z * inv for z in probs]
            return []

        def window_values(r, ts):
            return [(wide, (LOC0 + r // hr,
                            slice(r % hr + (t // 2 % 2) * hr, r % hr + (t // 2 % 2) * hr + 8),
                            _cols(t // 4 * 2 + t % 2)),
                     pltpu.bitcast(functools.reduce(
                         jnp.add, [weights[r][w] * taps(vb, t, w, r) for w in range(WIN)]), U32))
                    for t in ts]

        n_steps = 3 * 4 * 7 + 2 * 49
        order = (2, 4, 3, 1, 0, 6, 5)
        side = _SideWork()
        side.add([P(ctx_factor_store, u, lo, j, k) for u in range(8) for lo in range(0, qw, 8)
                  for j in order for k in order if not is_plain(j, k)], range(CTX_FIRST, CTX_LAST), 0)
        side.add([P(window_logits, r, ws) for r in range(0, RC, 8)
                  for ws in ((0, 4, 1, 5), (2, 6, 3, 7))],
                 range(LOGIT_FIRST, LOGIT_LAST - LOGIT_LAG), LOGIT_LAG)
        side.add([P(window_softmax, r) for r in range(0, RC, 8)],
                 range(VALUE_FIRST, n_steps - 2), 0)
        side.add([P(window_values, r, ts) for r in range(0, RC, 8)
                  for ts in (range(4), range(4, 8))], range(VALUE_FIRST + 2, n_steps), 0)
        wide_alias = wide.at[pl.ds(zero, CS0)]

        def mul(lhs, slab, *tiles):
            side.step()
            rhs = jnp.concatenate([wide[slab, :, _cols(t)] for t in tiles], axis=0)
            rhs = _with_corner(rhs, wide_alias[slab, 0:8, _cols(tiles[0])])
            val = _dot(_bf(lhs), _bf(rhs))
            for buf in (k_buf, v_buf):
                buf[0, S // 2:S // 2 + 8, :] = pltpu.bitcast(val[0:8], U32)
            return val

        xb_fac = _factors_of_words(_lhs_factors, *[
            jnp.concatenate([
                x_fac[4 * (i >> 1) + 2 * k + t, pl.ds(_mult(2 * (i & 1) + r, hr // 2), hr // 2)]
                for t in range(2)], axis=1) for r in range(2) for k in range(2)])
        for part, buf in ((1, kb), (0, None), (2, vb)):
            if part:
                wq_raw[:, :, buf:buf + HALO, :] = wq_raw[:, :, buf + RC:buf + RC + HALO, :]
            for t in range(4):
                blocks = _strassen(lambda j: mul(xb_fac[j], QKV0 + 7 * part + j, t), B_ORDER)
                for n, val in enumerate(blocks):
                    r, k = divmod(n, 2)
                    if part:
                        lo = buf + HALO + r * hr
                        wq_raw[2 * k + t // 2, t % 2, lo:lo + hr, :] = pltpu.bitcast(val, U32)
                    else:
                        v_buf[tile_at(4 * k + t, r * hr, hr)] = pltpu.bitcast(val, U32)

        def ctx_factor(j, k):
            return jnp.concatenate(
                [ref[idx] for ref, idx in (ctx_at(j, k, u, 0, qw) for u in range(8))], axis=1)

        for t in range(2):
            for r, k, val in _nested_strassen(
                    lambda j, k: mul(ctx_factor(j, k), OA0 + 7 * j + k, 2 * t, 2 * t + 1)):
                obuf[slot, r * RC // 4:(r + 1) * RC // 4, _cols(2 * k + t)] = val.astype(BF16)
        side.check_done()
        if last:
            last_copy(0).start()

        o_fac = [z.astype(BF16) for z in _lhs_factors(*[
            pltpu.bitcast(wide[LOC0 + r, e * hr:(e + 1) * hr, :], F32)
            for r in range(2) for e in range(2)])]
        for t in range(4):
            blocks = _strassen(lambda j: _dot(o_fac[j], _bf(wide[OB0 + j, :, _cols(t)])))
            for n, val in enumerate(blocks):
                r, k = divmod(n, 2)
                obuf[slot, r * hr:(r + 1) * hr, _cols(8 + 4 * k + t)] = val.astype(BF16)
            if last and t == 1:
                _start([last_copy(1), last_copy(2)])

        if last:
            _start([last_copy(n) for n in range(3, 5)])
        else:
            out_copy(i, slot).start()
        return -zero

    zero = lax.fori_loop(0, n_chunks - 1, chunk_body, 0)
    chunk_body(n_chunks - 1, zero, last=True)
    out_copy(n_chunks - 2, 0).wait()
    _wait([last_copy(n) for n in range(5)])


@jax.jit
def pallas_concat_heads__compressed_kv_cla__sliding_local_dilated__prompt_kernel(
    A_x: jax.Array,
    A_c_kv: jax.Array,
    A_w_q: jax.Array,
    A_w_uk: jax.Array,
    A_w_uv: jax.Array,
    A_w_o: jax.Array,
    B_x: jax.Array,
    B_wqkv: jax.Array,
    B_wo: jax.Array,
):
    scratch = [
        pltpu.VMEM((49, S // 8, M // 4), U32),
        pltpu.VMEM((N_SLABS, SLAB, W), U32),
        pltpu.VMEM((2 * NG + 1, G // 4, DC), U32),
        pltpu.VMEM((5, S // 4, DC // 2), U32),
        pltpu.VMEM((NP, 2, 7, DC // 4, D), U32),
        pltpu.VMEM((2, S // 2 + 8, D), U32),
        pltpu.VMEM((2, S // 2 + 8, D), U32),
        pltpu.VMEM((H + 2, S // 2, D), U32),
        pltpu.VMEM((2 * PP, 2, 2 * KV_ROWS + 8, D), U32),
        pltpu.VMEM((RING * PP + 1, 2, DC // 2, D), U32),
        pltpu.VMEM((RING * PP + 1, 2, DC // 2, D), U32),
        pltpu.VMEM((NG, PP * D, M), U32),
        pltpu.VMEM((RING, 2, PP * 16 + 8, 3 * M), U32),
        pltpu.VMEM((RING * PP, HB, M), U32),
        pltpu.VMEM((2, RC, 2 * M), BF16),
        pltpu.SemaphoreType.DMA((NG + 1,)),
        pltpu.SemaphoreType.DMA((4,)),
        pltpu.SemaphoreType.DMA((2,)),
    ]
    out = pl.pallas_call(
        _kernel,
        out_shape=jax.ShapeDtypeStruct((S, 2 * M), BF16),
        in_specs=[pl.BlockSpec(memory_space=pl.ANY)] * 9,
        out_specs=pl.BlockSpec(memory_space=pl.ANY),
        scratch_shapes=scratch,
        compiler_params=pltpu.CompilerParams(
            vmem_limit_bytes=127 * 2**20, disable_bounds_checks=True),
        name="fused_mla_sliding",
    )(
        A_x.reshape(S, M),
        A_c_kv.reshape(2 * NG, G // 2, DC),
        A_w_q.reshape(M // 2, 2, H, D),
        A_w_uk.reshape(DC // 2, 2, H, D),
        A_w_uv.reshape(DC // 2, 2, H, D),
        A_w_o.reshape(H * D, M),
        B_x.reshape(S, M),
        B_wqkv.reshape(2, M // 2, 3 * M),
        B_wo.reshape(HB, DB, M),
    )
    return out.reshape(1, S, 2 * M)
```
